```python
import jax
import jax.numpy as jnp

def _softmax(x, axis=-1):
    return jax.nn.softmax(x, axis=axis)
def _gelu(x):
    return jax.nn.gelu(x, approximate=True)
def _silu(x):
    return jax.nn.silu(x)
def _sigmoid(x):
    return jax.nn.sigmoid(x)
def _layernorm(x, axis=-1, eps=1e-5):
    m = jnp.mean(x, axis=axis, keepdims=True)
    v = jnp.var(x, axis=axis, keepdims=True)
    return (x - m) / jnp.sqrt(v + eps)
def _scatter_add(tgt, idx, src, axis=0):
    return tgt.at[idx].add(src)
def _segment_sum(src, seg, n):
    return jax.ops.segment_sum(src, seg, n)
class _Rng:
    def __init__(self, key):
        self._k = key
    def _next(self):
        self._k, sub = jax.random.split(self._k)
        return sub
    def normal(self, shape):
        return jax.random.normal(self._next(), shape, dtype=jnp.bfloat16)
    def randint(self, lo, hi, shape):
        return jax.random.randint(self._next(), shape, lo, hi, dtype=jnp.int32)
    def uniform(self, shape, lo=0.0, hi=1.0):
        return jax.random.uniform(self._next(), shape, jnp.bfloat16, lo, hi)
    def permutation(self, n):
        return jax.random.permutation(self._next(), n)


kernel_name = 'interleave_layers__sliding_local_dilated__glu_gated_bilinear__prompt'

def setup_inputs():
    _rng = _Rng(jax.random.key(int.from_bytes(__import__("os").urandom(4), "little")))
    _w = (lambda a: (lambda t: t.astype(jnp.bfloat16) if jnp.issubdtype(t.dtype, jnp.floating) else t)(jnp.asarray(a)))
    def _A_setup():
        B, S, D = 1, 2048, 576
        return {
            "x": _w((lambda *s: _rng.normal(s) * 0.05)(B, S, D)),
            "wqkv": _w((lambda *s: _rng.normal(s) * 0.05)(D, 3 * D)),
            "wo": _w((lambda *s: _rng.normal(s) * 0.05)(D, D)),
        }
    _A_in = _A_setup()

    def _B_setup():
        B, S, D, F = 1, 2048, 576, 4608
        return {
            "x": _w((lambda *s: _rng.normal(s) * 0.05)(B, S, D)),
            "w_gate": _w((lambda *s: _rng.normal(s) * 0.05)(D, F) * (D ** -0.5)),
            "w_up": _w((lambda *s: _rng.normal(s) * 0.05)(D, F) * (D ** -0.5)),
            "w_down": _w((lambda *s: _rng.normal(s) * 0.05)(F, D) * (F ** -0.5)),
        }
    _B_in = _B_setup()

    return {
        "A_x": _A_in["x"],
        "A_wqkv": _A_in["wqkv"],
        "A_wo": _A_in["wo"],
        "B_x": _B_in["x"],
        "B_w_gate": _B_in["w_gate"],
        "B_w_up": _B_in["w_up"],
        "B_w_down": _B_in["w_down"],
    }

def reference(A_x, A_wqkv, A_wo, B_x, B_w_gate, B_w_up, B_w_down):
    def _A_ref(x, wqkv, wo):
        B, S, D = x.shape
        H = 32; Dh = D // H
        W, dil = 8, 2
        qkv = (lambda x, *d: x.transpose(*d))((x @ wqkv).reshape(B, S, 3, H, Dh), 2, 0, 3, 1, 4)
        q, k, v = qkv[0], qkv[1], qkv[2]
        scale = Dh ** -0.5
        pos = jnp.arange(S)
        off = jnp.arange(W) * dil
        idx = pos[:, None] - off[None, :]
        mask = idx >= 0
        idx_c = jnp.where(mask, idx, 0).reshape(-1)
        kg = k[:, :, idx_c, :].reshape(B, H, S, W, Dh)
        vg = v[:, :, idx_c, :].reshape(B, H, S, W, Dh)
        logits = jnp.einsum("bhsd,bhswd->bhsw", q, kg) * scale
        logits = jnp.where(mask[None, None, :, :], logits, -1e9)
        attn = _softmax(logits, axis=-1)
        o = jnp.einsum("bhsw,bhswd->bhsd", attn, vg)
        return (lambda x, *d: x.transpose(*d))(o, 0, 2, 1, 3).reshape(B, S, D) @ wo

    def _B_ref(x, w_gate, w_up, w_down):
        g = jnp.einsum("bsd,df->bsf", x, w_gate)
        u = jnp.einsum("bsd,df->bsf", x, w_up)
        h = g * u
        return jnp.einsum("bsf,fd->bsd", h, w_down)

    x = A_x
    x = x + _A_ref(_layernorm(x, axis=-1), A_wqkv, A_wo)
    x = x + _B_ref(_layernorm(x, axis=-1), B_w_gate, B_w_up, B_w_down)
    x = x + _A_ref(_layernorm(x, axis=-1), A_wqkv, A_wo)
    x = x + _B_ref(_layernorm(x, axis=-1), B_w_gate, B_w_up, B_w_down)
    return x
```

```python
import math

import jax
import jax.numpy as jnp
from jax import lax
import jax.experimental.pallas as pl
import jax.experimental.pallas.tpu as pltpu

S, D, F = 2048, 576, 4608
H, DH, W = 32, 18, 8
NT_ = 8
TQ = 256
MQ = D // 4
FC = 512
NC = F // FC
RING = 3
EPS = 1e-5
SCALE = DH ** -0.5
EXP_C = SCALE * math.log2(math.e)
NEG = -1e9 / SCALE

BF, F32, U32 = jnp.bfloat16, jnp.float32, jnp.uint32
NT_DIMS = (((1,), (1,)), ((), ()))

LHS_SEL = {0: ((0, 0), 1, (1, 1)), 1: ((1, 0), 1, (1, 1)), 2: ((0, 0), 0, None), 3: ((1, 1), 0, None),
           4: ((0, 0), 1, (0, 1)), 5: ((1, 0), -1, (0, 0)), 6: ((0, 1), -1, (1, 1))}
RHS_SEL = {0: ((0, 0), 1, (1, 1)), 1: ((0, 0), 0, None), 2: ((0, 1), -1, (1, 1)), 3: ((1, 0), -1, (0, 0)),
           4: ((1, 1), 0, None), 5: ((0, 0), 1, (0, 1)), 6: ((1, 0), 1, (1, 1))}
G_ORDER = (0, 1, 2, 5, 3, 4, 6)


def _lhs1(a11, a12, a21, a22):
    return [a11 + a22, a21 + a22, a11, a22, a11 + a12, a21 - a11, a12 - a22]


def _rhs1(b11, b12, b21, b22):
    return [b11 + b22, b11, b12 - b22, b21 - b11, b22, b11 + b12, b21 + b22]


def _out1(m):
    return (m[0] + m[3] - m[4] + m[6], m[2] + m[4], m[1] + m[3], m[0] - m[1] + m[2] + m[5])


def _in2(fn, x):
    outer = [[fn(x[i][j], x[i][2 + j], x[2 + i][j], x[2 + i][2 + j]) for j in range(2)] for i in range(2)]
    return [v for a in range(7) for v in fn(outer[0][0][a], outer[0][1][a], outer[1][0][a], outer[1][1][a])]


def _out2(m):
    p = [_out1(m[7 * a:7 * a + 7]) for a in range(7)]
    c = [[None] * 4 for _ in range(4)]
    for q in range(4):
        i, j = q // 2, q % 2
        c[i][j], c[i][2 + j], c[2 + i][j], c[2 + i][2 + j] = _out1([p[a][q] for a in range(7)])
    return c


def _select(sel, load):
    first, sign, second = sel
    v = load(first)
    if sign == 1:
        v = [a + b for a, b in zip(v, load(second))]
    elif sign == -1:
        v = [a - b for a, b in zip(v, load(second))]
    return v


def _pk(lo, hi):
    return pltpu.pack_elementwise([lo, hi], packed_dtype=BF)


def _lo(w):
    return pltpu.unpack_elementwise(w, index=0, packed_dtype=BF, unpacked_dtype=F32)


def _hi(w):
    return pltpu.unpack_elementwise(w, index=1, packed_dtype=BF, unpacked_dtype=F32)


def _bf(w):
    return pltpu.bitcast(w, BF)


def _dot(a, b):
    return jnp.dot(a, b, preferred_element_type=F32)


def _layernorm_t(x):
    m = jnp.sum(x, axis=0, keepdims=True) * (1.0 / D)
    d = x - m
    v = jnp.sum(d * d, axis=0, keepdims=True) * (1.0 / D)
    return d * lax.rsqrt(v + EPS)


def _kernel(zero_ref, x_hbm, wqkv_hbm, wo_hbm, wg_hbm, wu_hbm, wd_hbm, out_hbm,
            xio, wqkv_raw, wo_raw, wg_raw, wu_raw, wd_raw, tg, tu,
            wts, wqkv_t, wo_t, xt, xn, kv, qb, pb, ob, xf,
            a_ref, at_ref, acc, h_ref, ti, to, hf, r_ref, l_ref, wt_ref, sems):
    z = zero_ref[0]

    def slab(kt):
        return pl.ds(128 * kt, 128 if kt < 4 else 64)

    def cp_x(kt):
        return pltpu.make_async_copy(x_hbm.at[:, slab(kt)], xio.at[:, slab(kt)], sems.at[kt])

    def cp_out(kt):
        return pltpu.make_async_copy(xio.at[:, slab(kt)], out_hbm.at[:, slab(kt)], sems.at[kt])

    qkv_cols = {"k": pl.ds(512, 640), "v": pl.ds(1152, 576), "q": pl.ds(0, 512)}

    def cp_qkv(name):
        idx = 5 + "kvq".index(name)
        return pltpu.make_async_copy(wqkv_hbm.at[:, qkv_cols[name]], wqkv_raw.at[:, qkv_cols[name]], sems.at[idx])

    def cp_wo():
        return pltpu.make_async_copy(wo_hbm, wo_raw, sems.at[8])

    def cp_ffn(c):
        c0 = c * FC if isinstance(c, int) else pl.multiple_of(c * FC, FC)
        cols = pl.ds(c0, FC)
        slot = c % RING
        return (pltpu.make_async_copy(wg_hbm.at[0:512, cols], wg_raw.at[slot], sems.at[11 + 3 * slot]),
                pltpu.make_async_copy(wu_hbm.at[0:512, cols], wu_raw.at[slot], sems.at[12 + 3 * slot]),
                pltpu.make_async_copy(wd_hbm.at[cols, :], wd_raw.at[slot], sems.at[13 + 3 * slot]))

    def cp_tails():
        return (pltpu.make_async_copy(wg_hbm.at[512:D, :], tg, sems.at[9]),
                pltpu.make_async_copy(wu_hbm.at[512:D, :], tu, sems.at[10]))

    def transpose_cols(src, nb0, ncols):
        for nb in range(nb0, nb0 + 5):
            wn = min(128, ncols - 128 * nb)
            for kt in range(5):
                wk = 128 if kt < 4 else 64
                blk = src[128 * kt:128 * kt + wk, 128 * nb:128 * nb + wn].astype(F32)
                wts[kt, 128 * (nb - nb0):128 * (nb - nb0) + wn, 0:wk] = blk.T

    def setup_qkv(name):
        part = "qkv".index(name)
        nb0 = (D * part) // 128
        base = D * part - 128 * nb0
        transpose_cols(wqkv_raw, nb0, D * part + D)
        for d in range(DH):
            for kt in range(5):
                wk = 128 if kt < 4 else 64
                lo = wts[kt, pl.ds(base + d, 16, stride=2 * DH), :][:, :wk]
                hi = wts[kt, pl.ds(base + d + DH, 16, stride=2 * DH), :][:, :wk]
                wqkv_t[part, 16 * d:16 * d + 16, 128 * kt:128 * kt + wk] = _pk(lo, hi)

    def setup_wo():
        for nb in range(5):
            wn = 128 if nb < 4 else 64
            xf[nb, 0:D, 0:wn] = wo_raw[:, 128 * nb:128 * nb + wn].astype(F32)
        for nb in range(5):
            wn = 128 if nb < 4 else 64
            rows = []
            for d in range(DH):
                for sl in range(2):
                    lo = xf[nb, pl.ds(16 * sl * DH + d, 8, stride=DH), :][:, :wn]
                    hi = xf[nb, pl.ds((16 * sl + 8) * DH + d, 8, stride=DH), :][:, :wn]
                    rows.append(_pk(lo, hi))
            wo_raw[:, 128 * nb:128 * nb + wn] = _bf(jnp.concatenate(rows, axis=0))
        transpose_cols(wo_raw, 0, D)
        for kt in range(5):
            wk = 128 if kt < 4 else 64
            lo = wts[kt, pl.ds(0, D // 2, stride=2), :][:, :wk]
            hi = wts[kt, pl.ds(1, D // 2, stride=2), :][:, :wk]
            wo_t[:, 128 * kt:128 * kt + wk] = _pk(lo, hi)

    def setup_x(kt):
        wk = 128 if kt < 4 else 64
        xf[kt, :, 0:wk] = pltpu.bitcast(xio[:, 128 * kt:128 * kt + wk], F32)
        for r in range(NT_):
            w = xf[kt, pl.ds(r, 128, stride=8), :][:, :wk]
            w = pltpu.bitcast(w.T, U32)
            xt[0, r, 128 * kt:128 * kt + wk, :] = _lo(w)
            xt[1, r, 128 * kt:128 * kt + wk, :] = _hi(w)

    def prep_r(c, a):
        slot = c % RING
        for w_ref, off in ((wg_raw, 0), (wu_raw, 128)):
            for g in range(8):
                def load(quad):
                    ws = [pltpu.bitcast(w_ref[slot, pl.ds(128 * (2 * quad[0] + i) + 16 * g, 16),
                                              pl.ds(256 * quad[1], 256)], U32) for i in range(2)]
                    ws = [w[:, 128 * j:128 * j + 128] for w in ws for j in range(2)]
                    return [_lo(w) for w in ws] + [_hi(w) for w in ws]
                v = _select(RHS_SEL[a], load)
                for b, (lo, hi) in enumerate(zip(_rhs1(*v[:4]), _rhs1(*v[4:]))):
                    r_ref[c, 7 * a + b, 8 * g:8 * g + 8, off:off + 128] = _pk(lo, hi)

    def prep_l(c):
        slot = c % RING
        for j in range(4):
            wt_ref[z + j] = wd_raw[slot, 128 * j:128 * j + 128, :].astype(F32).T
        for g in range(MQ // 16):
            ld = lambda e: [[wt_ref[z + j, pl.ds(MQ * i + 16 * g + e, 8, stride=2), :] for j in range(4)]
                            for i in range(4)]
            for k, (lo, hi) in enumerate(zip(_in2(_lhs1, ld(0)), _in2(_lhs1, ld(1)))):
                l_ref[c, k, 8 * g:8 * g + 8, :] = _pk(lo, hi)

    def prep_a(a):
        for half in range(2):
            for g in range(8):
                def load(quad):
                    return [xf[2 * quad[1] + j, pl.ds(TQ * (2 * quad[0] + i) + 32 * g + half + e, 8, stride=4), :]
                            for e in (0, 2) for i in range(2) for j in range(2)]
                v = _select(LHS_SEL[a], load)
                for b, (lo, hi) in enumerate(zip(_lhs1(*v[:4]), _lhs1(*v[4:]))):
                    a_ref[z + 7 * a + b, 64 * half + 8 * g:64 * half + 8 * g + 8, :] = _pk(lo, hi)

    def prep_a_tail():
        for i in range(4):
            for half in range(2):
                lo = xf[4, pl.ds(TQ * i + half, 64, stride=4), :][:, :64]
                hi = xf[4, pl.ds(TQ * i + half + 2, 64, stride=4), :][:, :64]
                at_ref[z + i, 64 * half:64 * half + 64, :] = _pk(lo, hi)

    def gate_up(c, before=None, late=None):
        c0 = c * FC if isinstance(c, int) else pl.multiple_of(c * FC, FC)

        def inner(a, emit):
            if before is not None:
                before(a)
            prod = lambda b: _dot(_bf(a_ref[z + 7 * a + b]), _bf(r_ref[c, 7 * a + b]))
            ld = lambda s: ti[z + s]
            for s in range(3):
                ti[z + s] = prod(s)
            emit(3, ((ld(0) - ld(1)) + ld(2)) + prod(5))
            m3 = prod(3)
            emit(2, ld(1) + m3)
            ti[z + 3] = ld(0) + m3
            m4 = prod(4)
            emit(1, ld(2) + m4)
            ti[z + 3] = ld(3) - m4
            emit(0, ld(3) + prod(6))

        def fin(quad, q, v):
            i, j = 2 * (quad // 2) + q // 2, 2 * (quad % 2) + q % 2
            cols = pl.ds(c0 + 128 * j, 128)
            wt = jnp.concatenate([tg[:, cols], tu[:, cols]], axis=1)
            v = v + _dot(_bf(at_ref[z + i]), wt)
            hf[z + 4 * quad + q] = v[:, :128] * v[:, 128:]

        def old(s, q):
            return to[z + 4 * s + q]

        def keep(s):
            def emit(q, v):
                to[z + 4 * s + q] = v
            return emit

        def put(a):
            if late is not None and a in (0, 1, 3, 5):
                late(a)
            for g in range(16):
                def load(quad):
                    return [hf[z + 4 * (2 * quad[1] + quad[0]) + t, pl.ds(o + 8 * g, 8), :]
                            for o in (0, 128) for t in (0, 2, 1, 3)]
                v = _select(RHS_SEL[a], load)
                for b, (lo, hi) in enumerate(zip(_rhs1(*v[:4]), _rhs1(*v[4:]))):
                    h_ref[7 * a + b, 8 * g:8 * g + 8, :] = _pk(lo, hi)

        def emit3(q, v):
            fin(2, q, old(1, q) + v)
            to[z + 12 + q] = old(0, q) + v

        def emit4(q, v):
            fin(1, q, old(2, q) + v)
            to[z + 12 + q] = old(3, q) - v

        inner(0, keep(0))
        inner(1, keep(1))
        inner(2, keep(2))
        inner(5, lambda q, v: fin(3, q, ((old(0, q) - old(1, q)) + old(2, q)) + v))
        put(4)
        inner(3, emit3)
        put(2)
        inner(4, emit4)
        put(6)
        inner(6, lambda q, v: fin(0, q, old(3, q) + v))
        for a in (0, 3, 5, 1):
            put(a)

    def down(s, c, a):
        for k in range(7 * a, 7 * a + 7):
            prev = acc[s, k]
            if not isinstance(c, int):
                prev = jnp.where(c == 0, 0.0, prev)
            acc[s, k] = prev + lax.dot_general(_bf(l_ref[c, k]), _bf(h_ref[k]), NT_DIMS,
                                               preferred_element_type=F32)

    def finalize(s, lane_half, valid=None):
        for g in range(MQ // 8):
            m = [acc[s, k, 8 * g:8 * g + 8, 128 * lane_half:128 * lane_half + 128] for k in range(49)]
            c = _out2(m)
            for i in range(4):
                for j in range(4):
                    v = c[i][j] if valid is None else jnp.where(valid, c[i][j], 0.0)
                    rows = pl.ds(MQ * i + 8 * g, 8)
                    xt[s, 2 * j + lane_half, rows, :] = xt[s, 2 * j + lane_half, rows, :] + v

    def ln1(s, e):
        for t in range(4):
            xn[z + e, :, 128 * t:128 * t + 128] = _layernorm_t(xt[s, 2 * t + e]).astype(BF)

    def project(name, e):
        y = _dot(_bf(wqkv_t["qkv".index(name)]), xn[z + e])
        for t in range(4):
            r = 2 * t + e
            tile = y[:, 128 * t:128 * t + 128]
            if name == "q":
                qb[z + r] = tile
            else:
                u = 0 if name == "k" else 1
                kv[z + u, 7 + r] = tile
                if r >= 1:
                    kv[z + u, r - 1] = pltpu.roll(tile, 1, 1)

    def scores(r):
        lane0 = lax.broadcasted_iota(jnp.int32, (16, 128), 1) == 0
        for sl in range(2):
            lg = [None] * W
            for d in range(DH):
                rows = pl.ds(32 * d + 16 * sl, 16)
                q = qb[z + r, rows, :]
                for w in range(W):
                    t = q * kv[z, 7 + r - w, rows, :]
                    lg[w] = t if d == 0 else lg[w] + t
            lg = [jnp.where(lane0, NEG, lg[w]) if w > r else lg[w] for w in range(W)]
            m = lg[0]
            for w in range(1, W):
                m = jnp.maximum(m, lg[w])
            ex = [jnp.exp2((lg[w] - m) * EXP_C) for w in range(W)]
            tot = ex[0]
            for w in range(1, W):
                tot = tot + ex[w]
            inv = 1.0 / tot
            for w in range(W):
                pb[z + r, w, 16 * sl:16 * sl + 16, :] = ex[w] * inv

    def mix(r):
        for sl in range(2):
            p = [pb[z + r, w, 16 * sl:16 * sl + 16, :] for w in range(W)]
            for d in range(DH):
                rows = pl.ds(32 * d + 16 * sl, 16)
                o = p[0] * kv[z + 1, 7 + r, rows, :]
                for w in range(1, W):
                    o = o + p[w] * kv[z + 1, 7 + r - w, rows, :]
                ob[z + r, 16 * d + 8 * sl:16 * d + 8 * sl + 8, :] = _pk(o[:8], o[8:])

    def out_proj(s, r):
        x = xt[s, r] + _dot(_bf(wo_t[...]), _bf(ob[z + r]))
        xt[s, r] = x
        y = _layernorm_t(x)
        for kt in range(5):
            wk = 128 if kt < 4 else 64
            xf[kt, 128 * r:128 * r + 128, 0:wk] = y[128 * kt:128 * kt + wk].T

    def attention_block(p, first):
        s = 0 if first else p % 2
        prev = 1 - s
        filler = (lambda a: None) if first else (lambda a: down(prev, NC - 1, a))
        filler(4)
        for e in range(2):
            if not first:
                finalize(s, e, p >= 2)
            ln1(s, e)
        for e in range(2):
            project("k", e)
        if first:
            cp_qkv("q").wait()
            setup_qkv("q")
        for e in range(2):
            project("q", e)
        if first:
            cp_qkv("v").wait()
            setup_qkv("v")
        for e in range(2):
            project("v", e)
        if first:
            cp_wo().wait()
            setup_wo()
        for r in range(NT_):
            scores(r)
        filler(2)
        for r in range(NT_):
            mix(r)
            out_proj(s, r)
        filler(6)
        if first:
            for cp in cp_ffn(0) + cp_tails():
                cp.wait()
        prep_a_tail()

        def before(a):
            prep_a(a)
            if first:
                prep_r(0, a)
        if first:
            prep_l(0)
        gate_up(0, before, None if first else filler)

    def ffn_loop(s, first):
        def body(c, carry):
            if first:
                for cp in cp_ffn(c + 1):
                    cp.wait()

                @pl.when(c + RING < NC)
                def _():
                    for cp in cp_ffn(c + RING):
                        cp.start()
            for a in (4, 2, 6):
                down(s, c, a)
            if first:
                prep_l(c + 1)
            gate_up(c + 1, (lambda a: prep_r(c + 1, a)) if first else None, lambda a: down(s, c, a))
            return carry
        lax.fori_loop(0, NC - 1, body, 0)

    cp_qkv("k").start()
    for kt in range(5):
        cp_x(kt).start()
    cp_qkv("q").start()
    cp_qkv("v").start()
    cp_wo().start()
    for cp in cp_ffn(0) + cp_tails():
        cp.start()
    for c in range(1, RING):
        for cp in cp_ffn(c):
            cp.start()

    cp_qkv("k").wait()
    setup_qkv("k")
    for kt in range(5):
        cp_x(kt).wait()
        setup_x(kt)

    attention_block(0, True)
    ffn_loop(0, True)

    def pass_body(p, carry):
        attention_block(p, False)
        ffn_loop(p % 2, False)
        return carry
    lax.fori_loop(1, 4, pass_body, 0)

    for a in range(7):
        down(1, NC - 1, a)
    for s in range(2):
        for e in range(2):
            finalize(s, e)
    for kt in range(5):
        wk = 128 if kt < 4 else 64
        for r in range(NT_):
            w = _pk(xt[0, r, 128 * kt:128 * kt + wk, :], xt[1, r, 128 * kt:128 * kt + wk, :])
            w = pltpu.bitcast(w, F32).T
            if wk < 128:
                w = jnp.concatenate([w, jnp.zeros((128, 128 - wk), F32)], axis=1)
            xf[kt, pl.ds(r, 128, stride=8), :] = w
        xio[:, 128 * kt:128 * kt + wk] = _bf(xf[kt, :, 0:wk])
        cp_out(kt).start()
    for kt in range(5):
        cp_out(kt).wait()


@jax.jit
def pallas_interleave_layers__sliding_local_dilated__glu_gated_bilinear__prompt_kernel(
    A_x: jax.Array,
    A_wqkv: jax.Array,
    A_wo: jax.Array,
    B_x: jax.Array,
    B_w_gate: jax.Array,
    B_w_up: jax.Array,
    B_w_down: jax.Array,
):
    del B_x
    vm = pltpu.VMEM
    scratch = [
        vm((S, D), BF), vm((D, 3 * D), BF), vm((D, D), BF),
        vm((RING, 512, FC), BF), vm((RING, 512, FC), BF), vm((RING, FC, D), BF),
        vm((D - 512, F), BF), vm((D - 512, F), BF),
        vm((5, 640, 128), F32),
        vm((3, D // 2, D), U32),
        vm((D // 2, D), U32),
        vm((2, NT_, D, 128), F32),
        vm((2, D, 512), BF),
        vm((2, 15, D, 128), F32),
        vm((NT_, D, 128), F32),
        vm((NT_, W, H, 128), F32),
        vm((NT_, D // 2, 128), U32),
        vm((5, S // 2, 128), F32),
        vm((49, TQ // 2, 128), U32),
        vm((4, TQ // 2, 64), U32),
        vm((2, 49, MQ, TQ), F32),
        vm((49, TQ // 2, 128), U32),
        vm((4, TQ, 256), F32),
        vm((16, TQ, 256), F32),
        vm((16, TQ, 128), F32),
        vm((NC, 49, 64, 256), U32),
        vm((NC, 49, MQ // 2, 128), U32),
        vm((4, D, 128), F32),
        pltpu.SemaphoreType.DMA((11 + 3 * RING,)),
    ]
    hbm = pl.BlockSpec(memory_space=pl.ANY)
    out = pl.pallas_call(
        _kernel,
        in_specs=[pl.BlockSpec(memory_space=pltpu.SMEM)] + [hbm] * 6,
        out_specs=hbm,
        out_shape=jax.ShapeDtypeStruct((S, D), BF),
        scratch_shapes=scratch,
        compiler_params=pltpu.CompilerParams(vmem_limit_bytes=126 * 1024 * 1024),
    )(jnp.zeros((1,), jnp.int32), A_x.reshape(S, D), A_wqkv, A_wo, B_w_gate, B_w_up, B_w_down)
    return out.reshape(1, S, D)
```

```python
import math

import jax
import jax.numpy as jnp
from jax import lax
import jax.experimental.pallas as pl
import jax.experimental.pallas.tpu as pltpu

S, D, F = 2048, 576, 4608
H, DH, W = 32, 18, 8
NT_ = 8
TQ = 256
MQ = D // 4
FC = 512
NC = F // FC
RING = 3
EPS = 1e-5
SCALE = DH ** -0.5
EXP_C = SCALE * math.log2(math.e)
NEG = -1e9 / SCALE

BF, F32, U32 = jnp.bfloat16, jnp.float32, jnp.uint32
NT_DIMS = (((1,), (1,)), ((), ()))

LHS_SEL = {0: ((0, 0), 1, (1, 1)), 1: ((1, 0), 1, (1, 1)), 2: ((0, 0), 0, None), 3: ((1, 1), 0, None),
           4: ((0, 0), 1, (0, 1)), 5: ((1, 0), -1, (0, 0)), 6: ((0, 1), -1, (1, 1))}
RHS_SEL = {0: ((0, 0), 1, (1, 1)), 1: ((0, 0), 0, None), 2: ((0, 1), -1, (1, 1)), 3: ((1, 0), -1, (0, 0)),
           4: ((1, 1), 0, None), 5: ((0, 0), 1, (0, 1)), 6: ((1, 0), 1, (1, 1))}
G_ORDER = (0, 1, 2, 5, 3, 4, 6)


def _lhs1(a11, a12, a21, a22):
    return [a11 + a22, a21 + a22, a11, a22, a11 + a12, a21 - a11, a12 - a22]


def _rhs1(b11, b12, b21, b22):
    return [b11 + b22, b11, b12 - b22, b21 - b11, b22, b11 + b12, b21 + b22]


def _out1(m):
    return (m[0] + m[3] - m[4] + m[6], m[2] + m[4], m[1] + m[3], m[0] - m[1] + m[2] + m[5])


def _in2(fn, x):
    outer = [[fn(x[i][j], x[i][2 + j], x[2 + i][j], x[2 + i][2 + j]) for j in range(2)] for i in range(2)]
    return [v for a in range(7) for v in fn(outer[0][0][a], outer[0][1][a], outer[1][0][a], outer[1][1][a])]


def _out2(m):
    p = [_out1(m[7 * a:7 * a + 7]) for a in range(7)]
    c = [[None] * 4 for _ in range(4)]
    for q in range(4):
        i, j = q // 2, q % 2
        c[i][j], c[i][2 + j], c[2 + i][j], c[2 + i][2 + j] = _out1([p[a][q] for a in range(7)])
    return c


def _select(sel, load):
    first, sign, second = sel
    v = load(first)
    if sign == 1:
        v = [a + b for a, b in zip(v, load(second))]
    elif sign == -1:
        v = [a - b for a, b in zip(v, load(second))]
    return v


def _pk(lo, hi):
    return pltpu.pack_elementwise([lo, hi], packed_dtype=BF)


def _lo(w):
    return pltpu.unpack_elementwise(w, index=0, packed_dtype=BF, unpacked_dtype=F32)


def _hi(w):
    return pltpu.unpack_elementwise(w, index=1, packed_dtype=BF, unpacked_dtype=F32)


def _bf(w):
    return pltpu.bitcast(w, BF)


def _dot(a, b):
    return jnp.dot(a, b, preferred_element_type=F32)


def _layernorm_t(x):
    m = jnp.sum(x, axis=0, keepdims=True) * (1.0 / D)
    d = x - m
    v = jnp.sum(d * d, axis=0, keepdims=True) * (1.0 / D)
    return d * lax.rsqrt(v + EPS)


def _kernel(zero_ref, x_hbm, wqkv_hbm, wo_hbm, wg_hbm, wu_hbm, wd_hbm, out_hbm,
            xio, wqkv_raw, wo_raw, wg_raw, wu_raw, wd_raw, tg, tu,
            wts, wqkv_t, wo_t, xr, xm, xn, xnn, kb, vb, pb, ob, xf,
            a_ref, at_ref, acc, h_ref, ti, to, hf, r_ref, l_ref, sems):
    z = zero_ref[0]
    z2 = zero_ref[1]

    def fence(ref, v):
        ref[z + (ref.shape[0] - 1), 0:8, 0:128] = v

    def run(jobs, v, n=1):
        for _ in range(n):
            if jobs:
                jobs.pop(0)(v)

    def slab(b):
        return pl.ds(256 * b, 256 if b < 2 else 64)

    def cp_x(b):
        return pltpu.make_async_copy(x_hbm.at[slab(b), :], xio.at[slab(b), :], sems.at[b])

    def cp_out(b):
        return pltpu.make_async_copy(xio.at[slab(b), :], out_hbm.at[slab(b), :], sems.at[b])

    qkv_cols = {"k": pl.ds(512, 640), "v": pl.ds(1152, 576), "q": pl.ds(0, 512)}

    def cp_qkv(name):
        idx = 5 + "kvq".index(name)
        return pltpu.make_async_copy(wqkv_hbm.at[:, qkv_cols[name]], wqkv_raw.at[:, qkv_cols[name]], sems.at[idx])

    def cp_wo():
        return pltpu.make_async_copy(wo_hbm, wo_raw, sems.at[8])

    def cp_ffn(c):
        c0 = c * FC if isinstance(c, int) else pl.multiple_of(c * FC, FC)
        cols = pl.ds(c0, FC)
        slot = c % RING
        return (pltpu.make_async_copy(wg_hbm.at[0:512, cols], wg_raw.at[slot], sems.at[11 + 3 * slot]),
                pltpu.make_async_copy(wu_hbm.at[0:512, cols], wu_raw.at[slot], sems.at[12 + 3 * slot]),
                pltpu.make_async_copy(wd_hbm.at[:, cols], wd_raw.at[slot], sems.at[13 + 3 * slot]))

    def cp_tails():
        return (pltpu.make_async_copy(wg_hbm.at[512:D, :], tg, sems.at[9]),
                pltpu.make_async_copy(wu_hbm.at[512:D, :], tu, sems.at[10]))

    def transpose_cols(src, nb0, ncols):
        for nb in range(nb0, nb0 + 5):
            wn = min(128, ncols - 128 * nb)
            for kt in range(5):
                wk = 128 if kt < 4 else 64
                blk = src[128 * kt:128 * kt + wk, 128 * nb:128 * nb + wn].astype(F32)
                wts[kt, 128 * (nb - nb0):128 * (nb - nb0) + wn, 0:wk] = blk.T

    def setup_qkv(name):
        part = "qkv".index(name)
        nb0 = (D * part) // 128
        base = D * part - 128 * nb0
        transpose_cols(wqkv_raw, nb0, D * part + D)
        for hg in range(4):
            for kt in range(5):
                wk = 128 if kt < 4 else 64
                rows = [wts[kt, pl.ds(base + MQ * hg + d, 8, stride=DH), :][:, :wk] for d in range(DH)]
                w = jnp.concatenate(rows, axis=0).astype(BF)
                wqkv_t[part, 72 * hg:72 * hg + 72, 128 * kt:128 * kt + wk] = pltpu.bitcast(w, U32)

    def setup_wo():
        for nb in range(5):
            wn = 128 if nb < 4 else 64
            xf[nb, 0:D, 0:wn] = wo_raw[:, 128 * nb:128 * nb + wn].astype(F32)
        for nb in range(5):
            wn = 128 if nb < 4 else 64
            rows = []
            for hg in range(4):
                for d in range(0, DH, 2):
                    lo = xf[nb, pl.ds(MQ * hg + d, 8, stride=DH), :][:, :wn]
                    hi = xf[nb, pl.ds(MQ * hg + d + 1, 8, stride=DH), :][:, :wn]
                    rows.append(_pk(lo, hi))
            wo_raw[:, 128 * nb:128 * nb + wn] = _bf(jnp.concatenate(rows, axis=0))
        transpose_cols(wo_raw, 0, D)
        for kt in range(5):
            wk = 128 if kt < 4 else 64
            lo = wts[kt, pl.ds(0, D // 2, stride=2), :][:, :wk]
            hi = wts[kt, pl.ds(1, D // 2, stride=2), :][:, :wk]
            wo_t[:, 128 * kt:128 * kt + wk] = _pk(lo, hi)

    def x_to_rows(b):
        nw = 128 if b < 2 else 32
        for t in range(16):
            w = pltpu.bitcast(xio[256 * b:256 * b + 2 * nw, 128 * t:128 * t + 128], F32)
            xf[2 * b + t // 8, 128 * (t % 8):128 * (t % 8) + 128, 0:nw] = w.T

    def rows_to_tiles(b, s):
        nw = 128 if b < 2 else 32
        for r in range(NT_):
            w = jnp.concatenate([xf[2 * b + u, pl.ds(2 * r + s, 64, stride=16), :] for u in range(2)], axis=0)
            xr[8 * s + r, 256 * b:256 * b + 2 * nw, :] = _bf(w[:, :nw].T).astype(F32)

    def tiles_to_rows(b, s):
        nw = 128 if b < 2 else 32
        for r in range(NT_):
            w = _pk(xr[8 * s + r, pl.ds(256 * b, nw, stride=2), :],
                    xr[8 * s + r, pl.ds(256 * b + 1, nw, stride=2), :])
            w = pltpu.bitcast(w, F32).T
            if nw < 128:
                w = jnp.concatenate([w, jnp.zeros((128, 128 - nw), F32)], axis=1)
            for u in range(2):
                xf[2 * b + u, pl.ds(2 * r + s, 64, stride=16), :] = w[64 * u:64 * u + 64]

    def rows_to_out(b):
        nw = 128 if b < 2 else 32
        for t in range(16):
            w = xf[2 * b + t // 8, 128 * (t % 8):128 * (t % 8) + 128, 0:nw]
            xio[256 * b:256 * b + 2 * nw, 128 * t:128 * t + 128] = _bf(w.T)

    def prep_r(c, a):
        slot = c % RING
        for w_ref, off in ((wg_raw, 0), (wu_raw, 128)):
            for g in range(8):
                def load(quad):
                    ws = [pltpu.bitcast(w_ref[slot, pl.ds(128 * (2 * quad[0] + i) + 16 * g, 16),
                                              pl.ds(256 * quad[1], 256)], U32) for i in range(2)]
                    ws = [w[:, 128 * j:128 * j + 128] for w in ws for j in range(2)]
                    return [_lo(w) for w in ws] + [_hi(w) for w in ws]
                v = _select(RHS_SEL[a], load)
                for b, (lo, hi) in enumerate(zip(_rhs1(*v[:4]), _rhs1(*v[4:]))):
                    r_ref[c, 7 * a + b, 8 * g:8 * g + 8, off:off + 128] = _pk(lo, hi)

    def prep_l(c):
        slot = c % RING
        for g in range(MQ // 16):
            ws = [pltpu.bitcast(wd_raw[slot, pl.ds(MQ * i + 16 * g, 16), :], U32) for i in range(4)]
            ws = [[w[:, 128 * j:128 * j + 128] for j in range(4)] for w in ws]
            lo = _in2(_lhs1, [[_lo(w) for w in row] for row in ws])
            hi = _in2(_lhs1, [[_hi(w) for w in row] for row in ws])
            for k in range(49):
                l_ref[c, k, 8 * g:8 * g + 8, :] = _pk(lo[k], hi[k])

    def prep_a(a, half, g, zz):
        def load(quad):
            return [xf[zz + 2 * quad[1] + j, pl.ds(TQ * (2 * quad[0] + i) + 32 * g + half + e, 8, stride=4), :]
                    for e in (0, 2) for i in range(2) for j in range(2)]
        v = _select(LHS_SEL[a], load)
        for b, (lo, hi) in enumerate(zip(_lhs1(*v[:4]), _lhs1(*v[4:]))):
            a_ref[z + 7 * a + b, 64 * half + 8 * g:64 * half + 8 * g + 8, :] = _pk(lo, hi)

    def prep_a_tail():
        for i in range(4):
            for half in range(2):
                lo = xf[z + 4, pl.ds(TQ * i + half, 64, stride=4), :][:, :64]
                hi = xf[z + 4, pl.ds(TQ * i + half + 2, 64, stride=4), :][:, :64]
                at_ref[z + i, 64 * half:64 * half + 64, :] = _pk(lo, hi)

    def gate_up(c, before=None, late=None, per=1):
        c0 = c * FC if isinstance(c, int) else pl.multiple_of(c * FC, FC)
        jobs = []

        def inner(a, emit):
            if before is not None:
                before(a, jobs)

            def prod(b):
                m = _dot(_bf(a_ref[z + 7 * a + b]), _bf(r_ref[c, 7 * a + b]))
                for u in range(per):
                    row = (TQ // per) * u
                    run(jobs, m[row:row + 8, 0:128])
                return m
            ld = lambda s: ti[z + s]
            for s in range(3):
                ti[z + s] = prod(s)
            emit(3, ((ld(0) - ld(1)) + ld(2)) + prod(5))
            m3 = prod(3)
            emit(2, ld(1) + m3)
            ti[z + 3] = ld(0) + m3
            m4 = prod(4)
            emit(1, ld(2) + m4)
            ti[z + 3] = ld(3) - m4
            emit(0, ld(3) + prod(6))

        def fin(quad, q, v):
            i, j = 2 * (quad // 2) + q // 2, 2 * (quad % 2) + q % 2
            cols = pl.ds(c0 + 128 * j, 128)
            wt = jnp.concatenate([tg[:, cols], tu[:, cols]], axis=1)
            v = v + _dot(_bf(at_ref[z + i]), wt)
            hf[z + 4 * quad + q] = v[:, :128] * v[:, 128:]

        def old(s, q):
            return to[z + 4 * s + q]

        def keep(s):
            def emit(q, v):
                to[z + 4 * s + q] = v
            return emit

        def put(a):
            def job(fv, g):
                if fv is not None:
                    fence(hf, fv)

                def load(quad):
                    return [hf[z2 + 4 * (2 * quad[1] + quad[0]) + t, pl.ds(o + 8 * g, 8), :]
                            for o in (0, 128) for t in (0, 2, 1, 3)]
                v = _select(RHS_SEL[a], load)
                for b, (lo, hi) in enumerate(zip(_rhs1(*v[:4]), _rhs1(*v[4:]))):
                    h_ref[7 * a + b, 8 * g:8 * g + 8, :] = _pk(lo, hi)
            return [lambda fv, g=g: job(fv, g) for g in range(16)]

        def emit3(q, v):
            fin(2, q, old(1, q) + v)
            to[z + 12 + q] = old(0, q) + v

        def emit4(q, v):
            fin(1, q, old(2, q) + v)
            to[z + 12 + q] = old(3, q) - v

        inner(0, keep(0))
        inner(1, keep(1))
        inner(2, keep(2))
        inner(5, lambda q, v: fin(3, q, ((old(0, q) - old(1, q)) + old(2, q)) + v))
        jobs += put(4)
        inner(3, emit3)
        jobs += put(2)
        inner(4, emit4)
        jobs += put(6)
        inner(6, lambda q, v: fin(0, q, old(3, q) + v))
        assert not jobs
        late(put)

    def down(c, a, jobs=(), per=0):
        for k in range(7 * a, 7 * a + 7):
            prev = acc[k]
            if not isinstance(c, int):
                prev = jnp.where(c == 0, 0.0, prev)
            m = prev + lax.dot_general(_bf(l_ref[c, k]), _bf(h_ref[k]), NT_DIMS, preferred_element_type=F32)
            acc[k] = m
            for u in range(per):
                row = (MQ // per) // 8 * 8 * u
                run(jobs, m[row:row + 8, 0:128])

    def add_stats(st, r, x):
        st[r] = (x, x * x) if st.get(r) is None else (st[r][0] + x, st[r][1] + x * x)

    def mean_rstd(st, r):
        m = jnp.sum(st[r][0], axis=0, keepdims=True) * (1.0 / D)
        v = jnp.sum(st[r][1], axis=0, keepdims=True) * (1.0 / D) - m * m
        return m, lax.rsqrt(jnp.maximum(v, 0.0) + EPS)

    def finalize_jobs(base, st):
        jobs = []
        for e in range(2):
            for g in range(MQ // 8):
                part = {}

                def inner(v, a, e=e, g=g, part=part):
                    if v is not None:
                        fence(acc, v)
                    part[a] = _out1([acc[z2 + 7 * a + b, 8 * g:8 * g + 8, 128 * e:128 * e + 128]
                                     for b in range(7)])
                    if a == 6:
                        for q in range(4):
                            c = _out1([part[t][q] for t in range(7)])
                            for u in range(4):
                                i, j = 2 * (u // 2) + q // 2, 2 * (u % 2) + q % 2
                                rows = pl.ds(MQ * i + 8 * g, 8)
                                x = xm[z + 2 * j + e, rows, :] + c[u]
                                xr[base + 2 * j + e, rows, :] = x
                                if st is not None:
                                    add_stats(st, 2 * j + e, x)
                for a in range(7):
                    jobs.append(lambda v, a=a, inner=inner: inner(v, a))
            if st is not None:
                def close(v, e=e):
                    for j in range(4):
                        st[2 * j + e] = mean_rstd(st, 2 * j + e)
                jobs.append(close)
        return jobs

    def ln1_jobs(base, st):
        def job(v, r, k):
            fence(xr, v)
            m, rs = st[r]
            rows = pl.ds(64 * k, 64)
            xnn[rows, 128 * r:128 * r + 128] = ((xr[z2 + base + r, rows, :] - m) * rs).astype(BF)
        return [lambda v, r=r, k=k: job(v, r, k) for r in range(NT_) for k in range(D // 64)]

    def project_kv(name, src, tiles, hgs, jobs, every):
        dst = kb if name == "k" else vb
        nrow = MQ * len(hgs)
        rows = pl.ds(MQ * hgs[0], nrow)
        lhs = wqkv_t["qkv".index(name), 72 * hgs[0]:72 * hgs[-1] + 72, :]
        y = _dot(_bf(lhs), src[:, 128 * tiles[0]:128 * tiles[-1] + 128])
        for t, r in enumerate(tiles):
            tile = y[:, 128 * t:128 * t + 128]
            dst[z + 7 + r, rows, :] = tile
            if r >= 1:
                dst[z + r - 1, rows, :] = pltpu.roll(tile, 1, 1)
            for g in range(0, nrow // 8, every):
                run(jobs, tile[8 * g:8 * g + 8])

    def project_q(tiles, jobs):
        y = _dot(_bf(wqkv_t[0]), xn[:, 128 * tiles[0]:128 * tiles[-1] + 128])
        for t, r in enumerate(tiles):
            for hg in range(4):
                lg = [None] * W
                for d in range(DH):
                    row = MQ * hg + 8 * d
                    q = y[row:row + 8, 128 * t:128 * t + 128]
                    for w in range(W):
                        v = q * kb[z + 7 + r - w, row:row + 8, :]
                        lg[w] = v if d == 0 else lg[w] + v
                    if d == 9:
                        run(jobs, q)
                for w in range(W):
                    pb[z + r, 32 * w + 8 * hg:32 * w + 8 * hg + 8, :] = lg[w]
                if hg % 2 == 1:
                    jobs.append(softmax_job(r, hg // 2))

    def tree(fn, v):
        while len(v) > 1:
            v = [fn(v[i], v[i + 1]) for i in range(0, len(v), 2)]
        return v[0]

    def softmax_job(r, sl):
        def job(v):
            fence(pb, v)
            lane0 = lax.broadcasted_iota(jnp.int32, (16, 128), 1) == 0
            lg = [pb[z2 + r, 32 * w + 16 * sl:32 * w + 16 * sl + 16, :] for w in range(W)]
            lg = [jnp.where(lane0, NEG, lg[w]) if w > r else lg[w] for w in range(W)]
            m = tree(jnp.maximum, lg)
            ex = [jnp.exp2((lg[w] - m) * EXP_C) for w in range(W)]
            inv = 1.0 / tree(jnp.add, ex)
            for w in range(W):
                pb[z2 + r, 32 * w + 16 * sl:32 * w + 16 * sl + 16, :] = ex[w] * inv
        return job

    def mix_jobs(hg, tiles):
        jobs = []
        for r in tiles:
            p = []

            def job(v, d, r=r, p=p):
                if d == 0:
                    fence(pb, v)
                    p.extend(pb[z2 + r, 32 * w + 8 * hg:32 * w + 8 * hg + 8, :] for w in range(W))
                fence(vb, v)
                o = [tree(jnp.add, [p[w] * vb[z2 + 7 + r - w, pl.ds(MQ * hg + 8 * (d + e), 8), :]
                                    for w in range(W)]) for e in range(2)]
                ob[z + r, 72 * hg + 4 * d:72 * hg + 4 * d + 8, :] = _pk(o[0], o[1])
            for d in range(0, DH, 2):
                jobs.append(lambda v, d=d, job=job: job(v, d))
        return jobs

    def ln2_jobs(st, r):
        mr = {}

        def job(v, kt):
            if kt == 0:
                mr[0] = mean_rstd(st, r)
            m, rs = mr[0]
            wk = 128 if kt < 4 else 64
            y = (xm[z2 + r, 128 * kt:128 * kt + wk, :] - m) * rs
            xf[z + kt, 128 * r:128 * r + 128, 0:wk] = y.T
        return [lambda v, kt=kt: job(v, kt) for kt in range(5)]

    def prep_a_jobs(outer, gs):
        def job(v, a, half, g):
            fence(xf, v)
            prep_a(a, half, g, z2)
        return [lambda v, a=a, half=half, g=g: job(v, a, half, g)
                for a in outer for half in range(2) for g in gs]

    def out_proj(base, st, r, jobs, slow):
        y = _dot(_bf(wo_t[...]), _bf(ob[z + r]))
        for g in range(D // 16):
            rows = pl.ds(16 * g, 16)
            x = xr[base + r, rows, :] + y[16 * g:16 * g + 16]
            xm[z + r, rows, :] = x
            add_stats(st, r, x[0:8])
            add_stats(st, r, x[8:16])
            run(jobs, x[0:8])
            if g % 7 == 3:
                run(slow, None)

    def attention_block(p, first):
        s = 0 if first else p % 2
        cur, nxt = 8 * s, 8 * (1 - s)
        order = (0, 2, 4, 6, 1, 3, 5, 7)
        allh = (0, 1, 2, 3)
        st1 = {}
        if first:
            for r in range(NT_):
                xn[:, 128 * r:128 * r + 128] = _layernorm_t(xr[r]).astype(BF)
            project_kv("k", xn, (0, 1, 2, 3), allh, [], 1)
            project_kv("k", xn, (4, 5, 6, 7), allh, [], 1)
            cp_qkv("q").wait()
            setup_qkv("q")
            for b in range(3):
                rows_to_tiles(b, 1)
            for r in range(NT_):
                xnn[:, 128 * r:128 * r + 128] = _layernorm_t(xr[8 + r]).astype(BF)
            fin = []
        else:
            xn[...] = xnn[...]
            for a in range(7):
                down(NC - 1, a)
            fin = finalize_jobs(nxt, st1) + ln1_jobs(nxt, st1)
            project_kv("k", xn, (3, 4, 5, 6, 7), allh, fin, 2)
        jobs = []
        project_q((0, 1, 2, 3), jobs)
        project_q((4, 5, 6, 7), jobs)
        if first:
            cp_qkv("v").wait()
            setup_qkv("v")
            cp_wo().wait()
            setup_wo()
        jobs += fin[:2 + len(fin) - 9 * 7]
        fin = fin[2 + len(fin) - 9 * 7:]
        for hg in range(4):
            project_kv("v", xn, range(NT_), (hg,), jobs, 1 if hg == 0 else 2)
            assert not jobs
            jobs = mix_jobs(hg, order)
        project_kv("k", xnn, (0,), allh, jobs, 2)
        jobs += fin
        st2, slow = {}, []
        for t, r in enumerate(order):
            out_proj(cur, st2, r, jobs, slow)
            assert not slow
            slow = ln2_jobs(st2, r)
            if t == 5:
                jobs += prep_a_jobs(G_ORDER, range(4))
        assert not jobs
        run(slow, None, 5)
        if first:
            for cp in cp_ffn(0) + cp_tails():
                cp.wait()
        jobs = [lambda v: None] * 4 + prep_a_jobs(G_ORDER[:1], range(4, 8))
        project_kv("k", xnn, (1,), allh, jobs, 4)
        prep_a_tail()

        def before(a, jobs):
            t = G_ORDER.index(a)
            jobs += prep_a_jobs(G_ORDER[t + 1:t + 2], range(4, 8))
            if first:
                prep_r(0, a)
        if first:
            prep_l(0)

        def late(put):
            jobs = put(0) + put(3) + put(5) + put(1)
            project_kv("k", xnn, (2,), allh, jobs, 1)
            assert not jobs
        gate_up(0, before, late, 4)

    def ffn_loop(first):
        def body(c, carry):
            if first:
                for cp in cp_ffn(c + 1):
                    cp.wait()

                @pl.when(c + RING < NC)
                def _():
                    for cp in cp_ffn(c + RING):
                        cp.start()
            for a in (4, 2, 6):
                down(c, a)
            if first:
                prep_l(c + 1)

            def late(put):
                jobs = []
                for a in (0, 3, 5, 1):
                    down(c, a, jobs, 3)
                    jobs += put(a)
                run(jobs, None, 100)
            gate_up(c + 1, (lambda a, jobs: prep_r(c + 1, a)) if first else None, late, 4)
            return carry
        lax.fori_loop(0, NC - 1, body, 0)

    cp_qkv("k").start()
    for b in range(3):
        cp_x(b).start()
    cp_qkv("q").start()
    cp_qkv("v").start()
    cp_wo().start()
    for cp in cp_ffn(0) + cp_tails():
        cp.start()
    for c in range(1, RING):
        for cp in cp_ffn(c):
            cp.start()

    cp_qkv("k").wait()
    setup_qkv("k")
    for b in range(3):
        cp_x(b).wait()
        x_to_rows(b)
        rows_to_tiles(b, 0)

    attention_block(0, True)
    ffn_loop(True)

    def pass_body(p, carry):
        attention_block(p, False)
        ffn_loop(False)
        return carry
    lax.fori_loop(1, 4, pass_body, 0)

    for a in range(7):
        down(NC - 1, a)
    for b in range(3):
        tiles_to_rows(b, 0)
    run(finalize_jobs(8, None), None, 1000)
    for b in range(3):
        tiles_to_rows(b, 1)
        rows_to_out(b)
        cp_out(b).start()
    for b in range(3):
        cp_out(b).wait()


@jax.jit
def pallas_interleave_layers__sliding_local_dilated__glu_gated_bilinear__prompt_kernel(
    A_x: jax.Array,
    A_wqkv: jax.Array,
    A_wo: jax.Array,
    B_x: jax.Array,
    B_w_gate: jax.Array,
    B_w_up: jax.Array,
    B_w_down: jax.Array,
):
    del B_x
    vm = pltpu.VMEM
    scratch = [
        vm((D, S), BF), vm((D, 3 * D), BF), vm((D, D), BF),
        vm((RING, 512, FC), BF), vm((RING, 512, FC), BF), vm((RING, D, FC), BF),
        vm((D - 512, F), BF), vm((D - 512, F), BF),
        vm((5, 640, 128), F32),
        vm((3, D // 2, D), U32),
        vm((D // 2, D), U32),
        vm((2 * NT_ + 1, D, 128), F32),
        vm((NT_, D, 128), F32),
        vm((D, S // 2), BF),
        vm((D, S // 2), BF),
        vm((15, D, 128), F32),
        vm((16, D, 128), F32),
        vm((NT_ + 1, W * H, 128), F32),
        vm((NT_, D // 2, 128), U32),
        vm((7, S // 2, 128), F32),
        vm((49, TQ // 2, 128), U32),
        vm((4, TQ // 2, 64), U32),
        vm((50, MQ, TQ), F32),
        vm((49, TQ // 2, 128), U32),
        vm((4, TQ, 256), F32),
        vm((16, TQ, 256), F32),
        vm((17, TQ, 128), F32),
        vm((NC, 49, 64, 256), U32),
        vm((NC, 49, MQ // 2, 128), U32),
        pltpu.SemaphoreType.DMA((11 + 3 * RING,)),
    ]
    hbm = pl.BlockSpec(memory_space=pl.ANY)
    out = pl.pallas_call(
        _kernel,
        in_specs=[pl.BlockSpec(memory_space=pltpu.SMEM)] + [hbm] * 6,
        out_specs=hbm,
        out_shape=jax.ShapeDtypeStruct((D, S), BF),
        scratch_shapes=scratch,
        compiler_params=pltpu.CompilerParams(vmem_limit_bytes=126 * 1024 * 1024),
    )(jnp.zeros((2,), jnp.int32), A_x.reshape(S, D).T, A_wqkv, A_wo, B_w_gate, B_w_up, B_w_down.T)
    return out.T.reshape(1, S, D)
```

```python
import math

import jax
import jax.numpy as jnp
from jax import lax
import jax.experimental.pallas as pl
import jax.experimental.pallas.tpu as pltpu

S, D, F = 2048, 576, 4608
H, DH, W = 32, 18, 8
NT_ = 8
TQ = 256
MQ = D // 4
FC = 512
NC = F // FC
RING = 3
EPS = 1e-5
SCALE = DH ** -0.5
EXP_C = SCALE * math.log2(math.e)
NEG = -1e9 / SCALE

BF, F32, U32 = jnp.bfloat16, jnp.float32, jnp.uint32
NT_DIMS = (((1,), (1,)), ((), ()))

LHS_SEL = {0: ((0, 0), 1, (1, 1)), 1: ((1, 0), 1, (1, 1)), 2: ((0, 0), 0, None), 3: ((1, 1), 0, None),
           4: ((0, 0), 1, (0, 1)), 5: ((1, 0), -1, (0, 0)), 6: ((0, 1), -1, (1, 1))}
RHS_SEL = {0: ((0, 0), 1, (1, 1)), 1: ((0, 0), 0, None), 2: ((0, 1), -1, (1, 1)), 3: ((1, 0), -1, (0, 0)),
           4: ((1, 1), 0, None), 5: ((0, 0), 1, (0, 1)), 6: ((1, 0), 1, (1, 1))}
G_ORDER = (2, 0, 1, 5, 3, 4, 6)


def _lhs1(a11, a12, a21, a22):
    return [a11 + a22, a21 + a22, a11, a22, a11 + a12, a21 - a11, a12 - a22]


def _rhs1(b11, b12, b21, b22):
    return [b11 + b22, b11, b12 - b22, b21 - b11, b22, b11 + b12, b21 + b22]


def _out1(m):
    return (m[0] + m[3] - m[4] + m[6], m[2] + m[4], m[1] + m[3], m[0] - m[1] + m[2] + m[5])


def _in2(fn, x):
    outer = [[fn(x[i][j], x[i][2 + j], x[2 + i][j], x[2 + i][2 + j]) for j in range(2)] for i in range(2)]
    return [v for a in range(7) for v in fn(outer[0][0][a], outer[0][1][a], outer[1][0][a], outer[1][1][a])]


def _out2(m):
    p = [_out1(m[7 * a:7 * a + 7]) for a in range(7)]
    c = [[None] * 4 for _ in range(4)]
    for q in range(4):
        i, j = q // 2, q % 2
        c[i][j], c[i][2 + j], c[2 + i][j], c[2 + i][2 + j] = _out1([p[a][q] for a in range(7)])
    return c


def _select(sel, load):
    first, sign, second = sel
    v = load(first)
    if sign == 1:
        v = [a + b for a, b in zip(v, load(second))]
    elif sign == -1:
        v = [a - b for a, b in zip(v, load(second))]
    return v


def _pk(lo, hi):
    return pltpu.pack_elementwise([lo, hi], packed_dtype=BF)


def _lo(w):
    return pltpu.unpack_elementwise(w, index=0, packed_dtype=BF, unpacked_dtype=F32)


def _hi(w):
    return pltpu.unpack_elementwise(w, index=1, packed_dtype=BF, unpacked_dtype=F32)


def _bf(w):
    return pltpu.bitcast(w, BF)


def _dot(a, b):
    return jnp.dot(a, b, preferred_element_type=F32)


def _layernorm_t(x):
    m = jnp.sum(x, axis=0, keepdims=True) * (1.0 / D)
    d = x - m
    v = jnp.sum(d * d, axis=0, keepdims=True) * (1.0 / D)
    return d * lax.rsqrt(v + EPS)


def _kernel(zero_ref, x_hbm, wqkv_hbm, wo_hbm, wg_hbm, wu_hbm, wd_hbm, out_hbm,
            xio, wqkv_raw, wo_raw, wg_raw, wu_raw, wd_raw, tg, tu,
            wts, wqkv_t, wo_t, xr, xm, xn, xnn, kb, vb0, vb1, vb2, vb3, pb, ob, xf, xo,
            a_ref, at_ref, acc, h_ref, ti, to, hf, r_ref, l_ref, sems):
    z = zero_ref[0]
    z2 = zero_ref[1]
    vbs = (vb0, vb1, vb2, vb3)

    def fence(ref, v):
        ref[z + (ref.shape[0] - 1), 0:8, 0:128] = v

    def prime(ref, other):
        ref[z2 + (ref.shape[0] - 1), 0:8, 0:128] = pltpu.bitcast(other[z, 0:8, 0:128], F32)

    def run(jobs, v, n=1):
        for _ in range(n):
            if jobs:
                jobs.pop(0)(v)

    def tree(fn, v):
        while len(v) > 1:
            v = [fn(v[i], v[i + 1]) for i in range(0, len(v), 2)]
        return v[0]

    def slab(b):
        return pl.ds(256 * b, 256 if b < 2 else 64)

    def cp_x(b):
        return pltpu.make_async_copy(x_hbm.at[slab(b), :], xio.at[slab(b), :], sems.at[b])

    def cp_out(b):
        return pltpu.make_async_copy(xio.at[slab(b), :], out_hbm.at[slab(b), :], sems.at[b])

    qkv_cols = {"k": pl.ds(512, 640), "v": pl.ds(1152, 576), "q": pl.ds(0, 512)}

    def cp_qkv(name):
        idx = 5 + "kvq".index(name)
        return pltpu.make_async_copy(wqkv_hbm.at[:, qkv_cols[name]], wqkv_raw.at[:, qkv_cols[name]], sems.at[idx])

    def cp_wo():
        return pltpu.make_async_copy(wo_hbm, wo_raw, sems.at[8])

    def cp_ffn(c):
        c0 = c * FC if isinstance(c, int) else pl.multiple_of(c * FC, FC)
        cols = pl.ds(c0, FC)
        slot = c % RING
        return (pltpu.make_async_copy(wg_hbm.at[0:512, cols], wg_raw.at[slot], sems.at[11 + 3 * slot]),
                pltpu.make_async_copy(wu_hbm.at[0:512, cols], wu_raw.at[slot], sems.at[12 + 3 * slot]),
                pltpu.make_async_copy(wd_hbm.at[:, cols], wd_raw.at[slot], sems.at[13 + 3 * slot]))

    def cp_tails():
        return (pltpu.make_async_copy(wg_hbm.at[512:D, :], tg, sems.at[9]),
                pltpu.make_async_copy(wu_hbm.at[512:D, :], tu, sems.at[10]))

    def transpose_cols(src, nb0, ncols):
        for nb in range(nb0, nb0 + 5):
            wn = min(128, ncols - 128 * nb)
            for kt in range(5):
                wk = 128 if kt < 4 else 64
                blk = src[128 * kt:128 * kt + wk, 128 * nb:128 * nb + wn].astype(F32)
                wts[kt, 128 * (nb - nb0):128 * (nb - nb0) + wn, 0:wk] = blk.T

    def setup_qkv(name):
        part = "qkv".index(name)
        nb0 = (D * part) // 128
        base = D * part - 128 * nb0
        transpose_cols(wqkv_raw, nb0, D * part + D)
        for hg in range(4):
            for kt in range(5):
                wk = 128 if kt < 4 else 64
                rows = [wts[kt, pl.ds(base + MQ * hg + d, 8, stride=DH), :][:, :wk] for d in range(DH)]
                w = jnp.concatenate(rows, axis=0).astype(BF)
                wqkv_t[part, 72 * hg:72 * hg + 72, 128 * kt:128 * kt + wk] = pltpu.bitcast(w, U32)

    def setup_wo():
        for nb in range(5):
            wn = 128 if nb < 4 else 64
            xf[nb, 0:D, 0:wn] = wo_raw[:, 128 * nb:128 * nb + wn].astype(F32)
        for nb in range(5):
            wn = 128 if nb < 4 else 64
            rows = []
            for hg in range(4):
                for d in range(0, DH, 2):
                    lo = xf[nb, pl.ds(MQ * hg + d, 8, stride=DH), :][:, :wn]
                    hi = xf[nb, pl.ds(MQ * hg + d + 1, 8, stride=DH), :][:, :wn]
                    rows.append(_pk(lo, hi))
            wo_raw[:, 128 * nb:128 * nb + wn] = _bf(jnp.concatenate(rows, axis=0))
        transpose_cols(wo_raw, 0, D)
        for kt in range(5):
            wk = 128 if kt < 4 else 64
            lo = wts[kt, pl.ds(0, D // 2, stride=2), :][:, :wk]
            hi = wts[kt, pl.ds(1, D // 2, stride=2), :][:, :wk]
            wo_t[:, 128 * kt:128 * kt + wk] = _pk(lo, hi)

    def x_to_rows(b):
        nw = 128 if b < 2 else 32
        for t in range(16):
            w = pltpu.bitcast(xio[256 * b:256 * b + 2 * nw, 128 * t:128 * t + 128], F32)
            xf[2 * b + t // 8, 128 * (t % 8):128 * (t % 8) + 128, 0:nw] = w.T

    def rows_to_tiles(b, s):
        nw = 128 if b < 2 else 32
        for r in range(NT_):
            w = jnp.concatenate([xf[2 * b + u, pl.ds(2 * r + s, 64, stride=16), :] for u in range(2)], axis=0)
            xr[8 * s + r, 256 * b:256 * b + 2 * nw, :] = _bf(w[:, :nw].T).astype(F32)

    def tiles_to_rows(b, s):
        nw = 128 if b < 2 else 32
        for r in range(NT_):
            w = _pk(xr[8 * s + r, pl.ds(256 * b, nw, stride=2), :],
                    xr[8 * s + r, pl.ds(256 * b + 1, nw, stride=2), :])
            w = pltpu.bitcast(w, F32).T
            if nw < 128:
                w = jnp.concatenate([w, jnp.zeros((128, 128 - nw), F32)], axis=1)
            for u in range(2):
                xf[2 * b + u, pl.ds(2 * r + s, 64, stride=16), :] = w[64 * u:64 * u + 64]

    def rows_to_out(b):
        nw = 128 if b < 2 else 32
        for t in range(16):
            w = xf[2 * b + t // 8, 128 * (t % 8):128 * (t % 8) + 128, 0:nw]
            xio[256 * b:256 * b + 2 * nw, 128 * t:128 * t + 128] = _bf(w.T)

    def prep_r(c, a):
        slot = c % RING
        for w_ref, off in ((wg_raw, 0), (wu_raw, 128)):
            for g in range(8):
                def load(quad):
                    ws = [pltpu.bitcast(w_ref[slot, pl.ds(128 * (2 * quad[0] + i) + 16 * g, 16),
                                              pl.ds(256 * quad[1], 256)], U32) for i in range(2)]
                    ws = [w[:, 128 * j:128 * j + 128] for w in ws for j in range(2)]
                    return [_lo(w) for w in ws] + [_hi(w) for w in ws]
                v = _select(RHS_SEL[a], load)
                for b, (lo, hi) in enumerate(zip(_rhs1(*v[:4]), _rhs1(*v[4:]))):
                    r_ref[c, 7 * a + b, 8 * g:8 * g + 8, off:off + 128] = _pk(lo, hi)

    def prep_l(c):
        slot = c % RING
        for g in range(MQ // 16):
            ws = [pltpu.bitcast(wd_raw[slot, pl.ds(MQ * i + 16 * g, 16), :], U32) for i in range(4)]
            ws = [[w[:, 128 * j:128 * j + 128] for j in range(4)] for w in ws]
            lo = _in2(_lhs1, [[_lo(w) for w in row] for row in ws])
            hi = _in2(_lhs1, [[_hi(w) for w in row] for row in ws])
            for k in range(49):
                l_ref[c, k, 8 * g:8 * g + 8, :] = _pk(lo[k], hi[k])

    def prep_a(a, half, g):
        src, row = (xf, xo)[g // 4], 32 * (g % 4) + half

        def load(quad):
            return [src[z2 + 2 * quad[1] + j, pl.ds(128 * (2 * quad[0] + i) + row + e, 8, stride=4), :]
                    for e in (0, 2) for i in range(2) for j in range(2)]
        v = _select(LHS_SEL[a], load)
        o = [_pk(lo, hi) for lo, hi in zip(_lhs1(*v[:4]), _lhs1(*v[4:]))]
        for b in range(7):
            a_ref[z + 7 * a + b, 64 * half + 8 * g:64 * half + 8 * g + 8, :] = o[b]
        return o[5] ^ o[6]

    def prep_a_tail():
        for i in range(4):
            for half in range(2):
                for u, src in enumerate((xf, xo)):
                    lo = src[z + 4, pl.ds(128 * i + half, 32, stride=4), :][:, :64]
                    hi = src[z + 4, pl.ds(128 * i + half + 2, 32, stride=4), :][:, :64]
                    at_ref[z + i, pl.ds(64 * half + 32 * u, 32), :] = _pk(lo, hi)

    def put(a):
        for g in range(16):
            def load(quad):
                return [hf[z + 4 * (2 * quad[1] + quad[0]) + t, pl.ds(o + 8 * g, 8), :]
                        for o in (0, 128) for t in (0, 2, 1, 3)]
            v = _select(RHS_SEL[a], load)
            for b, (lo, hi) in enumerate(zip(_rhs1(*v[:4]), _rhs1(*v[4:]))):
                h_ref[7 * a + b, 8 * g:8 * g + 8, :] = _pk(lo, hi)

    def gate_up(c, before=None):
        c0 = c * FC if isinstance(c, int) else pl.multiple_of(c * FC, FC)

        def inner(a, emit):
            if before is not None:
                before(a)
            prod = lambda b: _dot(_bf(a_ref[z + 7 * a + b]), _bf(r_ref[c, 7 * a + b]))
            ld = lambda s: ti[z + s]
            for s in range(3):
                ti[z + s] = prod(s)
            emit(3, ((ld(0) - ld(1)) + ld(2)) + prod(5))
            m3 = prod(3)
            emit(2, ld(1) + m3)
            ti[z + 3] = ld(0) + m3
            m4 = prod(4)
            emit(1, ld(2) + m4)
            ti[z + 3] = ld(3) - m4
            emit(0, ld(3) + prod(6))

        def fin(quad, q, v):
            i, j = 2 * (quad // 2) + q // 2, 2 * (quad % 2) + q % 2
            cols = pl.ds(c0 + 128 * j, 128)
            wt = jnp.concatenate([tg[:, cols], tu[:, cols]], axis=1)
            v = v + _dot(_bf(at_ref[z + i]), wt)
            hf[z + 4 * quad + q] = v[:, :128] * v[:, 128:]

        def old(s, q):
            return to[z + 4 * s + q]

        def keep(s):
            def emit(q, v):
                to[z + 4 * s + q] = v
            return emit

        def emit3(q, v):
            fin(2, q, old(1, q) + v)
            to[z + 12 + q] = old(0, q) + v

        def emit4(q, v):
            fin(1, q, old(2, q) + v)
            to[z + 12 + q] = old(3, q) - v

        inner(2, keep(2))
        inner(0, keep(0))
        inner(1, keep(1))
        inner(5, lambda q, v: fin(3, q, ((old(0, q) - old(1, q)) + old(2, q)) + v))
        put(4)
        inner(3, emit3)
        put(2)
        inner(4, emit4)
        put(6)
        inner(6, lambda q, v: fin(0, q, old(3, q) + v))

    def down(c):
        for a, late in ((4, 1), (2, 0), (6, 3), (1, 5), (0, None), (3, None), (5, None)):
            for k in range(7 * a, 7 * a + 7):
                prev = acc[k]
                if not isinstance(c, int):
                    prev = jnp.where(c == 0, 0.0, prev)
                acc[k] = prev + lax.dot_general(_bf(l_ref[c, k]), _bf(h_ref[k]), NT_DIMS,
                                                preferred_element_type=F32)
            if late is not None:
                put(late)

    def add_stats(st, r, x):
        st[r] = (x, x * x) if st.get(r) is None else (st[r][0] + x, st[r][1] + x * x)

    def mean_rstd(st, r):
        m = jnp.sum(st[r][0], axis=0, keepdims=True) * (1.0 / D)
        v = jnp.sum(st[r][1], axis=0, keepdims=True) * (1.0 / D) - m * m
        return m, lax.rsqrt(jnp.maximum(v, 0.0) + EPS)

    def finalize_jobs(base, st):
        jobs = []
        for e in range(2):
            for g in range(MQ // 8):
                part = {}

                def inner(v, a, e=e, g=g, part=part):
                    if v is not None:
                        fence(acc, v)
                    part[a] = _out1([acc[z2 + 7 * a + b, 8 * g:8 * g + 8, 128 * e:128 * e + 128]
                                     for b in range(7)])
                    if a == 6:
                        for q in range(4):
                            c = _out1([part[t][q] for t in range(7)])
                            for u in range(4):
                                i, j = 2 * (u // 2) + q // 2, 2 * (u % 2) + q % 2
                                rows = pl.ds(MQ * i + 8 * g, 8)
                                x = xm[z + 2 * j + e, rows, :] + c[u]
                                xr[base + 2 * j + e, rows, :] = x
                                if st is not None:
                                    add_stats(st, 2 * j + e, x)
                for a in range(7):
                    jobs.append(lambda v, a=a, inner=inner: inner(v, a))
            if st is not None:
                def close(v, e=e):
                    for j in range(4):
                        st[2 * j + e] = mean_rstd(st, 2 * j + e)
                jobs.append(close)
        return jobs

    def chain(ref, last, v, skew=1):
        last.append(pltpu.bitcast(v, F32))
        if len(last) > skew:
            fence(ref, last.pop(0))

    def ln1_chain(base, st):
        last = []
        for r in range(NT_):
            m, rs = st[r]
            for k in range(3):
                rows = pl.ds(192 * k, 192)
                y = ((xr[z2 + base + r, rows, :] - m) * rs).astype(BF)
                xnn[rows, 128 * r:128 * r + 128] = y
                y = pltpu.bitcast(y, U32)
                chain(xr, last, tree(jnp.bitwise_xor, [y[8 * u:8 * u + 8] for u in (2, 5, 8, 11)]))

    def project_kv(name, src, tiles, hgs, jobs=(), every=1):
        dst = kb if name == "k" else vbs[hgs[0]]
        nrow = MQ * len(hgs)
        rows = pl.ds(MQ * hgs[0] if name == "k" else 0, nrow)
        lhs = wqkv_t["qkv".index(name), 72 * hgs[0]:72 * hgs[-1] + 72, :]
        y = _dot(_bf(lhs), src[:, 128 * tiles[0]:128 * tiles[-1] + 128])
        for t, r in enumerate(tiles):
            tile = y[:, 128 * t:128 * t + 128]
            dst[z + 7 + r, rows, :] = tile
            if r >= 1:
                dst[z + r - 1, rows, :] = pltpu.roll(tile, 1, 1)
            for g in range(0, nrow // 8, every):
                run(jobs, tile[8 * g:8 * g + 8])

    def project_q(tiles, jobs):
        y = _dot(_bf(wqkv_t[0]), xn[:, 128 * tiles[0]:128 * tiles[-1] + 128])
        for t, r in enumerate(tiles):
            for hg in range(4):
                lg = [None] * W
                for d in range(DH):
                    row = MQ * hg + 8 * d
                    q = y[row:row + 8, 128 * t:128 * t + 128]
                    for w in range(W):
                        v = q * kb[z + 7 + r - w, row:row + 8, :]
                        lg[w] = v if d == 0 else lg[w] + v
                    if d == 9:
                        run(jobs, q)
                for w in range(W):
                    pb[z + r, 32 * w + 8 * hg:32 * w + 8 * hg + 8, :] = lg[w]
                if hg % 2 == 1:
                    jobs.append(softmax_job(r, hg // 2))

    def softmax_job(r, sl):
        def job(v):
            fence(pb, v)
            lane0 = lax.broadcasted_iota(jnp.int32, (16, 128), 1) == 0
            lg = [pb[z2 + r, 32 * w + 16 * sl:32 * w + 16 * sl + 16, :] for w in range(W)]
            lg = [jnp.where(lane0, NEG, lg[w]) if w > r else lg[w] for w in range(W)]
            m = tree(jnp.maximum, lg)
            ex = [jnp.exp2((lg[w] - m) * EXP_C) for w in range(W)]
            inv = 1.0 / tree(jnp.add, ex)
            for w in range(W):
                pb[z2 + r, 32 * w + 16 * sl:32 * w + 16 * sl + 16, :] = ex[w] * inv
        return job

    def mix_jobs(hg, tiles):
        vb = vbs[hg]

        def job(v, r, d0):
            p = [pb[z2 + r, 32 * w + 8 * hg:32 * w + 8 * hg + 8, :] for w in range(W)]
            o = [tree(jnp.add, [p[w] * vb[z2 + 7 + r - w, pl.ds(8 * d, 8), :] for w in range(W)])
                 for d in range(d0, d0 + 6)]
            o = [_pk(o[e], o[e + 1]) for e in range(0, 6, 2)]
            ob[z + r, 72 * hg + 4 * d0:72 * hg + 4 * d0 + 24, :] = jnp.concatenate(o, axis=0)
            fence(vb, v)
        return [lambda v, r=r, d0=d0: job(v, r, d0) for r in tiles for d0 in range(0, DH, 6)]

    def ln2(st, r):
        m, rs = mean_rstd(st, r)
        last = []
        for kt in range(5):
            wk = 128 if kt < 4 else 64
            y = ((xm[z2 + r, 128 * kt:128 * kt + wk, :] - m) * rs).T
            (xf, xo)[r % 2][z + kt, pl.ds(128 * (r // 2), 128), 0:wk] = y
            if kt < 4:
                chain(xm, last, y[0:8])

    def prep_a_jobs(outer, odd):
        def job(v, a, half, g):
            prep_a(a, half, g)
            fence((xf, xo)[odd], v)
        return [lambda v, a=a, half=half, g=g: job(v, a, half, g)
                for a in outer for half in range(2) for g in range(4 * odd, 4 * odd + 4)]

    def out_proj(base, st, r, jobs):
        y = _dot(_bf(wo_t[...]), _bf(ob[z + r]))
        for g in range(D // 16):
            rows = pl.ds(16 * g, 16)
            x = xr[base + r, rows, :] + y[16 * g:16 * g + 16]
            xm[z + r, rows, :] = x
            add_stats(st, r, x[0:8])
            add_stats(st, r, x[8:16])
            run(jobs, x[0:8])

    def attention_block(p, first):
        s = 0 if first else p % 2
        cur, nxt = 8 * s, 8 * (1 - s)
        order = (0, 2, 4, 6, 1, 3, 5, 7)
        allh = (0, 1, 2, 3)
        st1 = {}
        if first:
            for r in range(NT_):
                xn[:, 128 * r:128 * r + 128] = _layernorm_t(xr[r]).astype(BF)
            project_kv("k", xn, (0, 1, 2, 3), allh, [], 1)
            project_kv("k", xn, (4, 5, 6, 7), allh, [], 1)
            cp_qkv("q").wait()
            setup_qkv("q")
            for b in range(3):
                rows_to_tiles(b, 1)
            for r in range(NT_):
                xnn[:, 128 * r:128 * r + 128] = _layernorm_t(xr[8 + r]).astype(BF)
            fin = []
        else:
            xn[...] = xnn[...]
            down(NC - 1)
            fin = finalize_jobs(nxt, st1)
            project_kv("k", xn, (3, 4, 5, 6, 7), allh, fin, 2)
        jobs = []
        project_q((0, 1, 2, 3), jobs)
        project_q((4, 5, 6, 7), jobs)
        if first:
            cp_qkv("v").wait()
            setup_qkv("v")
            cp_wo().wait()
            setup_wo()
        jobs += [lambda v: fence(pb, v)] + fin
        for vb in vbs:
            prime(vb, ob)
        prime(xf, a_ref)
        prime(xo, a_ref)
        for hg in range(4):
            for u in range(2):
                project_kv("v", xn, range(4 * u, 4 * u + 4), (hg,), jobs, 1 if hg == 0 else 6)
            assert not jobs
            jobs = mix_jobs(hg, order)
        if not first:
            ln1_chain(nxt, st1)
        for t in range(2):
            for hg in range(4):
                project_kv("k", xnn, (t,), (hg,), jobs, 6)
        assert not jobs
        st2 = {}
        for t, r in enumerate(order):
            if t > 0:
                ln2(st2, order[t - 1])
            jobs = {4: prep_a_jobs((2, 0, 1, 5), 0), 5: prep_a_jobs((3, 4, 6), 0),
                    6: prep_a_jobs((2, 4), 1)}.get(t, [])
            out_proj(cur, st2, r, jobs)
            assert not jobs
        ln2(st2, order[-1])
        if first:
            for cp in cp_ffn(0) + cp_tails():
                cp.wait()
        last = []
        project_kv("k", xnn, (2,), allh, [last.append])
        for a in (0, 1, 5, 3, 6):
            for half in range(2):
                for g in range(4, 8):
                    chain(xo, last, prep_a(a, half, g))
        prep_a_tail()
        before = (lambda a: prep_r(0, a)) if first else None
        if first:
            prep_l(0)
        gate_up(0, before)

    def ffn_loop(first):
        def body(c, carry):
            if first:
                for cp in cp_ffn(c + 1):
                    cp.wait()

                @pl.when(c + RING < NC)
                def _():
                    for cp in cp_ffn(c + RING):
                        cp.start()
            down(c)
            if first:
                prep_l(c + 1)

            gate_up(c + 1, (lambda a: prep_r(c + 1, a)) if first else None)
            return carry
        lax.fori_loop(0, NC - 1, body, 0)

    cp_qkv("k").start()
    for b in range(3):
        cp_x(b).start()
    cp_qkv("q").start()
    cp_qkv("v").start()
    cp_wo().start()
    for cp in cp_ffn(0) + cp_tails():
        cp.start()
    for c in range(1, RING):
        for cp in cp_ffn(c):
            cp.start()

    cp_qkv("k").wait()
    setup_qkv("k")
    for b in range(3):
        cp_x(b).wait()
        x_to_rows(b)
        rows_to_tiles(b, 0)

    attention_block(0, True)
    ffn_loop(True)

    def pass_body(p, carry):
        attention_block(p, False)
        ffn_loop(False)
        return carry
    lax.fori_loop(1, 4, pass_body, 0)

    down(NC - 1)
    for b in range(3):
        tiles_to_rows(b, 0)
    run(finalize_jobs(8, None), None, 1000)
    for b in range(3):
        tiles_to_rows(b, 1)
        rows_to_out(b)
        cp_out(b).start()
    for b in range(3):
        cp_out(b).wait()


@jax.jit
def pallas_interleave_layers__sliding_local_dilated__glu_gated_bilinear__prompt_kernel(
    A_x: jax.Array,
    A_wqkv: jax.Array,
    A_wo: jax.Array,
    B_x: jax.Array,
    B_w_gate: jax.Array,
    B_w_up: jax.Array,
    B_w_down: jax.Array,
):
    del B_x
    vm = pltpu.VMEM
    scratch = [
        vm((D, S), BF), vm((D, 3 * D), BF), vm((D, D), BF),
        vm((RING, 512, FC), BF), vm((RING, 512, FC), BF), vm((RING, D, FC), BF),
        vm((D - 512, F), BF), vm((D - 512, F), BF),
        vm((5, 640, 128), F32),
        vm((3, D // 2, D), U32),
        vm((D // 2, D), U32),
        vm((2 * NT_ + 1, D, 128), F32),
        vm((NT_ + 1, D, 128), F32),
        vm((D, S // 2), BF),
        vm((D, S // 2), BF),
        vm((15, D, 128), F32),
        vm((16, MQ, 128), F32), vm((16, MQ, 128), F32), vm((16, MQ, 128), F32), vm((16, MQ, 128), F32),
        vm((NT_ + 1, W * H, 128), F32),
        vm((NT_, D // 2, 128), U32),
        vm((7, S // 2, 128), F32),
        vm((6, S // 4, 128), F32),
        vm((49, TQ // 2, 128), U32),
        vm((4, TQ // 2, 64), U32),
        vm((50, MQ, TQ), F32),
        vm((49, TQ // 2, 128), U32),
        vm((4, TQ, 256), F32),
        vm((16, TQ, 256), F32),
        vm((16, TQ, 128), F32),
        vm((NC, 49, 64, 256), U32),
        vm((NC, 49, MQ // 2, 128), U32),
        pltpu.SemaphoreType.DMA((11 + 3 * RING,)),
    ]
    hbm = pl.BlockSpec(memory_space=pl.ANY)
    out = pl.pallas_call(
        _kernel,
        in_specs=[pl.BlockSpec(memory_space=pltpu.SMEM)] + [hbm] * 6,
        out_specs=hbm,
        out_shape=jax.ShapeDtypeStruct((D, S), BF),
        scratch_shapes=scratch,
        compiler_params=pltpu.CompilerParams(vmem_limit_bytes=126 * 1024 * 1024),
    )(jnp.zeros((2,), jnp.int32), A_x.reshape(S, D).T, A_wqkv, A_wo, B_w_gate, B_w_up, B_w_down.T)
    return out.T.reshape(1, S, D)
```

```python
import math

import jax
import jax.numpy as jnp
from jax import lax
import jax.experimental.pallas as pl
import jax.experimental.pallas.tpu as pltpu

S, D, F = 2048, 576, 4608
H, DH, W = 32, 18, 8
NT_ = 8
TQ = 256
MQ = D // 4
FC = 512
NC = F // FC
RING = 3
X_SPLIT = (0, 5, 10, 14, 16)
EPS = 1e-5
SCALE = DH ** -0.5
EXP_C = SCALE * math.log2(math.e)
NEG = -1e9 / SCALE

BF, F32, U32 = jnp.bfloat16, jnp.float32, jnp.uint32
NT_DIMS = (((1,), (1,)), ((), ()))

LHS_SEL = {0: ((0, 0), 1, (1, 1)), 1: ((1, 0), 1, (1, 1)), 2: ((0, 0), 0, None), 3: ((1, 1), 0, None),
           4: ((0, 0), 1, (0, 1)), 5: ((1, 0), -1, (0, 0)), 6: ((0, 1), -1, (1, 1))}
RHS_SEL = {0: ((0, 0), 1, (1, 1)), 1: ((0, 0), 0, None), 2: ((0, 1), -1, (1, 1)), 3: ((1, 0), -1, (0, 0)),
           4: ((1, 1), 0, None), 5: ((0, 0), 1, (0, 1)), 6: ((1, 0), 1, (1, 1))}
G_ORDER = (2, 0, 1, 5, 3, 4, 6)


def _lhs1(a11, a12, a21, a22):
    return [a11 + a22, a21 + a22, a11, a22, a11 + a12, a21 - a11, a12 - a22]


def _rhs1(b11, b12, b21, b22):
    return [b11 + b22, b11, b12 - b22, b21 - b11, b22, b11 + b12, b21 + b22]


def _in2(fn, x):
    outer = [[fn(x[i][j], x[i][2 + j], x[2 + i][j], x[2 + i][2 + j]) for j in range(2)] for i in range(2)]
    return [v for a in range(7) for v in fn(outer[0][0][a], outer[0][1][a], outer[1][0][a], outer[1][1][a])]


def _select(sel, load):
    first, sign, second = sel
    v = load(first)
    if sign == 1:
        v = [a + b for a, b in zip(v, load(second))]
    elif sign == -1:
        v = [a - b for a, b in zip(v, load(second))]
    return v


def _pk(lo, hi):
    return pltpu.pack_elementwise([lo, hi], packed_dtype=BF)


def _lo(w):
    return pltpu.unpack_elementwise(w, index=0, packed_dtype=BF, unpacked_dtype=F32)


def _hi(w):
    return pltpu.unpack_elementwise(w, index=1, packed_dtype=BF, unpacked_dtype=F32)


def _bf(w):
    return pltpu.bitcast(w, BF)


def _dot(a, b):
    return jnp.dot(a, b, preferred_element_type=F32)


def _kernel(x_hbm, wqkv_hbm, wo_hbm, wg_hbm, wu_hbm, wd_hbm, out_hbm,
            xio, wqkv_raw, wo_raw, wg_raw, wu_raw, wd_raw, tg, tu,
            wts, wqkv_t, wo_t, xr, xm, xn, xnn, kb, vb0, vb1, vb2, vb3, pb, ob, xf, xo, perm,
            a_ref, at_ref, acc, h_ref, ti, to, hf, r_ref, l_ref, zero_ref, sems):
    def clear(i, carry):
        zero_ref[i] = 0
        return carry
    lax.fori_loop(0, 2, clear, 0)
    z = zero_ref[0]
    z2 = zero_ref[1]
    vbs = (vb0, vb1, vb2, vb3)

    def fence(ref, v):
        ref[z + (ref.shape[0] - 1), 0:8, 0:128] = v

    def prime(ref, other):
        ref[z2 + (ref.shape[0] - 1), 0:8, 0:128] = pltpu.bitcast(other[z, 0:8, 0:128], F32)

    def run(jobs, v, n=1):
        for _ in range(n):
            if jobs:
                jobs.pop(0)(v)

    def tree(fn, v):
        while len(v) > 1:
            v = [fn(v[i], v[i + 1]) for i in range(0, len(v), 2)]
        return v[0]

    def slab(b):
        return pl.ds(256 * b, 256 if b < 2 else 64)

    def cp_x(u):
        cols = pl.ds(128 * X_SPLIT[u], 128 * (X_SPLIT[u + 1] - X_SPLIT[u]))
        return pltpu.make_async_copy(x_hbm.at[:, cols], xio.at[:, cols], sems.at[u])

    def cp_out(b):
        return pltpu.make_async_copy(xio.at[slab(b), :], out_hbm.at[slab(b), :], sems.at[b])

    qkv_cols = {"k": pl.ds(512, 640), "v": pl.ds(1152, 576), "q": pl.ds(0, 512)}

    def cp_qkv(name):
        idx = 5 + "kvq".index(name)
        return pltpu.make_async_copy(wqkv_hbm.at[:, qkv_cols[name]], wqkv_raw.at[:, qkv_cols[name]], sems.at[idx])

    def cp_wo():
        return pltpu.make_async_copy(wo_hbm, wo_raw, sems.at[8])

    def cp_ffn(c):
        c0 = c * FC if isinstance(c, int) else pl.multiple_of(c * FC, FC)
        cols = pl.ds(c0, FC)
        slot = c % RING
        return (pltpu.make_async_copy(wg_hbm.at[0:512, cols], wg_raw.at[slot], sems.at[11 + 3 * slot]),
                pltpu.make_async_copy(wu_hbm.at[0:512, cols], wu_raw.at[slot], sems.at[12 + 3 * slot]),
                pltpu.make_async_copy(wd_hbm.at[:, cols], wd_raw.at[slot], sems.at[13 + 3 * slot]))

    def cp_tails():
        return (pltpu.make_async_copy(wg_hbm.at[512:D, :], tg, sems.at[9]),
                pltpu.make_async_copy(wu_hbm.at[512:D, :], tu, sems.at[10]))

    def transpose_cols(src, nb0, ncols):
        for nb in range(nb0, nb0 + 5):
            wn = min(128, ncols - 128 * nb)
            for kt in range(5):
                wk = 128 if kt < 4 else 64
                blk = src[128 * kt:128 * kt + wk, 128 * nb:128 * nb + wn].astype(F32)
                wts[kt, 128 * (nb - nb0):128 * (nb - nb0) + wn, 0:wk] = blk.T

    def setup_qkv(name):
        part = "qkv".index(name)
        nb0 = (D * part) // 128
        base = D * part - 128 * nb0
        transpose_cols(wqkv_raw, nb0, D * part + D)
        for hg in range(4):
            for kt in range(5):
                wk = 128 if kt < 4 else 64
                rows = [wts[kt, pl.ds(base + MQ * hg + d, 8, stride=DH), :][:, :wk] for d in range(DH)]
                w = jnp.concatenate(rows, axis=0).astype(BF)
                wqkv_t[part, 72 * hg:72 * hg + 72, 128 * kt:128 * kt + wk] = pltpu.bitcast(w, U32)

    def setup_wo():
        for nb in range(5):
            wn = 128 if nb < 4 else 64
            xf[nb, 0:D, 0:wn] = wo_raw[:, 128 * nb:128 * nb + wn].astype(F32)
        for nb in range(5):
            wn = 128 if nb < 4 else 64
            rows = []
            for hg in range(4):
                for d in range(0, DH, 2):
                    lo = xf[nb, pl.ds(MQ * hg + d, 8, stride=DH), :][:, :wn]
                    hi = xf[nb, pl.ds(MQ * hg + d + 1, 8, stride=DH), :][:, :wn]
                    rows.append(_pk(lo, hi))
            for kt in range(5):
                blk = _bf(jnp.concatenate(rows[8 * kt:8 * kt + 8], axis=0)).astype(F32).T
                wo_t[64 * nb:64 * nb + wn // 2, pl.ds(128 * kt, blk.shape[1])] = pltpu.bitcast(blk.astype(BF), U32)

    def pad_lanes(w):
        if w.shape[1] == 128:
            return w
        return jnp.concatenate([w, jnp.zeros((128, 128 - w.shape[1]), F32)], axis=1)

    def x_to_rows(t):
        for b in range(3):
            nw = 128 if b < 2 else 32
            w = pltpu.bitcast(xio[256 * b:256 * b + 2 * nw, 128 * t:128 * t + 128], F32)
            w = pad_lanes(w.T)
            for jj in range(8):
                perm[pl.ds(49 * (8 * t + jj) + b, 16, stride=3), :] = w[16 * jj:16 * jj + 16]

    def rows_to_tile(s, r, st):
        for b in range(3):
            nw = 128 if b < 2 else 32
            w = perm[pl.ds(3 * (2 * r + s) + b, 128, stride=49), :]
            x = _bf(w[:, :nw].T).astype(F32)
            xr[8 * s + r, 256 * b:256 * b + 2 * nw, :] = x
            for g in range(nw // 4):
                add_stats(st, r, x[8 * g:8 * g + 8])

    def tiles_to_rows(b, s, tiles):
        nw = 128 if b < 2 else 32
        for r in tiles:
            w = _pk(xr[8 * s + r, pl.ds(256 * b, nw, stride=2), :],
                    xr[8 * s + r, pl.ds(256 * b + 1, nw, stride=2), :])
            perm[pl.ds(3 * (2 * r + s) + b, 128, stride=49), :] = pad_lanes(pltpu.bitcast(w, F32).T)

    def rows_to_out(b):
        nw = 128 if b < 2 else 32
        for t in range(16):
            w = jnp.concatenate([perm[pl.ds(49 * (8 * t + jj) + b, 16, stride=3), :] for jj in range(8)], axis=0)
            xio[256 * b:256 * b + 2 * nw, 128 * t:128 * t + 128] = _bf(w[:, :nw].T)

    def prep_r(c, a):
        slot = c % RING
        for w_ref, off in ((wg_raw, 0), (wu_raw, 128)):
            for g in range(8):
                def load(quad):
                    ws = [pltpu.bitcast(w_ref[slot, pl.ds(128 * (2 * quad[0] + i) + 16 * g, 16),
                                              pl.ds(256 * quad[1], 256)], U32) for i in range(2)]
                    ws = [w[:, 128 * j:128 * j + 128] for w in ws for j in range(2)]
                    return [_lo(w) for w in ws] + [_hi(w) for w in ws]
                v = _select(RHS_SEL[a], load)
                for b, (lo, hi) in enumerate(zip(_rhs1(*v[:4]), _rhs1(*v[4:]))):
                    r_ref[c, 7 * a + b, 8 * g:8 * g + 8, off:off + 128] = _pk(lo, hi)

    def prep_l(c):
        slot = c % RING
        for g in range(MQ // 16):
            ws = [pltpu.bitcast(wd_raw[slot, pl.ds(MQ * i + 16 * g, 16), :], U32) for i in range(4)]
            ws = [[w[:, 128 * j:128 * j + 128] for j in range(4)] for w in ws]
            lo = _in2(_lhs1, [[_lo(w) for w in row] for row in ws])
            hi = _in2(_lhs1, [[_hi(w) for w in row] for row in ws])
            for k in range(49):
                l_ref[c, k, 8 * g:8 * g + 8, :] = _pk(lo[k], hi[k])

    def prep_a(a, half, g):
        src, row = (xf, xo)[g // 4], 32 * (g % 4) + half

        def load(quad):
            return [src[z2 + 2 * quad[1] + j, pl.ds(128 * (2 * quad[0] + i) + row + e, 8, stride=4), :]
                    for e in (0, 2) for i in range(2) for j in range(2)]
        v = _select(LHS_SEL[a], load)
        o = [_pk(lo, hi) for lo, hi in zip(_lhs1(*v[:4]), _lhs1(*v[4:]))]
        for b in range(7):
            a_ref[z + 7 * a + b, 64 * half + 8 * g:64 * half + 8 * g + 8, :] = o[b]
        return o[5] ^ o[6]

    def prep_a_tail():
        for i in range(4):
            for half in range(2):
                for u, src in enumerate((xf, xo)):
                    lo = src[z + 4, pl.ds(128 * i + half, 32, stride=4), :][:, :64]
                    hi = src[z + 4, pl.ds(128 * i + half + 2, 32, stride=4), :][:, :64]
                    at_ref[z + i, pl.ds(64 * half + 32 * u, 32), :] = _pk(lo, hi)

    def put(a):
        for g in range(16):
            def load(quad):
                return [hf[z + 4 * (2 * quad[1] + quad[0]) + t, pl.ds(o + 8 * g, 8), :]
                        for o in (0, 128) for t in (0, 2, 1, 3)]
            v = _select(RHS_SEL[a], load)
            for b, (lo, hi) in enumerate(zip(_rhs1(*v[:4]), _rhs1(*v[4:]))):
                h_ref[7 * a + b, 8 * g:8 * g + 8, :] = _pk(lo, hi)

    def strassen_inner(prod, nrow, emit):
        ld = lambda s: ti[z + s, 0:nrow, :]
        for s in range(3):
            ti[z + s, 0:nrow, :] = prod(s)
        emit(3, ((ld(0) - ld(1)) + ld(2)) + prod(5))
        m3 = prod(3)
        emit(2, ld(1) + m3)
        ti[z + 3, 0:nrow, :] = ld(0) + m3
        m4 = prod(4)
        emit(1, ld(2) + m4)
        ti[z + 3, 0:nrow, :] = ld(3) - m4
        emit(0, ld(3) + prod(6))

    def gate_up(c, before=None):
        c0 = c * FC if isinstance(c, int) else pl.multiple_of(c * FC, FC)

        def inner(a, emit):
            if before is not None:
                before(a)
            strassen_inner(lambda b: _dot(_bf(a_ref[z + 7 * a + b]), _bf(r_ref[c, 7 * a + b])), TQ, emit)

        def fin(quad, q, v):
            i, j = 2 * (quad // 2) + q // 2, 2 * (quad % 2) + q % 2
            cols = pl.ds(c0 + 128 * j, 128)
            wt = jnp.concatenate([tg[:, cols], tu[:, cols]], axis=1)
            v = v + _dot(_bf(at_ref[z + i]), wt)
            hf[z + 4 * quad + q] = v[:, :128] * v[:, 128:]

        def old(s, q):
            return to[z + 4 * s + q]

        def keep(s):
            def emit(q, v):
                to[z + 4 * s + q] = v
            return emit

        def emit3(q, v):
            fin(2, q, old(1, q) + v)
            to[z + 12 + q] = old(0, q) + v

        def emit4(q, v):
            fin(1, q, old(2, q) + v)
            to[z + 12 + q] = old(3, q) - v

        inner(2, keep(2))
        inner(0, keep(0))
        inner(1, keep(1))
        inner(5, lambda q, v: fin(3, q, ((old(0, q) - old(1, q)) + old(2, q)) + v))
        put(4)
        inner(3, emit3)
        put(2)
        inner(4, emit4)
        put(6)
        inner(6, lambda q, v: fin(0, q, old(3, q) + v))

    def down_prod(c, k, prev):
        return prev + lax.dot_general(_bf(l_ref[c, k]), _bf(h_ref[k]), NT_DIMS, preferred_element_type=F32)

    def down(c):
        for a, late in ((4, 1), (2, 0), (6, 3), (1, 5), (0, None), (3, None), (5, None)):
            for k in range(7 * a, 7 * a + 7):
                acc[k] = down_prod(c, k, jnp.where(c == 0, 0.0, acc[k]))
            if late is not None:
                put(late)

    def add_stats(st, r, x):
        st[r] = (x, x * x) if st.get(r) is None else (st[r][0] + x, st[r][1] + x * x)

    def mean_rstd(st, r):
        m = jnp.sum(st[r][0], axis=0, keepdims=True) * (1.0 / D)
        v = jnp.sum(st[r][1], axis=0, keepdims=True) * (1.0 / D) - m * m
        return m, lax.rsqrt(jnp.maximum(v, 0.0) + EPS)

    def down_final(base, st, after=None, between=None):
        def inner(a, emit, late=None):
            strassen_inner(lambda b: down_prod(NC - 1, 7 * a + b, acc[7 * a + b]), MQ, emit)
            if late is not None:
                put(late)
            if between is not None:
                between(a)

        def old(s, q):
            return to[z + 4 * s + q, 0:MQ, :]

        def keep(s, q, v):
            to[z + 4 * s + q, 0:MQ, :] = v

        def fin(quad, q, v):
            i, j = 2 * (quad // 2) + q // 2, 2 * (quad % 2) + q % 2
            rows = pl.ds(MQ * i, MQ)
            for e in range(2):
                x = xm[z + 2 * j + e, rows, :] + v[:, 128 * e:128 * e + 128]
                xr[base + 2 * j + e, rows, :] = x
                if st is not None:
                    for g in range(MQ // 8):
                        add_stats(st, 2 * j + e, x[8 * g:8 * g + 8])
            if after is not None and q == 0:
                after(quad)

        inner(4, lambda q, v: keep(0, q, v), 0)
        inner(2, lambda q, v: (fin(1, q, old(0, q) + v), keep(1, q, v)), 3)
        inner(6, lambda q, v: keep(0, q, v - old(0, q)), 1)
        inner(0, lambda q, v: (keep(0, q, old(0, q) + v), keep(1, q, old(1, q) + v)), 5)
        inner(3, lambda q, v: (fin(0, q, old(0, q) + v), keep(2, q, v)))
        inner(1, lambda q, v: (fin(2, q, old(2, q) + v), keep(1, q, old(1, q) - v)))
        inner(5, lambda q, v: fin(3, q, old(1, q) + v))

    def chain(ref, last, v, skew=1):
        last.append(pltpu.bitcast(v, F32))
        if len(last) > skew:
            fence(ref, last.pop(0))

    def ln1_jobs(base, st):
        mr = [mean_rstd(st, r) for r in range(NT_)]

        def job(v, r, k):
            fence(xr, v)
            y = (xr[z2 + base + r, pl.ds(64 * k, 64), :] - mr[r][0]) * mr[r][1]
            xnn[32 * k:32 * k + 32, 128 * r:128 * r + 128] = pltpu.bitcast(y.astype(BF), U32)
        return [lambda v, r=r, k=k: job(v, r, k) for r in range(NT_) for k in range(D // 64)]

    def project_kv(name, src, tiles, hgs, jobs=(), every=1):
        dst = kb if name == "k" else vbs[hgs[0]]
        nrow = MQ * len(hgs)
        rows = pl.ds(MQ * hgs[0] if name == "k" else 0, nrow)
        lhs = wqkv_t["qkv".index(name), 72 * hgs[0]:72 * hgs[-1] + 72, :]
        y = _dot(_bf(lhs), _bf(src[:, 128 * tiles[0]:128 * tiles[-1] + 128]))
        for t, r in enumerate(tiles):
            tile = y[:, 128 * t:128 * t + 128]
            dst[z + 7 + r, rows, :] = tile
            if r >= 1:
                dst[z + r - 1, rows, :] = pltpu.roll(tile, 1, 1)
            for g in range(0, nrow // 8, every):
                run(jobs, tile[8 * g:8 * g + 8])

    def project_q(tiles, jobs):
        y = _dot(_bf(wqkv_t[0]), _bf(xn[:, 128 * tiles[0]:128 * tiles[-1] + 128]))
        for t, r in enumerate(tiles):
            for hg in range(4):
                lg = [None] * W
                for d in range(DH):
                    row = MQ * hg + 8 * d
                    q = y[row:row + 8, 128 * t:128 * t + 128]
                    for w in range(W):
                        v = q * kb[z + 7 + r - w, row:row + 8, :]
                        lg[w] = v if d == 0 else lg[w] + v
                    if d == 9:
                        run(jobs, q)
                for w in range(W):
                    pb[z + r, 32 * w + 8 * hg:32 * w + 8 * hg + 8, :] = lg[w]
                if hg % 2 == 1:
                    jobs.append(softmax_job(r, hg // 2))

    def softmax_job(r, sl):
        def job(v):
            fence(pb, v)
            lane0 = lax.broadcasted_iota(jnp.int32, (16, 128), 1) == 0
            lg = [pb[z2 + r, 32 * w + 16 * sl:32 * w + 16 * sl + 16, :] for w in range(W)]
            lg = [jnp.where(lane0, NEG, lg[w]) if w > r else lg[w] for w in range(W)]
            m = tree(jnp.maximum, lg)
            ex = [jnp.exp2((lg[w] - m) * EXP_C) for w in range(W)]
            inv = 1.0 / tree(jnp.add, ex)
            for w in range(W):
                pb[z2 + r, 32 * w + 16 * sl:32 * w + 16 * sl + 16, :] = ex[w] * inv
        return job

    def mix_jobs(hg, tiles):
        vb = vbs[hg]

        def job(v, r, d0):
            p = [pb[z2 + r, 32 * w + 8 * hg:32 * w + 8 * hg + 8, :] for w in range(W)]
            o = [tree(jnp.add, [p[w] * vb[z2 + 7 + r - w, pl.ds(8 * d, 8), :] for w in range(W)])
                 for d in range(d0, d0 + 6)]
            o = [_pk(o[e], o[e + 1]) for e in range(0, 6, 2)]
            ob[z + r, 72 * hg + 4 * d0:72 * hg + 4 * d0 + 24, :] = jnp.concatenate(o, axis=0)
            fence(vb, v)
        return [lambda v, r=r, d0=d0: job(v, r, d0) for r in tiles for d0 in range(0, DH, 6)]

    def ln2(st, r):
        m, rs = mean_rstd(st, r)
        last = []
        for kt in range(5):
            wk = 128 if kt < 4 else 64
            y = ((xm[z2 + r, 128 * kt:128 * kt + wk, :] - m) * rs).T
            (xf, xo)[r % 2][z + kt, pl.ds(128 * (r // 2), 128), 0:wk] = y
            if kt < 4:
                chain(xm, last, y[0:8])

    def prep_a_jobs(outer, odd):
        def job(v, a, half, g):
            prep_a(a, half, g)
            fence((xf, xo)[odd], v)
        return [lambda v, a=a, half=half, g=g: job(v, a, half, g)
                for a in outer for half in range(2) for g in range(4 * odd, 4 * odd + 4)]

    def out_proj(base, st, r, jobs):
        y = _dot(_bf(wo_t[...]), _bf(ob[z + r]))
        for g in range(D // 16):
            rows = pl.ds(16 * g, 16)
            x = xr[base + r, rows, :] + y[16 * g:16 * g + 16]
            xm[z + r, rows, :] = x
            add_stats(st, r, x[0:8])
            add_stats(st, r, x[8:16])
            run(jobs, x[0:8])

    def attention_block(p, first):
        s = 0 if first else p % 2
        cur, nxt = 8 * s, 8 * (1 - s)
        order = (0, 2, 4, 6, 1, 3, 5, 7)
        allh = (0, 1, 2, 3)
        st1 = {}
        if first:
            st0 = {}
            for r in range(NT_):
                rows_to_tile(0, r, st0)
                m, rs = mean_rstd(st0, r)
                xn[:, 128 * r:128 * r + 128] = pltpu.bitcast(((xr[z + r] - m) * rs).astype(BF), U32)
            for r in range(4):
                project_kv("k", xn, (r,), allh)
            cp_qkv("q").wait()
            cp_qkv("v").wait()
            cp_wo().wait()
            setup_qkv("q")
            project_kv("k", xn, (4, 5, 6, 7), allh)
            setup_qkv("v")
            setup_wo()
            for r in range(NT_):
                rows_to_tile(1, r, st1)
        else:
            xn[...] = xnn[...]
            ktile = {2: 3, 0: 4, 3: 5, 1: 6, 5: 7}
            down_final(nxt, st1, None, lambda a: a in ktile and project_kv("k", xn, (ktile[a],), allh))
        jobs = []
        project_q((0, 1, 2, 3), jobs)
        project_q((4, 5, 6, 7), jobs)
        if first:
            for cp in cp_ffn(0) + cp_tails():
                cp.wait()
        jobs += [lambda v: fence(pb, v)]
        jobs += [j for job in ln1_jobs(nxt, st1) for j in (job, lambda v: None)][:-1]
        del jobs[-4:-1:2]
        for vb in vbs:
            prime(vb, ob)
        prime(xf, a_ref)
        prime(xo, a_ref)
        for hg in range(4):
            for u in range(2):
                project_kv("v", xn, range(4 * u, 4 * u + 4), (hg,), jobs, 1 if hg == 0 else 6)
            assert not jobs
            jobs = mix_jobs(hg, order)
        for t in range(2):
            for hg in range(4):
                project_kv("k", xnn, (t,), (hg,), jobs, 6)
        assert not jobs
        st2 = {}
        for t, r in enumerate(order):
            if t > 0:
                ln2(st2, order[t - 1])
            jobs = {4: prep_a_jobs((2, 0, 1, 5), 0), 5: prep_a_jobs((3, 4, 6), 0),
                    6: prep_a_jobs((2, 4), 1)}.get(t, [])
            out_proj(cur, st2, r, jobs)
            assert not jobs
        ln2(st2, order[-1])
        last = []
        project_kv("k", xnn, (2,), allh, [last.append])
        for a in (0, 1, 5, 3, 6):
            for half in range(2):
                for g in range(4, 8):
                    chain(xo, last, prep_a(a, half, g))
        prep_a_tail()
        before = (lambda a: prep_r(0, a)) if first else None
        if first:
            prep_l(0)
        gate_up(0, before)

    def ffn_loop(first):
        def body(c, carry):
            if first:
                for cp in cp_ffn(c + 1):
                    cp.wait()

                @pl.when(c + RING < NC)
                def _():
                    for cp in cp_ffn(c + RING):
                        cp.start()
            down(c)
            if first:
                prep_l(c + 1)

            gate_up(c + 1, (lambda a: prep_r(c + 1, a)) if first else None)
            return carry
        lax.fori_loop(0, NC - 1, body, 0)

    cp_qkv("k").start()
    for u in range(4):
        cp_x(u).start()
    for cp in (cp_qkv("q"), cp_qkv("v"), cp_wo()) + cp_ffn(0) + cp_tails() + cp_ffn(1) + cp_ffn(2):
        cp.start()
    cp_qkv("k").wait()
    setup_qkv("k")
    for u in range(4):
        cp_x(u).wait()
        for t in range(X_SPLIT[u], X_SPLIT[u + 1]):
            x_to_rows(t)

    attention_block(0, True)
    ffn_loop(True)

    def pass_body(p, carry):
        attention_block(p, False)
        ffn_loop(False)
        return carry
    lax.fori_loop(1, 4, pass_body, 0)

    for b in range(3):
        tiles_to_rows(b, 0, range(NT_))

    def after(quad):
        tiles = range(4 * (quad % 2), 4 * (quad % 2) + 4)
        for b in ((0,), (1, 2))[quad // 2]:
            tiles_to_rows(b, 1, tiles)
            if quad in (0, 3):
                rows_to_out(b)
                cp_out(b).start()
    down_final(8, None, after)
    for b in range(3):
        cp_out(b).wait()


@jax.jit
def pallas_interleave_layers__sliding_local_dilated__glu_gated_bilinear__prompt_kernel(
    A_x: jax.Array,
    A_wqkv: jax.Array,
    A_wo: jax.Array,
    B_x: jax.Array,
    B_w_gate: jax.Array,
    B_w_up: jax.Array,
    B_w_down: jax.Array,
):
    del B_x
    vm = pltpu.VMEM
    scratch = [
        vm((D, S), BF), vm((D, 3 * D), BF), vm((D, D), BF),
        vm((RING, 512, FC), BF), vm((RING, 512, FC), BF), vm((RING, D, FC), BF),
        vm((D - 512, F), BF), vm((D - 512, F), BF),
        vm((5, 640, 128), F32),
        vm((3, D // 2, D), U32),
        vm((D // 2, D), U32),
        vm((2 * NT_ + 1, D, 128), F32),
        vm((NT_ + 1, D, 128), F32),
        vm((D // 2, S // 2), U32),
        vm((D // 2, S // 2), U32),
        vm((15, D, 128), F32),
        vm((16, MQ, 128), F32), vm((16, MQ, 128), F32), vm((16, MQ, 128), F32), vm((16, MQ, 128), F32),
        vm((NT_ + 1, W * H, 128), F32),
        vm((NT_, D // 2, 128), U32),
        vm((6, D, 128), F32),
        vm((6, S // 4, 128), F32),
        vm((49 * 128, 128), F32),
        vm((49, TQ // 2, 128), U32),
        vm((4, TQ // 2, 64), U32),
        vm((49, MQ, TQ), F32),
        vm((49, TQ // 2, 128), U32),
        vm((4, TQ, 256), F32),
        vm((16, TQ, 256), F32),
        vm((16, TQ, 128), F32),
        vm((NC, 49, 64, 256), U32),
        vm((NC, 49, MQ // 2, 128), U32),
        pltpu.SMEM((2,), jnp.int32),
        pltpu.SemaphoreType.DMA((11 + 3 * RING,)),
    ]
    hbm = pl.BlockSpec(memory_space=pl.ANY)
    out = pl.pallas_call(
        _kernel,
        in_specs=[hbm] * 6,
        out_specs=hbm,
        out_shape=jax.ShapeDtypeStruct((D, S), BF),
        scratch_shapes=scratch,
        compiler_params=pltpu.CompilerParams(vmem_limit_bytes=126 * 1024 * 1024),
    )(A_x.reshape(S, D).T, A_wqkv, A_wo, B_w_gate, B_w_up, B_w_down.T)
    return out.T.reshape(1, S, D)
```

```python
import math

import jax
import jax.numpy as jnp
from jax import lax
import jax.experimental.pallas as pl
import jax.experimental.pallas.tpu as pltpu

S, D, F = 2048, 576, 4608
H, DH, W = 32, 18, 8
NT_ = 8
TQ = 256
MQ = D // 4
FC = 512
NC = F // FC
RING = 3
X_SPLIT = (0, 5, 10, 14, 16)
EPS = 1e-5
SCALE = DH ** -0.5
EXP_C = SCALE * math.log2(math.e)
NEG = -1e9 / SCALE

BF, F32, U32 = jnp.bfloat16, jnp.float32, jnp.uint32
NT_DIMS = (((1,), (1,)), ((), ()))

LHS_SEL = {0: ((0, 0), 1, (1, 1)), 1: ((1, 0), 1, (1, 1)), 2: ((0, 0), 0, None), 3: ((1, 1), 0, None),
           4: ((0, 0), 1, (0, 1)), 5: ((1, 0), -1, (0, 0)), 6: ((0, 1), -1, (1, 1))}
RHS_SEL = {0: ((0, 0), 1, (1, 1)), 1: ((0, 0), 0, None), 2: ((0, 1), -1, (1, 1)), 3: ((1, 0), -1, (0, 0)),
           4: ((1, 1), 0, None), 5: ((0, 0), 1, (0, 1)), 6: ((1, 0), 1, (1, 1))}
G_ORDER = (2, 0, 1, 5, 3, 4, 6)


def _lhs1(a11, a12, a21, a22):
    return [a11 + a22, a21 + a22, a11, a22, a11 + a12, a21 - a11, a12 - a22]


def _rhs1(b11, b12, b21, b22):
    return [b11 + b22, b11, b12 - b22, b21 - b11, b22, b11 + b12, b21 + b22]


def _in2(fn, x):
    outer = [[fn(x[i][j], x[i][2 + j], x[2 + i][j], x[2 + i][2 + j]) for j in range(2)] for i in range(2)]
    return [v for a in range(7) for v in fn(outer[0][0][a], outer[0][1][a], outer[1][0][a], outer[1][1][a])]


def _select(sel, load):
    first, sign, second = sel
    v = load(first)
    if sign == 1:
        v = [a + b for a, b in zip(v, load(second))]
    elif sign == -1:
        v = [a - b for a, b in zip(v, load(second))]
    return v


def _pk(lo, hi):
    return pltpu.pack_elementwise([lo, hi], packed_dtype=BF)


def _lo(w):
    return pltpu.unpack_elementwise(w, index=0, packed_dtype=BF, unpacked_dtype=F32)


def _hi(w):
    return pltpu.unpack_elementwise(w, index=1, packed_dtype=BF, unpacked_dtype=F32)


def _bf(w):
    return pltpu.bitcast(w, BF)


def _dot(a, b):
    return jnp.dot(a, b, preferred_element_type=F32)


def _kernel(x_hbm, wqkv_hbm, wo_hbm, wg_hbm, wu_hbm, wd_hbm, out_hbm,
            xio, wqkv_raw, wo_raw, wg_raw, wu_raw, wd_raw, tg, tu,
            wts, wqkv_t, wo_t, xr, xm0, xm1, xn, xnn, kb, vb0, vb1, vb2, vb3, pb, ob, xf, xo, perm,
            a_ref, at_ref, acc, h_ref, ti, to, hf, r_ref, l_ref, zero_ref, sems):
    def clear(i, carry):
        zero_ref[i] = 0
        return carry
    lax.fori_loop(0, 2, clear, 0)
    z = zero_ref[0]
    z2 = zero_ref[1]
    vbs = (vb0, vb1, vb2, vb3)
    xm = [((xm0, xm1)[r // 2 % 2], r // 4 * 2 + r % 2) for r in range(NT_)]

    def fence(ref, v):
        ref[z + (ref.shape[0] - 1), 0:8, 0:128] = v

    def gate(ref, v):
        ref[pl.ds(pl.multiple_of(8 * z + (ref.shape[0] - 8), 8), 8), :] = v

    def prime(ref, other):
        ref[z2 + (ref.shape[0] - 1), 0:8, 0:128] = pltpu.bitcast(other[z, 0:8, 0:128], F32)

    def paced(ref, fns, skew):
        last = []

        def job(v, fn):
            last.append(fn())
            if len(last) > skew:
                v = pltpu.bitcast(last.pop(0) ^ pltpu.bitcast(v, U32), F32)
            fence(ref, v)
        return [lambda v, fn=fn: job(v, fn) for fn in fns]

    def spread(jobs, n):
        slots = [lambda v: None] * n
        for i, job in enumerate(jobs):
            slots[i * n // len(jobs)] = job
        return slots

    def run(jobs, v, n=1):
        for _ in range(n):
            if jobs:
                jobs.pop(0)(v)

    def tree(fn, v):
        while len(v) > 1:
            v = [fn(v[i], v[i + 1]) for i in range(0, len(v), 2)]
        return v[0]

    def cp_x(u):
        cols = pl.ds(128 * X_SPLIT[u], 128 * (X_SPLIT[u + 1] - X_SPLIT[u]))
        return pltpu.make_async_copy(x_hbm.at[:, cols], xio.at[:, cols], sems.at[u])

    def cp_out(b, u):
        rows, cols = (pl.ds(256 * b, 256), pl.ds(512 * u, 512)) if b < 2 else (pl.ds(512, 64), pl.ds(0, S))
        return pltpu.make_async_copy(xio.at[rows, cols], out_hbm.at[rows, cols], sems.at[4 * b + u])

    qkv_cols = {"k": pl.ds(512, 640), "v": pl.ds(1152, 576), "q": pl.ds(0, 512)}

    def cp_qkv(name):
        idx = 5 + "kvq".index(name)
        return pltpu.make_async_copy(wqkv_hbm.at[:, qkv_cols[name]], wqkv_raw.at[:, qkv_cols[name]], sems.at[idx])

    def cp_wo():
        return pltpu.make_async_copy(wo_hbm, wo_raw, sems.at[8])

    def cp_ffn(c):
        c0 = c * FC if isinstance(c, int) else pl.multiple_of(c * FC, FC)
        cols = pl.ds(c0, FC)
        slot = c % RING
        return (pltpu.make_async_copy(wg_hbm.at[0:512, cols], wg_raw.at[slot], sems.at[11 + 3 * slot]),
                pltpu.make_async_copy(wu_hbm.at[0:512, cols], wu_raw.at[slot], sems.at[12 + 3 * slot]),
                pltpu.make_async_copy(wd_hbm.at[:, cols], wd_raw.at[slot], sems.at[13 + 3 * slot]))

    def cp_tails():
        return (pltpu.make_async_copy(wg_hbm.at[512:D, :], tg, sems.at[9]),
                pltpu.make_async_copy(wu_hbm.at[512:D, :], tu, sems.at[10]))

    def transpose_cols(src, nb0, ncols):
        for nb in range(nb0, nb0 + 5):
            wn = min(128, ncols - 128 * nb)
            for kt in range(5):
                wk = 128 if kt < 4 else 64
                blk = src[128 * kt:128 * kt + wk, 128 * nb:128 * nb + wn].astype(F32)
                wts[kt, 128 * (nb - nb0):128 * (nb - nb0) + wn, 0:wk] = blk.T

    def setup_qkv(name):
        part = "qkv".index(name)
        nb0 = (D * part) // 128
        base = D * part - 128 * nb0
        transpose_cols(wqkv_raw, nb0, D * part + D)
        for hg in range(4):
            for kt in range(5):
                wk = 128 if kt < 4 else 64
                rows = [wts[kt, pl.ds(base + MQ * hg + d, 8, stride=DH), :][:, :wk] for d in range(DH)]
                w = jnp.concatenate(rows, axis=0).astype(BF)
                wqkv_t[part, 72 * hg:72 * hg + 72, 128 * kt:128 * kt + wk] = pltpu.bitcast(w, U32)

    def setup_wo():
        for nb in range(5):
            wn = 128 if nb < 4 else 64
            xf[nb, 0:D, 0:wn] = wo_raw[:, 128 * nb:128 * nb + wn].astype(F32)
        for nb in range(5):
            wn = 128 if nb < 4 else 64
            rows = []
            for hg in range(4):
                for d in range(0, DH, 2):
                    lo = xf[nb, pl.ds(MQ * hg + d, 8, stride=DH), :][:, :wn]
                    hi = xf[nb, pl.ds(MQ * hg + d + 1, 8, stride=DH), :][:, :wn]
                    rows.append(_pk(lo, hi))
            for kt in range(5):
                blk = _bf(jnp.concatenate(rows[8 * kt:8 * kt + 8], axis=0)).astype(F32).T
                wo_t[64 * nb:64 * nb + wn // 2, pl.ds(128 * kt, blk.shape[1])] = pltpu.bitcast(blk.astype(BF), U32)

    def pad_lanes(w):
        if w.shape[1] == 128:
            return w
        return jnp.concatenate([w, jnp.zeros((128, 128 - w.shape[1]), F32)], axis=1)

    def x_to_rows(t):
        for b in range(3):
            nw = 128 if b < 2 else 32
            w = pltpu.bitcast(xio[256 * b:256 * b + 2 * nw, 128 * t:128 * t + 128], F32)
            w = pad_lanes(w.T)
            for jj in range(8):
                perm[pl.ds(49 * (8 * t + jj) + b, 16, stride=3), :] = w[16 * jj:16 * jj + 16]

    def rows_to_tile(s, r, st):
        for b in range(3):
            nw = 128 if b < 2 else 32
            w = perm[pl.ds(3 * (2 * r + s) + b, 128, stride=49), :]
            x = _bf(w[:, :nw].T).astype(F32)
            xr[8 * s + r, 256 * b:256 * b + 2 * nw, :] = x
            for g in range(nw // 4):
                add_stats(st, r, x[8 * g:8 * g + 8])

    def tiles_to_rows(b, s, tiles):
        nw = 128 if b < 2 else 32
        for r in tiles:
            if s == 0:
                w = _pk(xr[r, pl.ds(256 * b, nw, stride=2), :], xr[r, pl.ds(256 * b + 1, nw, stride=2), :])
            else:
                w = ob[z + r, 128 * b:128 * b + nw, :]
            w = jnp.concatenate([pltpu.bitcast(w, F32)] * (128 // nw), axis=0)
            perm[pl.ds(3 * (2 * r + s) + b, 128, stride=49), :] = w.T

    def rows_to_out(b):
        def rows(t):
            return jnp.concatenate([perm[pl.ds(49 * (8 * t + jj) + b, 16, stride=3), :] for jj in range(8)], axis=0)
        group = lax.broadcasted_iota(jnp.int32, (128, 128), 1) // 32
        for u in range(4):
            if b < 2:
                for t in range(4 * u, 4 * u + 4):
                    xio[256 * b:256 * b + 256, 128 * t:128 * t + 128] = _bf(rows(t).T)
                cp_out(b, u).start()
            else:
                w = rows(4 * u)
                for t in range(1, 4):
                    w = jnp.where(group == t, rows(4 * u + t), w)
                w = _bf(w.T)
                for t in range(4):
                    xio[512:D, pl.ds(128 * (4 * u + t), 128)] = w[64 * t:64 * t + 64]
        if b == 2:
            cp_out(b, 0).start()

    def prep_r(c, a):
        slot = c % RING
        for u in range(2):
            for g in range(8):
                def load(quad):
                    ws = [pltpu.bitcast((wg_raw, wu_raw)[u][slot, pl.ds(128 * (2 * quad[0] + i) + 16 * g, 16),
                                                            pl.ds(256 * quad[1], 256)], U32) for i in range(2)]
                    ws = [w[:, 128 * j:128 * j + 128] for w in ws for j in range(2)]
                    return [_lo(w) for w in ws] + [_hi(w) for w in ws]
                v = _select(RHS_SEL[a], load)
                for b, (lo, hi) in enumerate(zip(_rhs1(*v[:4]), _rhs1(*v[4:]))):
                    r_ref[c, 7 * a + b, 8 * g:8 * g + 8, 128 * u:128 * u + 128] = _pk(lo, hi)

    def prep_l(c):
        slot = c % RING
        for g in range(MQ // 16):
            ws = [pltpu.bitcast(wd_raw[slot, pl.ds(MQ * i + 16 * g, 16), :], U32) for i in range(4)]
            ws = [[w[:, 128 * j:128 * j + 128] for j in range(4)] for w in ws]
            lo = _in2(_lhs1, [[_lo(w) for w in row] for row in ws])
            hi = _in2(_lhs1, [[_hi(w) for w in row] for row in ws])
            for k in range(49):
                l_ref[c, pl.ds(72 * k + 8 * g, 8), :] = _pk(lo[k], hi[k])

    def prep_a(a, half, g):
        src, row = (xf, xo)[g // 4], 32 * (g % 4) + half

        def load(quad):
            return [src[z2 + 2 * quad[1] + j, pl.ds(128 * (2 * quad[0] + i) + row + e, 8, stride=4), :]
                    for e in (0, 2) for i in range(2) for j in range(2)]
        v = _select(LHS_SEL[a], load)
        o = [_pk(lo, hi) for lo, hi in zip(_lhs1(*v[:4]), _lhs1(*v[4:]))]
        for b in range(7):
            a_ref[z + 7 * a + b, 64 * half + 8 * g:64 * half + 8 * g + 8, :] = o[b]
        return o[5] ^ o[6]

    def prep_a_tail():
        for i in range(4):
            for half in range(2):
                for u, src in enumerate((xf, xo)):
                    lo = src[z + 4, pl.ds(128 * i + half, 32, stride=4), :][:, :64]
                    hi = src[z + 4, pl.ds(128 * i + half + 2, 32, stride=4), :][:, :64]
                    at_ref[z + i, pl.ds(64 * half + 32 * u, 32), :] = _pk(lo, hi)

    def put(a):
        for g in range(16):
            def load(quad):
                return [hf[z + 4 * (2 * quad[1] + quad[0]) + t, pl.ds(o + 8 * g, 8), :]
                        for o in (0, 128) for t in (0, 2, 1, 3)]
            v = _select(RHS_SEL[a], load)
            for b, (lo, hi) in enumerate(zip(_rhs1(*v[:4]), _rhs1(*v[4:]))):
                h_ref[7 * a + b, 8 * g:8 * g + 8, :] = _pk(lo, hi)

    def strassen_inner(prod, nrow, emit):
        ld = lambda s: ti[z + s, 0:nrow, :]
        for s in range(3):
            ti[z + s, 0:nrow, :] = prod(s)
        emit(3, ((ld(0) - ld(1)) + ld(2)) + prod(5))
        m3 = prod(3)
        emit(2, ld(1) + m3)
        ti[z + 3, 0:nrow, :] = ld(0) + m3
        m4 = prod(4)
        emit(1, ld(2) + m4)
        ti[z + 3, 0:nrow, :] = ld(3) - m4
        emit(0, ld(3) + prod(6))

    def gate_up(c, before=None):
        c0 = c * FC if isinstance(c, int) else pl.multiple_of(c * FC, FC)

        def inner(a, emit):
            if before is not None:
                before(a)
            strassen_inner(lambda b: _dot(_bf(a_ref[z + 7 * a + b]), _bf(r_ref[c, 7 * a + b])), TQ, emit)

        def fin(quad, q, v):
            i, j = 2 * (quad // 2) + q // 2, 2 * (quad % 2) + q % 2
            cols = pl.ds(c0 + 128 * j, 128)
            wt = jnp.concatenate([tg[:, cols], tu[:, cols]], axis=1)
            v = v + _dot(_bf(at_ref[z + i]), wt)
            hf[z + 4 * quad + q] = v[:, :128] * v[:, 128:]

        def old(s, q):
            return to[z + 4 * s + q]

        def keep(s):
            def emit(q, v):
                to[z + 4 * s + q] = v
            return emit

        def emit3(q, v):
            fin(2, q, old(1, q) + v)
            to[z + 12 + q] = old(0, q) + v

        def emit4(q, v):
            fin(1, q, old(2, q) + v)
            to[z + 12 + q] = old(3, q) - v

        inner(2, keep(2))
        inner(0, keep(0))
        inner(1, keep(1))
        inner(5, lambda q, v: fin(3, q, ((old(0, q) - old(1, q)) + old(2, q)) + v))
        put(4)
        inner(3, emit3)
        put(2)
        inner(4, emit4)
        put(6)
        inner(6, lambda q, v: fin(0, q, old(3, q) + v))

    def down_prod(c, k, prev):
        return prev + lax.dot_general(_bf(l_ref[c, 72 * k:72 * k + 72, :]), _bf(h_ref[k]), NT_DIMS, preferred_element_type=F32)

    def down(c):
        for a, late in ((4, 1), (2, 0), (6, 3), (1, 5), (0, None), (3, None), (5, None)):
            for k in range(7 * a, 7 * a + 7):
                acc[k] = down_prod(c, k, jnp.where(c == 0, 0.0, acc[k]))
            if late is not None:
                put(late)

    def add_stats(st, r, x):
        st[r] = (x, x * x) if st.get(r) is None else (st[r][0] + x, st[r][1] + x * x)

    def mean_rstd(st, r):
        m = jnp.sum(st[r][0], axis=0, keepdims=True) * (1.0 / D)
        v = jnp.sum(st[r][1], axis=0, keepdims=True) * (1.0 / D) - m * m
        return m, lax.rsqrt(jnp.maximum(v, 0.0) + EPS)

    def down_final(base, st, after=None, between=None):
        def inner(a, emit, late=None):
            strassen_inner(lambda b: down_prod(NC - 1, 7 * a + b, acc[7 * a + b]), MQ, emit)
            if late is not None:
                put(late)
            if between is not None:
                between(a)

        def old(s, q):
            return to[z + 4 * s + q, 0:MQ, :]

        def keep(s, q, v):
            to[z + 4 * s + q, 0:MQ, :] = v

        def fin(quad, q, v):
            i, j = 2 * (quad // 2) + q // 2, 2 * (quad % 2) + q % 2
            rows = pl.ds(MQ * i, MQ)
            for e in range(2):
                ref, slot = xm[2 * j + e]
                x = ref[z + slot, rows, :] + v[:, 128 * e:128 * e + 128]
                if st is None:
                    ob[z + 2 * j + e, 72 * i:72 * i + 72, :] = pltpu.bitcast(x.astype(BF), U32)
                    continue
                xr[base + 2 * j + e, rows, :] = x
                for g in range(MQ // 8):
                    add_stats(st, 2 * j + e, x[8 * g:8 * g + 8])
            if after is not None and q == 0:
                after(quad)

        inner(4, lambda q, v: keep(0, q, v), 0)
        inner(2, lambda q, v: (fin(1, q, old(0, q) + v), keep(1, q, v)), 3)
        inner(6, lambda q, v: keep(0, q, v - old(0, q)), 1)
        inner(0, lambda q, v: (keep(0, q, old(0, q) + v), keep(1, q, old(1, q) + v)), 5)
        inner(3, lambda q, v: (fin(0, q, old(0, q) + v), keep(2, q, v)))
        inner(1, lambda q, v: (fin(2, q, old(2, q) + v), keep(1, q, old(1, q) - v)))
        inner(5, lambda q, v: fin(3, q, old(1, q) + v))

    def chain(ref, last, v, skew=1):
        last.append(pltpu.bitcast(v, F32))
        if len(last) > skew:
            fence(ref, last.pop(0))

    def ln1_jobs(base, st):
        mr = [mean_rstd(st, r) for r in range(NT_)]

        def job(r, k):
            y = (xr[z2 + base + r, pl.ds(64 * k, 64), :] - mr[r][0]) * mr[r][1]
            y = pltpu.bitcast(y.astype(BF), U32)
            xnn[32 * k:32 * k + 32, 128 * r:128 * r + 128] = y
            return tree(jnp.bitwise_xor, [y[8 * u:8 * u + 8] for u in range(4)])
        fns = [lambda r=r, k=k: job(r, k) for r in range(NT_) for k in range(9)]
        return [lambda v: fence(xr, v)] + paced(xr, fns, 2)

    def project_kv(name, src, tiles, hgs, jobs=(), every=1):
        dst = kb if name == "k" else vbs[hgs[0]]
        nrow = MQ * len(hgs)
        rows = pl.ds(MQ * hgs[0] if name == "k" else 0, nrow)
        lhs = wqkv_t["qkv".index(name), 72 * hgs[0]:72 * hgs[-1] + 72, :]
        y = _dot(_bf(lhs), _bf(src[:, 128 * tiles[0]:128 * tiles[-1] + 128]))
        for t, r in enumerate(tiles):
            tile = y[:, 128 * t:128 * t + 128]
            dst[z + 7 + r, rows, :] = tile
            if r >= 1:
                dst[z + r - 1, rows, :] = pltpu.roll(tile, 1, 1)
            for g in range(0, nrow // 8, every):
                run(jobs, tile[8 * g:8 * g + 8])

    def project_q(tiles, jobs):
        y = _dot(_bf(wqkv_t[0]), _bf(xn[:, 128 * tiles[0]:128 * tiles[-1] + 128]))
        for t, r in enumerate(tiles):
            for hg in range(4):
                lg = [None] * W
                for d in range(DH):
                    row = MQ * hg + 8 * d
                    q = y[row:row + 8, 128 * t:128 * t + 128]
                    for w in range(W):
                        v = q * kb[z + 7 + r - w, row:row + 8, :]
                        lg[w] = v if d == 0 else lg[w] + v
                    if d == 9:
                        run(jobs, q)
                for w in range(W):
                    pb[z + r, 32 * w + 8 * hg:32 * w + 8 * hg + 8, :] = lg[w]
                if hg % 2 == 1:
                    jobs.append(softmax_job(r, hg // 2))

    def softmax_job(r, sl):
        def job(v):
            fence(pb, v)
            lane0 = lax.broadcasted_iota(jnp.int32, (16, 128), 1) == 0
            lg = [pb[z2 + r, 32 * w + 16 * sl:32 * w + 16 * sl + 16, :] for w in range(W)]
            lg = [jnp.where(lane0, NEG, lg[w]) if w > r else lg[w] for w in range(W)]
            m = tree(jnp.maximum, lg)
            ex = [jnp.exp2((lg[w] - m) * EXP_C) for w in range(W)]
            inv = 1.0 / tree(jnp.add, ex)
            for w in range(W):
                pb[z2 + r, 32 * w + 16 * sl:32 * w + 16 * sl + 16, :] = ex[w] * inv
        return job

    def mix_jobs(hg, tiles):
        vb = vbs[hg]

        def job(r, d0):
            p = [pb[z2 + r, 32 * w + 8 * hg:32 * w + 8 * hg + 8, :] for w in range(W)]
            o = [tree(jnp.add, [p[w] * vb[z2 + 7 + r - w, pl.ds(8 * d, 8), :] for w in range(W)])
                 for d in range(d0, d0 + 6)]
            o = [_pk(o[e], o[e + 1]) for e in range(0, 6, 2)]
            ob[z + r, 72 * hg + 4 * d0:72 * hg + 4 * d0 + 24, :] = jnp.concatenate(o, axis=0)
            return o[0] ^ o[1] ^ o[2]
        return paced(vb, [lambda r=r, d0=d0: job(r, d0) for r in tiles for d0 in range(0, DH, 6)], 1)

    def ln2(st, r):
        m, rs = mean_rstd(st, r)
        (ref, slot), last = xm[r], []
        for kt in range(5):
            wk = 128 if kt < 4 else 64
            y = ((ref[z2 + slot, 128 * kt:128 * kt + wk, :] - m) * rs).T
            (xf, xo)[r % 2][z + kt, pl.ds(128 * (r // 2), 128), 0:wk] = y
            if kt < 4:
                chain(ref, last, y[0:8], 2)

    def prep_a_jobs(outer, odd):
        return paced((xf, xo)[odd], [lambda a=a, half=half, g=g: prep_a(a, half, g) for a in outer
                                     for half in range(2) for g in range(4 * odd, 4 * odd + 4)], 2)

    def out_proj(base, st, r, jobs):
        y = _dot(_bf(wo_t[...]), _bf(ob[z + r]))
        for g in range(D // 16):
            rows = pl.ds(16 * g, 16)
            x = xr[base + r, rows, :] + y[16 * g:16 * g + 16]
            xm[r][0][z + xm[r][1], rows, :] = x
            add_stats(st, r, x[0:8])
            add_stats(st, r, x[8:16])
            run(jobs, x[0:8])

    def attention_block(p, first):
        s = 0 if first else p % 2
        cur, nxt = 8 * s, 8 * (1 - s)
        order = (0, 2, 4, 6, 1, 3, 5, 7)
        allh = (0, 1, 2, 3)
        st1 = {}
        if first:
            st0 = {}

            def load_tiles(v, s, tiles):
                if v is not None:
                    gate(perm, v)
                for r in tiles:
                    rows_to_tile(s, r, (st0, st1)[s])
                    if s == 0:
                        m, rs = mean_rstd(st0, r)
                        xn[:, 128 * r:128 * r + 128] = pltpu.bitcast(((xr[z + r] - m) * rs).astype(BF), U32)
            load_tiles(None, 0, range(NT_))
            for r in range(4):
                project_kv("k", xn, (r,), allh, [lambda v: load_tiles(v, 1, range(NT_))] if r == 1 else [])
            cp_qkv("q").wait()
            cp_qkv("v").wait()
            cp_wo().wait()
            setup_qkv("q")
            project_kv("k", xn, (4, 5, 6, 7), allh)
            setup_qkv("v")
            setup_wo()
        else:
            xn[...] = xnn[...]
            ktile = {2: 3, 0: 4, 3: 5, 1: 6, 5: 7}
            down_final(nxt, st1, None, lambda a: a in ktile and project_kv("k", xn, (ktile[a],), allh))
        jobs = []
        project_q((0, 1, 2, 3), jobs)
        project_q((4, 5, 6, 7), jobs)
        if first:
            for cp in cp_ffn(0) + cp_tails():
                cp.wait()
        jobs += [lambda v: fence(pb, v)]
        jobs = spread(jobs, 3) + spread(ln1_jobs(nxt, st1), 141)
        for vb in vbs:
            prime(vb, ob)
        prime(xf, a_ref)
        prime(xo, a_ref)
        for hg in range(4):
            for u in range(2):
                project_kv("v", xn, range(4 * u, 4 * u + 4), (hg,), jobs, 1 if hg == 0 else 6)
            assert not jobs
            jobs = mix_jobs(hg, order)
        for t in range(2):
            for hg in range(4):
                project_kv("k", xnn, (t,), (hg,), jobs, 6)
        assert not jobs
        st2 = {}
        for t, r in enumerate(order):
            if t > 0:
                ln2(st2, order[t - 1])
            if t == 0 and first:
                prep_l(0)
            if t == 4:
                assert not jobs
                jobs = spread(prep_a_jobs(G_ORDER, 0), 100) + prep_a_jobs((2,), 1)
            out_proj(cur, st2, r, jobs)
        assert not jobs
        ln2(st2, order[-1])
        last = []
        project_kv("k", xnn, (2,), allh, [last.append])
        for a in G_ORDER[1:]:
            for half in range(2):
                for g in range(4, 8):
                    chain(xo, last, prep_a(a, half, g))
        prep_a_tail()
        gate_up(0, (lambda a: prep_r(0, a)) if first else None)

    def ffn_loop(first):
        def body(c, carry):
            if first:
                for cp in cp_ffn(c + 1):
                    cp.wait()

                @pl.when(c + RING < NC)
                def _():
                    for cp in cp_ffn(c + RING):
                        cp.start()
            down(c)
            if first:
                prep_l(c + 1)

            gate_up(c + 1, (lambda a: prep_r(c + 1, a)) if first else None)
            return carry
        lax.fori_loop(0, NC - 1, body, 0)

    cp_qkv("k").start()
    for u in range(4):
        cp_x(u).start()
    for cp in (cp_qkv("q"), cp_qkv("v"), cp_wo()) + cp_ffn(0) + cp_tails() + cp_ffn(1) + cp_ffn(2):
        cp.start()
    cp_qkv("k").wait()
    setup_qkv("k")
    for u in range(4):
        cp_x(u).wait()
        for t in range(X_SPLIT[u], X_SPLIT[u + 1]):
            x_to_rows(t)

    attention_block(0, True)
    ffn_loop(True)

    def pass_body(p, carry):
        attention_block(p, False)
        ffn_loop(False)
        return carry
    lax.fori_loop(1, 4, pass_body, 0)

    for b in range(3):
        tiles_to_rows(b, 0, range(NT_))

    def after(quad):
        tiles = range(4 * (quad % 2), 4 * (quad % 2) + 4)
        slabs = ((0,), (2, 1))[quad // 2]
        for b in slabs:
            tiles_to_rows(b, 1, tiles)
        if quad in (0, 3):
            for b in slabs:
                rows_to_out(b)
    down_final(None, None, after)
    for b, u in [(b, u) for b in range(2) for u in range(4)] + [(2, 0)]:
        cp_out(b, u).wait()


@jax.jit
def pallas_interleave_layers__sliding_local_dilated__glu_gated_bilinear__prompt_kernel(
    A_x: jax.Array,
    A_wqkv: jax.Array,
    A_wo: jax.Array,
    B_x: jax.Array,
    B_w_gate: jax.Array,
    B_w_up: jax.Array,
    B_w_down: jax.Array,
):
    del B_x
    vm = pltpu.VMEM
    scratch = [
        vm((D, S), BF), vm((D, 3 * D), BF), vm((D, D), BF),
        vm((RING, 512, FC), BF), vm((RING, 512, FC), BF), vm((RING, D, FC), BF),
        vm((D - 512, F), BF), vm((D - 512, F), BF),
        vm((5, 640, 128), F32),
        vm((3, D // 2, D), U32),
        vm((D // 2, D), U32),
        vm((2 * NT_ + 1, D, 128), F32),
        vm((5, D, 128), F32),
        vm((5, D, 128), F32),
        vm((D // 2, S // 2), U32),
        vm((D // 2, S // 2), U32),
        vm((15, D, 128), F32),
        vm((16, MQ, 128), F32), vm((16, MQ, 128), F32), vm((16, MQ, 128), F32), vm((16, MQ, 128), F32),
        vm((NT_ + 1, W * H, 128), F32),
        vm((NT_, D // 2, 128), U32),
        vm((6, D, 128), F32),
        vm((6, S // 4, 128), F32),
        vm((49 * 128 + 32, 128), F32),
        vm((49, TQ // 2, 128), U32),
        vm((4, TQ // 2, 64), U32),
        vm((49, MQ, TQ), F32),
        vm((49, TQ // 2, 128), U32),
        vm((4, TQ, 256), F32),
        vm((16, TQ, 256), F32),
        vm((16, TQ, 128), F32),
        vm((NC, 49, 64, 256), U32),
        vm((NC, 3552, 128), U32),
        pltpu.SMEM((2,), jnp.int32),
        pltpu.SemaphoreType.DMA((11 + 3 * RING,)),
    ]
    hbm = pl.BlockSpec(memory_space=pl.ANY)
    out = pl.pallas_call(
        _kernel,
        in_specs=[hbm] * 6,
        out_specs=hbm,
        out_shape=jax.ShapeDtypeStruct((D, S), BF),
        scratch_shapes=scratch,
        compiler_params=pltpu.CompilerParams(vmem_limit_bytes=126 * 1024 * 1024),
    )(A_x.reshape(S, D).T, A_wqkv, A_wo, B_w_gate, B_w_up, B_w_down.T)
    return out.T.reshape(1, S, D)
```

```python
import math

import jax
import jax.numpy as jnp
from jax import lax
import jax.experimental.pallas as pl
import jax.experimental.pallas.tpu as pltpu

S, D, F = 2048, 576, 4608
H, DH, W = 32, 18, 8
NT_ = 8
TQ = 256
MQ = D // 4
FC = 512
NC = F // FC
RING = 3
X_SPLIT = (0, 5, 10, 14, 16)
EPS = 1e-5
SCALE = DH ** -0.5
EXP_C = SCALE * math.log2(math.e)
NEG = -1e9 / SCALE

BF, F32, U32 = jnp.bfloat16, jnp.float32, jnp.uint32
NT_DIMS = (((1,), (1,)), ((), ()))

LHS_SEL = {0: ((0, 0), 1, (1, 1)), 1: ((1, 0), 1, (1, 1)), 2: ((0, 0), 0, None), 3: ((1, 1), 0, None),
           4: ((0, 0), 1, (0, 1)), 5: ((1, 0), -1, (0, 0)), 6: ((0, 1), -1, (1, 1))}
RHS_SEL = {0: ((0, 0), 1, (1, 1)), 1: ((0, 0), 0, None), 2: ((0, 1), -1, (1, 1)), 3: ((1, 0), -1, (0, 0)),
           4: ((1, 1), 0, None), 5: ((0, 0), 1, (0, 1)), 6: ((1, 0), 1, (1, 1))}
G_ORDER = (2, 0, 1, 5, 3, 4, 6)


def _lhs1(a11, a12, a21, a22):
    return [a11 + a22, a21 + a22, a11, a22, a11 + a12, a21 - a11, a12 - a22]


def _rhs1(b11, b12, b21, b22):
    return [b11 + b22, b11, b12 - b22, b21 - b11, b22, b11 + b12, b21 + b22]


def _in2(fn, x):
    outer = [[fn(x[i][j], x[i][2 + j], x[2 + i][j], x[2 + i][2 + j]) for j in range(2)] for i in range(2)]
    return [v for a in range(7) for v in fn(outer[0][0][a], outer[0][1][a], outer[1][0][a], outer[1][1][a])]


def _select(sel, load):
    first, sign, second = sel
    v = load(first)
    if sign == 1:
        v = [a + b for a, b in zip(v, load(second))]
    elif sign == -1:
        v = [a - b for a, b in zip(v, load(second))]
    return v


def _pk(lo, hi):
    return pltpu.pack_elementwise([lo, hi], packed_dtype=BF)


def _lo(w):
    return pltpu.unpack_elementwise(w, index=0, packed_dtype=BF, unpacked_dtype=F32)


def _hi(w):
    return pltpu.unpack_elementwise(w, index=1, packed_dtype=BF, unpacked_dtype=F32)


def _bf(w):
    return pltpu.bitcast(w, BF)


def _u32(x):
    return pltpu.bitcast(x.astype(BF), U32)


def _dot(a, b):
    return jnp.dot(a, b, preferred_element_type=F32)


def _kernel(x_hbm, wqkv_hbm, wo_hbm, wg_hbm, wu_hbm, wd_hbm, out_hbm,
            xio, wqkv_raw, wo_raw, wg_raw, wu_raw, wd_raw, tg, tu,
            wts, wqkv_t, wo_t, xr, xm0, xm1, xn, xnn, kb, vb0, vb1, vb2, vb3, pb, ob, xf, xo, perm,
            a_ref, at_ref, acc, h_ref, ti, to, hf, r_ref, l_ref, zero_ref, sems):
    def clear(i, carry):
        zero_ref[i] = 0
        return carry
    lax.fori_loop(0, 2, clear, 0)
    z = zero_ref[0]
    z2 = zero_ref[1]
    vbs = (vb0, vb1, vb2, vb3)
    xm = [((xm0, xm1)[r // 2 % 2], r // 4 * 2 + r % 2) for r in range(NT_)]

    def fence(ref, v):
        ref[z + (ref.shape[0] - 1), 0:8, 0:128] = v

    def gate(ref, v):
        ref[pl.ds(pl.multiple_of(8 * z + (ref.shape[0] - 8), 8), 8), :] = v

    def prime(ref, other):
        ref[z2 + (ref.shape[0] - 1), 0:8, 0:128] = pltpu.bitcast(other[z, 0:8, 0:128], F32)

    def paced(ref, fns, skew):
        last = []

        def job(v, fn):
            last.append(fn())
            if len(last) > skew:
                v = pltpu.bitcast(last.pop(0) ^ pltpu.bitcast(v, U32), F32)
            fence(ref, v)
        return [lambda v, fn=fn: job(v, fn) for fn in fns]

    def spread(jobs, n):
        slots = [lambda v: None] * n
        for i, job in enumerate(jobs):
            slots[i * n // len(jobs)] = job
        return slots

    def run(jobs, v, n=1):
        for _ in range(n):
            if jobs:
                jobs.pop(0)(v)

    def tree(fn, v):
        while len(v) > 1:
            v = [fn(v[i], v[i + 1]) for i in range(0, len(v), 2)]
        return v[0]

    def cp_x(u):
        cols = pl.ds(128 * X_SPLIT[u], 128 * (X_SPLIT[u + 1] - X_SPLIT[u]))
        return pltpu.make_async_copy(x_hbm.at[:, cols], xio.at[:, cols], sems.at[u])

    def cp_out(b, u):
        rows, cols = (pl.ds(256 * b, 256), pl.ds(512 * u, 512)) if b < 2 else (pl.ds(512, 64), pl.ds(0, S))
        return pltpu.make_async_copy(xio.at[rows, cols], out_hbm.at[rows, cols], sems.at[4 * b + u])

    qkv_cols = {"k": pl.ds(512, 640), "v": pl.ds(1152, 576), "q": pl.ds(0, 512)}

    def cp_qkv(name):
        idx = 5 + "kvq".index(name)
        return pltpu.make_async_copy(wqkv_hbm.at[:, qkv_cols[name]], wqkv_raw.at[:, qkv_cols[name]], sems.at[idx])

    def cp_wo():
        return pltpu.make_async_copy(wo_hbm, wo_raw, sems.at[8])

    def cp_ffn(c):
        c0 = c * FC if isinstance(c, int) else pl.multiple_of(c * FC, FC)
        cols = pl.ds(c0, FC)
        slot = c % RING
        return (pltpu.make_async_copy(wg_hbm.at[0:512, cols], wg_raw.at[slot], sems.at[11 + 3 * slot]),
                pltpu.make_async_copy(wu_hbm.at[0:512, cols], wu_raw.at[slot], sems.at[12 + 3 * slot]),
                pltpu.make_async_copy(wd_hbm.at[:, cols], wd_raw.at[slot], sems.at[13 + 3 * slot]))

    def cp_tails():
        return (pltpu.make_async_copy(wg_hbm.at[512:D, :], tg, sems.at[9]),
                pltpu.make_async_copy(wu_hbm.at[512:D, :], tu, sems.at[10]))

    def transpose_cols(src, nb0, ncols):
        for nb in range(nb0, nb0 + 5):
            wn = min(128, ncols - 128 * nb)
            for kt in range(5):
                wk = 128 if kt < 4 else 64
                blk = src[128 * kt:128 * kt + wk, 128 * nb:128 * nb + wn].astype(F32)
                wts[kt, 128 * (nb - nb0):128 * (nb - nb0) + wn, 0:wk] = blk.T

    def setup_qkv(name):
        part = "qkv".index(name)
        nb0 = (D * part) // 128
        base = D * part - 128 * nb0
        transpose_cols(wqkv_raw, nb0, D * part + D)

        def rows(hg, kt, d):
            return jnp.concatenate([wts[kt, pl.ds(base + MQ * hg + d + e, 8, stride=DH), :] for e in range(2)], axis=0)
        for a in range(2):
            for d in range(0, DH, 2):
                for j in range(2):
                    w = _lhs1(rows(a, j, d), rows(a, 2 + j, d), rows(a + 2, j, d), rows(a + 2, 2 + j, d))
                    for b in range(7):
                        wqkv_t[2 * part + a, b, 4 * d:4 * d + 8, 128 * j:128 * j + 128] = _u32(w[b])
                    wqkv_t[2 * part + a, 7, 4 * d:4 * d + 8, 128 * j:128 * j + 64] = _u32(rows(a + 2 * j, 4, d)[:, :64])

    def setup_wo():
        for nb in range(5):
            wn = 128 if nb < 4 else 64
            xf[nb, 0:D, 0:wn] = wo_raw[:, 128 * nb:128 * nb + wn].astype(F32)
        for nb in range(5):
            wn = 128 if nb < 4 else 64
            rows = []
            for hg in range(4):
                for d in range(0, DH, 2):
                    lo = xf[nb, pl.ds(MQ * hg + d, 8, stride=DH), :][:, :wn]
                    hi = xf[nb, pl.ds(MQ * hg + d + 1, 8, stride=DH), :][:, :wn]
                    rows.append(_pk(lo, hi))
            for kt in range(5):
                blk = _bf(jnp.concatenate(rows[8 * kt:8 * kt + 8], axis=0)).astype(F32).T
                wo_t[64 * nb:64 * nb + wn // 2, pl.ds(128 * kt, blk.shape[1])] = pltpu.bitcast(blk.astype(BF), U32)

    def pad_lanes(w):
        if w.shape[1] == 128:
            return w
        return jnp.concatenate([w, jnp.zeros((128, 128 - w.shape[1]), F32)], axis=1)

    def x_to_rows(t):
        for b in range(3):
            nw = 128 if b < 2 else 32
            w = pltpu.bitcast(xio[256 * b:256 * b + 2 * nw, 128 * t:128 * t + 128], F32)
            w = pad_lanes(w.T)
            for jj in range(8):
                perm[pl.ds(49 * (8 * t + jj) + b, 16, stride=3), :] = w[16 * jj:16 * jj + 16]

    def rows_to_tile(s, r, st):
        for b in range(3):
            nw = 128 if b < 2 else 32
            w = perm[pl.ds(3 * (2 * r + s) + b, 128, stride=49), :]
            x = _bf(w[:, :nw].T).astype(F32)
            xr[8 * s + r, 256 * b:256 * b + 2 * nw, :] = x
            for g in range(nw // 4):
                add_stats(st, r, x[8 * g:8 * g + 8])

    def tiles_to_rows(b, s, tiles):
        nw = 128 if b < 2 else 32
        for r in tiles:
            if s == 0:
                w = _pk(xr[r, pl.ds(256 * b, nw, stride=2), :], xr[r, pl.ds(256 * b + 1, nw, stride=2), :])
            else:
                w = ob[z + r, 128 * b:128 * b + nw, :]
            w = jnp.concatenate([pltpu.bitcast(w, F32)] * (128 // nw), axis=0)
            perm[pl.ds(3 * (2 * r + s) + b, 128, stride=49), :] = w.T

    def rows_to_out(b):
        def rows(t):
            return jnp.concatenate([perm[pl.ds(49 * (8 * t + jj) + b, 16, stride=3), :] for jj in range(8)], axis=0)
        group = lax.broadcasted_iota(jnp.int32, (128, 128), 1) // 32
        for u in range(4):
            if b < 2:
                for t in range(4 * u, 4 * u + 4):
                    xio[256 * b:256 * b + 256, 128 * t:128 * t + 128] = _bf(rows(t).T)
                cp_out(b, u).start()
            else:
                w = rows(4 * u)
                for t in range(1, 4):
                    w = jnp.where(group == t, rows(4 * u + t), w)
                w = _bf(w.T)
                for t in range(4):
                    xio[512:D, pl.ds(128 * (4 * u + t), 128)] = w[64 * t:64 * t + 64]
        if b == 2:
            cp_out(b, 0).start()

    def prep_r(c, a):
        slot = c % RING
        for u in range(2):
            for g in range(8):
                def load(quad):
                    ws = [pltpu.bitcast((wg_raw, wu_raw)[u][slot, pl.ds(128 * (2 * quad[0] + i) + 16 * g, 16),
                                                            pl.ds(256 * quad[1], 256)], U32) for i in range(2)]
                    ws = [w[:, 128 * j:128 * j + 128] for w in ws for j in range(2)]
                    return [_lo(w) for w in ws] + [_hi(w) for w in ws]
                v = _select(RHS_SEL[a], load)
                for b, (lo, hi) in enumerate(zip(_rhs1(*v[:4]), _rhs1(*v[4:]))):
                    r_ref[c, 7 * a + b, 8 * g:8 * g + 8, 128 * u:128 * u + 128] = _pk(lo, hi)

    def prep_l(c):
        slot = c % RING
        for g in range(MQ // 16):
            ws = [pltpu.bitcast(wd_raw[slot, pl.ds(MQ * i + 16 * g, 16), :], U32) for i in range(4)]
            ws = [[w[:, 128 * j:128 * j + 128] for j in range(4)] for w in ws]
            lo = _in2(_lhs1, [[_lo(w) for w in row] for row in ws])
            hi = _in2(_lhs1, [[_hi(w) for w in row] for row in ws])
            for k in range(49):
                l_ref[c, pl.ds(72 * k + 8 * g, 8), :] = _pk(lo[k], hi[k])

    def prep_a(a, half, g):
        src, row = (xf, xo)[g // 4], 32 * (g % 4) + half

        def load(quad):
            return [src[z2 + 2 * quad[1] + j, pl.ds(128 * (2 * quad[0] + i) + row + e, 8, stride=4), :]
                    for e in (0, 2) for i in range(2) for j in range(2)]
        v = _select(LHS_SEL[a], load)
        o = [_pk(lo, hi) for lo, hi in zip(_lhs1(*v[:4]), _lhs1(*v[4:]))]
        for b in range(7):
            a_ref[z + 7 * a + b, 64 * half + 8 * g:64 * half + 8 * g + 8, :] = o[b]
        return o[5] ^ o[6]

    def prep_a_tail():
        for i in range(4):
            for half in range(2):
                for u, src in enumerate((xf, xo)):
                    lo = src[z + 4, pl.ds(128 * i + half, 32, stride=4), :][:, :64]
                    hi = src[z + 4, pl.ds(128 * i + half + 2, 32, stride=4), :][:, :64]
                    at_ref[z + i, pl.ds(64 * half + 32 * u, 32), :] = _pk(lo, hi)

    def put(a):
        for g in range(16):
            def load(quad):
                return [hf[z + 4 * (2 * quad[1] + quad[0]) + t, pl.ds(o + 8 * g, 8), :]
                        for o in (0, 128) for t in (0, 2, 1, 3)]
            v = _select(RHS_SEL[a], load)
            for b, (lo, hi) in enumerate(zip(_rhs1(*v[:4]), _rhs1(*v[4:]))):
                h_ref[7 * a + b, 8 * g:8 * g + 8, :] = _pk(lo, hi)

    def strassen_inner(prod, nrow, emit):
        ld = lambda s: ti[z + s, 0:nrow, :]
        for s in range(3):
            ti[z + s, 0:nrow, :] = prod(s)
        emit(3, ((ld(0) - ld(1)) + ld(2)) + prod(5))
        m3 = prod(3)
        emit(2, ld(1) + m3)
        ti[z + 3, 0:nrow, :] = ld(0) + m3
        m4 = prod(4)
        emit(1, ld(2) + m4)
        ti[z + 3, 0:nrow, :] = ld(3) - m4
        emit(0, ld(3) + prod(6))

    def gate_up(c, before=None):
        c0 = c * FC if isinstance(c, int) else pl.multiple_of(c * FC, FC)

        def inner(a, emit):
            if before is not None:
                before(a)
            strassen_inner(lambda b: _dot(_bf(a_ref[z + 7 * a + b]), _bf(r_ref[c, 7 * a + b])), TQ, emit)

        def fin(quad, q, v):
            i, j = 2 * (quad // 2) + q // 2, 2 * (quad % 2) + q % 2
            cols = pl.ds(c0 + 128 * j, 128)
            wt = jnp.concatenate([tg[:, cols], tu[:, cols]], axis=1)
            v = v + _dot(_bf(at_ref[z + i]), wt)
            hf[z + 4 * quad + q] = v[:, :128] * v[:, 128:]

        def old(s, q):
            return to[z + 4 * s + q]

        def keep(s):
            def emit(q, v):
                to[z + 4 * s + q] = v
            return emit

        def emit3(q, v):
            fin(2, q, old(1, q) + v)
            to[z + 12 + q] = old(0, q) + v

        def emit4(q, v):
            fin(1, q, old(2, q) + v)
            to[z + 12 + q] = old(3, q) - v

        inner(2, keep(2))
        inner(0, keep(0))
        inner(1, keep(1))
        inner(5, lambda q, v: fin(3, q, ((old(0, q) - old(1, q)) + old(2, q)) + v))
        put(4)
        inner(3, emit3)
        put(2)
        inner(4, emit4)
        put(6)
        inner(6, lambda q, v: fin(0, q, old(3, q) + v))

    def down_prod(c, k, prev):
        return prev + lax.dot_general(_bf(l_ref[c, 72 * k:72 * k + 72, :]), _bf(h_ref[k]), NT_DIMS, preferred_element_type=F32)

    def down(c):
        for a, late in ((4, 1), (2, 0), (6, 3), (1, 5), (0, None), (3, None), (5, None)):
            for k in range(7 * a, 7 * a + 7):
                acc[k] = down_prod(c, k, jnp.where(c == 0, 0.0, acc[k]))
            if late is not None:
                put(late)

    def add_stats(st, r, x):
        st[r] = (x, x * x) if st.get(r) is None else (st[r][0] + x, st[r][1] + x * x)

    def mean_rstd(st, r):
        m = jnp.sum(st[r][0], axis=0, keepdims=True) * (1.0 / D)
        v = jnp.sum(st[r][1], axis=0, keepdims=True) * (1.0 / D) - m * m
        return m, lax.rsqrt(jnp.maximum(v, 0.0) + EPS)

    def down_final(base, st, after=None, between=None):
        def inner(a, emit, late=None):
            strassen_inner(lambda b: down_prod(NC - 1, 7 * a + b, acc[7 * a + b]), MQ, emit)
            if late is not None:
                put(late)
            if between is not None:
                between(a)

        def old(s, q):
            return to[z + 4 * s + q, 0:MQ, :]

        def keep(s, q, v):
            to[z + 4 * s + q, 0:MQ, :] = v

        def fin(quad, q, v):
            i, j = 2 * (quad // 2) + q // 2, 2 * (quad % 2) + q % 2
            rows = pl.ds(MQ * i, MQ)
            for e in range(2):
                ref, slot = xm[2 * j + e]
                x = ref[z + slot, rows, :] + v[:, 128 * e:128 * e + 128]
                if st is None:
                    ob[z + 2 * j + e, 72 * i:72 * i + 72, :] = pltpu.bitcast(x.astype(BF), U32)
                    continue
                xr[base + 2 * j + e, rows, :] = x
                for g in range(MQ // 8):
                    add_stats(st, 2 * j + e, x[8 * g:8 * g + 8])
            if after is not None and q == 0:
                after(quad)

        inner(4, lambda q, v: keep(0, q, v), 0)
        inner(2, lambda q, v: (fin(1, q, old(0, q) + v), keep(1, q, v)), 3)
        inner(6, lambda q, v: keep(0, q, v - old(0, q)), 1)
        inner(0, lambda q, v: (keep(0, q, old(0, q) + v), keep(1, q, old(1, q) + v)), 5)
        inner(3, lambda q, v: (fin(0, q, old(0, q) + v), keep(2, q, v)))
        inner(1, lambda q, v: (fin(2, q, old(2, q) + v), keep(1, q, old(1, q) - v)))
        inner(5, lambda q, v: fin(3, q, old(1, q) + v))

    def chain(ref, last, v, skew=1):
        last.append(pltpu.bitcast(v, F32))
        if len(last) > skew:
            fence(ref, last.pop(0))

    def ln1_fns(dst, base, st, pairs):
        mr = {r: mean_rstd(st, r) for u in pairs for r in (2 * u, 2 * u + 1)}

        def norm(r, row, n):
            return (xr[z2 + base + r, pl.ds(row, n), :] - mr[r][0]) * mr[r][1]

        def job(u, g):
            if g == 16:
                y = jnp.concatenate([_u32(norm(2 * u + e, 512, 64)) for e in range(2)], axis=0)
                dst[u, 896:960, :] = y
                return tree(jnp.bitwise_xor, [y[8 * k:8 * k + 8] for k in range(8)])
            y = [_u32(v) for v in _rhs1(*[norm(2 * u + e, 256 * k + 16 * g, 16) for k in range(2) for e in range(2)])]
            for b in range(7):
                dst[u, pl.ds(128 * b + 8 * g, 8), :] = y[b]
            return y[5] ^ y[6]
        return [lambda u=u, g=g: job(u, g) for u in pairs for g in range(17)]

    def project(name, src, a, u, emit):
        w = 2 * "qkv".index(name) + a
        m = lambda b: _dot(_bf(wqkv_t[w, b]), _bf(src[u, 128 * b:128 * b + 128, :]))
        xt = lambda: _bf(jnp.concatenate([src[u, 896:928, :], src[u, 928:960, :]], axis=1))
        tail = lambda i: _dot(_bf(wqkv_t[w, 7, :, 128 * i:128 * i + 64]), xt())
        ta, m4 = tail(0), m(4)
        s11, s12 = ta[:, :128] - m4, ta[:, 128:] + m4
        s22 = m(2)
        emit(a, 2 * u + 1, s12 + s22)
        s11 = s11 + m(6)
        m0 = m(0)
        s11, s22 = s11 + m0, s22 + m0
        s21 = m(3)
        emit(a, 2 * u, s11 + s21)
        tb = tail(1)
        s21, s22 = s21 + tb[:, :128], s22 + tb[:, 128:]
        m1 = m(1)
        emit(a + 2, 2 * u, s21 + m1)
        emit(a + 2, 2 * u + 1, (s22 - m1) + m(5))

    def project_kv(name, src, a, u, jobs=(), every=1):
        def emit(hg, r, y):
            dst, rows = (kb, pl.ds(MQ * hg, MQ)) if name == "k" else (vbs[hg], pl.ds(0, MQ))
            dst[z + 7 + r, rows, :] = y
            if r >= 1:
                dst[z + r - 1, rows, :] = pltpu.roll(y, 1, 1)
            for g in range(0, DH, every):
                run(jobs, y[8 * g:8 * g + 8])
        project(name, src, a, u, emit)

    def prow(hg, w):
        return pl.ds(32 * w + 16 * (hg % 2) + 8 * (hg // 2), 8)

    def project_q(a, u, jobs):
        def emit(hg, r, y):
            lg = [None] * W
            for d in range(DH):
                q = y[8 * d:8 * d + 8]
                for w in range(W):
                    v = q * kb[z + 7 + r - w, pl.ds(MQ * hg + 8 * d, 8), :]
                    lg[w] = v if d == 0 else lg[w] + v
                if d == 9:
                    run(jobs, q)
            for w in range(W):
                pb[z + r, prow(hg, w), :] = lg[w]
            if hg >= 2:
                jobs.append(softmax_job(r, a))
        project("q", xn, a, u, emit)

    def softmax_job(r, sl):
        def job(v):
            fence(pb, v)
            lane0 = lax.broadcasted_iota(jnp.int32, (16, 128), 1) == 0
            lg = [pb[z2 + r, 32 * w + 16 * sl:32 * w + 16 * sl + 16, :] for w in range(W)]
            lg = [jnp.where(lane0, NEG, lg[w]) if w > r else lg[w] for w in range(W)]
            m = tree(jnp.maximum, lg)
            ex = [jnp.exp2((lg[w] - m) * EXP_C) for w in range(W)]
            inv = 1.0 / tree(jnp.add, ex)
            for w in range(W):
                pb[z2 + r, 32 * w + 16 * sl:32 * w + 16 * sl + 16, :] = ex[w] * inv
        return job

    def mix_jobs(hg, tiles):
        vb = vbs[hg]

        def job(r, d0):
            p = [pb[z2 + r, prow(hg, w), :] for w in range(W)]
            o = [tree(jnp.add, [p[w] * vb[z2 + 7 + r - w, pl.ds(8 * d, 8), :] for w in range(W)])
                 for d in range(d0, d0 + 6)]
            o = [_pk(o[e], o[e + 1]) for e in range(0, 6, 2)]
            ob[z + r, 72 * hg + 4 * d0:72 * hg + 4 * d0 + 24, :] = jnp.concatenate(o, axis=0)
            return o[0] ^ o[1] ^ o[2]
        return paced(vb, [lambda r=r, d0=d0: job(r, d0) for r in tiles for d0 in range(0, DH, 6)], 1)

    def ln2(st, r):
        m, rs = mean_rstd(st, r)
        (ref, slot), last = xm[r], []
        for kt in range(5):
            wk = 128 if kt < 4 else 64
            y = ((ref[z2 + slot, 128 * kt:128 * kt + wk, :] - m) * rs).T
            (xf, xo)[r % 2][z + kt, pl.ds(128 * (r // 2), 128), 0:wk] = y
            if kt < 4:
                chain(ref, last, y[0:8], 2)

    def prep_a_jobs(outer, odd):
        return paced((xf, xo)[odd], [lambda a=a, half=half, g=g: prep_a(a, half, g) for a in outer
                                     for half in range(2) for g in range(4 * odd, 4 * odd + 4)], 2)

    def out_proj(base, st, r, jobs):
        y = _dot(_bf(wo_t[...]), _bf(ob[z + r]))
        for g in range(D // 16):
            rows = pl.ds(16 * g, 16)
            x = xr[base + r, rows, :] + y[16 * g:16 * g + 16]
            xm[r][0][z + xm[r][1], rows, :] = x
            add_stats(st, r, x[0:8])
            add_stats(st, r, x[8:16])
            run(jobs, x[0:8])

    def attention_block(p, first):
        s = 0 if first else p % 2
        cur, nxt = 8 * s, 8 * (1 - s)
        order = (0, 2, 4, 6, 1, 3, 5, 7)
        st1 = {}
        if first:
            st0 = {}
            for u in range(4):
                rows_to_tile(0, 2 * u, st0)
                rows_to_tile(0, 2 * u + 1, st0)
                for fn in ln1_fns(xn, 0, st0, (u,)):
                    fn()

            def load_next(v):
                gate(perm, v)
                for r in range(NT_):
                    rows_to_tile(1, r, st1)
            for u in range(2):
                for a in range(2):
                    project_kv("k", xn, a, u, [load_next] if (u, a) == (0, 1) else [])
            cp_qkv("q").wait()
            cp_qkv("v").wait()
            cp_wo().wait()
            setup_qkv("q")
            for u in range(2, 4):
                for a in range(2):
                    project_kv("k", xn, a, u)
            setup_qkv("v")
            setup_wo()
        else:
            xn[...] = xnn[...]
            unit = {2: (0, 2), 0: (1, 2), 3: (0, 3), 1: (1, 3)}
            down_final(nxt, st1, None, lambda a: a in unit and project_kv("k", xn, *unit[a]))
        jobs = []
        for u in range(4):
            for a in range(2):
                project_q(a, u, jobs)
        if first:
            for cp in cp_ffn(0) + cp_tails():
                cp.wait()
        jobs += [lambda v: fence(pb, v)]
        ln1 = [lambda v: fence(xr, v)] + paced(xr, ln1_fns(xnn, nxt, st1, range(4)), 2)
        jobs = spread(jobs, 36) + spread(ln1, 2 * MQ - 36)
        for vb in vbs:
            prime(vb, ob)
        prime(xf, a_ref)
        prime(xo, a_ref)
        for a in range(2):
            for u in range(4):
                project_kv("v", xn, a, u, jobs, 1 if a == 0 else 6)
            assert not jobs
            lo, hi = mix_jobs(a, order), mix_jobs(a + 2, order)
            jobs = [job for t in range(NT_) for job in lo[3 * t:3 * t + 3] + hi[3 * t:3 * t + 3]]
        for a in range(2):
            project_kv("k", xnn, a, 0, jobs, 6)
        jobs = spread(jobs, 72)
        st2 = {}
        for t, r in enumerate(order):
            if t > 0:
                ln2(st2, order[t - 1])
            if t == 0 and first:
                prep_l(0)
            if t == 4:
                assert not jobs
                jobs = spread(prep_a_jobs(G_ORDER, 0), 100) + prep_a_jobs((2,), 1)
            out_proj(cur, st2, r, jobs)
        assert not jobs
        ln2(st2, order[-1])
        last = []
        project_kv("k", xnn, 0, 1)
        project_kv("k", xnn, 1, 1, [last.append])
        for a in G_ORDER[1:]:
            for half in range(2):
                for g in range(4, 8):
                    chain(xo, last, prep_a(a, half, g))
        prep_a_tail()
        gate_up(0, (lambda a: prep_r(0, a)) if first else None)

    def ffn_loop(first):
        def body(c, carry):
            if first:
                for cp in cp_ffn(c + 1):
                    cp.wait()

                @pl.when(c + RING < NC)
                def _():
                    for cp in cp_ffn(c + RING):
                        cp.start()
            down(c)
            if first:
                prep_l(c + 1)

            gate_up(c + 1, (lambda a: prep_r(c + 1, a)) if first else None)
            return carry
        lax.fori_loop(0, NC - 1, body, 0)

    cp_qkv("k").start()
    for u in range(4):
        cp_x(u).start()
    for cp in (cp_qkv("q"), cp_qkv("v"), cp_wo()) + cp_ffn(0) + cp_tails() + cp_ffn(1) + cp_ffn(2):
        cp.start()
    cp_qkv("k").wait()
    setup_qkv("k")
    for u in range(4):
        cp_x(u).wait()
        for t in range(X_SPLIT[u], X_SPLIT[u + 1]):
            x_to_rows(t)

    attention_block(0, True)
    ffn_loop(True)

    def pass_body(p, carry):
        attention_block(p, False)
        ffn_loop(False)
        return carry
    lax.fori_loop(1, 4, pass_body, 0)

    for b in range(3):
        tiles_to_rows(b, 0, range(NT_))

    def after(quad):
        tiles = range(4 * (quad % 2), 4 * (quad % 2) + 4)
        slabs = ((0,), (2, 1))[quad // 2]
        for b in slabs:
            tiles_to_rows(b, 1, tiles)
        if quad in (0, 3):
            for b in slabs:
                rows_to_out(b)
    down_final(None, None, after)
    for b, u in [(b, u) for b in range(2) for u in range(4)] + [(2, 0)]:
        cp_out(b, u).wait()


@jax.jit
def pallas_interleave_layers__sliding_local_dilated__glu_gated_bilinear__prompt_kernel(
    A_x: jax.Array,
    A_wqkv: jax.Array,
    A_wo: jax.Array,
    B_x: jax.Array,
    B_w_gate: jax.Array,
    B_w_up: jax.Array,
    B_w_down: jax.Array,
):
    del B_x
    vm = pltpu.VMEM
    scratch = [
        vm((D, S), BF), vm((D, 3 * D), BF), vm((D, D), BF),
        vm((RING, 512, FC), BF), vm((RING, 512, FC), BF), vm((RING, D, FC), BF),
        vm((D - 512, F), BF), vm((D - 512, F), BF),
        vm((5, 640, 128), F32),
        vm((6, 8, MQ // 2, 256), U32),
        vm((D // 2, D), U32),
        vm((2 * NT_ + 1, D, 128), F32),
        vm((5, D, 128), F32),
        vm((5, D, 128), F32),
        vm((4, 960, 128), U32),
        vm((4, 960, 128), U32),
        vm((15, D, 128), F32),
        vm((16, MQ, 128), F32), vm((16, MQ, 128), F32), vm((16, MQ, 128), F32), vm((16, MQ, 128), F32),
        vm((NT_ + 1, W * H, 128), F32),
        vm((NT_, D // 2, 128), U32),
        vm((6, D, 128), F32),
        vm((6, S // 4, 128), F32),
        vm((49 * 128 + 32, 128), F32),
        vm((49, TQ // 2, 128), U32),
        vm((4, TQ // 2, 64), U32),
        vm((49, MQ, TQ), F32),
        vm((49, TQ // 2, 128), U32),
        vm((4, TQ, 256), F32),
        vm((16, TQ, 256), F32),
        vm((16, TQ, 128), F32),
        vm((NC, 49, 64, 256), U32),
        vm((NC, 3552, 128), U32),
        pltpu.SMEM((2,), jnp.int32),
        pltpu.SemaphoreType.DMA((11 + 3 * RING,)),
    ]
    hbm = pl.BlockSpec(memory_space=pl.ANY)
    out = pl.pallas_call(
        _kernel,
        in_specs=[hbm] * 6,
        out_specs=hbm,
        out_shape=jax.ShapeDtypeStruct((D, S), BF),
        scratch_shapes=scratch,
        compiler_params=pltpu.CompilerParams(vmem_limit_bytes=126 * 1024 * 1024),
    )(A_x.reshape(S, D).T, A_wqkv, A_wo, B_w_gate, B_w_up, B_w_down.T)
    return out.T.reshape(1, S, D)
```

```python
import math

import jax
import jax.numpy as jnp
from jax import lax
import jax.experimental.pallas as pl
import jax.experimental.pallas.tpu as pltpu

S, D, F = 2048, 576, 4608
H, DH, W = 32, 18, 8
NT_ = 8
TQ = 256
MQ = D // 4
FC = 512
NC = F // FC
RING = 3
X_SPLIT = (0, 5, 10, 14, 16)
EPS = 1e-5
SCALE = DH ** -0.5
EXP_C = SCALE * math.log2(math.e)
NEG = -1e9 / SCALE

BF, F32, U32 = jnp.bfloat16, jnp.float32, jnp.uint32
NT_DIMS = (((1,), (1,)), ((), ()))

LHS_SEL = {0: ((0, 0), 1, (1, 1)), 1: ((1, 0), 1, (1, 1)), 2: ((0, 0), 0, None), 3: ((1, 1), 0, None),
           4: ((0, 0), 1, (0, 1)), 5: ((1, 0), -1, (0, 0)), 6: ((0, 1), -1, (1, 1))}
RHS_SEL = {0: ((0, 0), 1, (1, 1)), 1: ((0, 0), 0, None), 2: ((0, 1), -1, (1, 1)), 3: ((1, 0), -1, (0, 0)),
           4: ((1, 1), 0, None), 5: ((0, 0), 1, (0, 1)), 6: ((1, 0), 1, (1, 1))}
G_ORDER = (2, 0, 1, 5, 3, 4, 6)


def _lhs1(a11, a12, a21, a22):
    return [a11 + a22, a21 + a22, a11, a22, a11 + a12, a21 - a11, a12 - a22]


def _rhs1(b11, b12, b21, b22):
    return [b11 + b22, b11, b12 - b22, b21 - b11, b22, b11 + b12, b21 + b22]


def _in2(fn, x):
    outer = [[fn(x[i][j], x[i][2 + j], x[2 + i][j], x[2 + i][2 + j]) for j in range(2)] for i in range(2)]
    return [v for a in range(7) for v in fn(outer[0][0][a], outer[0][1][a], outer[1][0][a], outer[1][1][a])]


def _select(sel, load):
    first, sign, second = sel
    v = load(first)
    if sign == 1:
        v = [a + b for a, b in zip(v, load(second))]
    elif sign == -1:
        v = [a - b for a, b in zip(v, load(second))]
    return v


def _pk(lo, hi):
    return pltpu.pack_elementwise([lo, hi], packed_dtype=BF)


def _lo(w):
    return pltpu.unpack_elementwise(w, index=0, packed_dtype=BF, unpacked_dtype=F32)


def _hi(w):
    return pltpu.unpack_elementwise(w, index=1, packed_dtype=BF, unpacked_dtype=F32)


def _bf(w):
    return pltpu.bitcast(w, BF)


def _u32(x):
    return pltpu.bitcast(x.astype(BF), U32)


def _dot(a, b):
    return jnp.dot(a, b, preferred_element_type=F32)


def _kernel(x_hbm, wqkv_hbm, wo_hbm, wg_hbm, wu_hbm, wd_hbm, out_hbm,
            xio, wqkv_raw, wo_raw, wg_raw, wu_raw, wd_raw, tg, tu,
            wts, wqkv_t, wo_t, xr, xm0, xm1, xn, kb, vb0, vb1, vb2, vb3, pb, ob, xf, xo, perm,
            a_ref, at_ref, acc, h_ref, ti, to, hf, r_ref, l_ref, zero_ref, sems):
    def clear(i, carry):
        zero_ref[i] = 0
        return carry
    lax.fori_loop(0, 2, clear, 0)
    z = zero_ref[0]
    z2 = zero_ref[1]
    vbs = (vb0, vb1, vb2, vb3)
    xm = [((xm0, xm1)[r // 2 % 2], r // 4 * 2 + r % 2) for r in range(NT_)]

    def fence(ref, v):
        ref[z + (ref.shape[0] - 1), 0:8, 0:128] = v

    def gate(ref, fn):
        def job(v):
            if len(ref.shape) == 3:
                fence(ref, v)
            else:
                rows = pl.ds(pl.multiple_of(16 * z + (ref.shape[0] - 16), 16), 16)
                ref[rows, 0:128] = jnp.concatenate([v, v], axis=0).astype(ref.dtype)
            fn()
        return job

    def prime(ref, other):
        ref[z2 + (ref.shape[0] - 1), 0:8, 0:128] = pltpu.bitcast(other[z, 0:8, 0:128], F32)

    def paced(ref, fns, skew):
        last = []

        def job(v, fn):
            last.append(fn())
            if len(last) > skew:
                v = pltpu.bitcast(last.pop(0) ^ pltpu.bitcast(v, U32), F32)
            fence(ref, v)
        return [lambda v, fn=fn: job(v, fn) for fn in fns]

    def spread(jobs, n):
        slots = [lambda v: None] * n
        for i, job in enumerate(jobs):
            slots[i * n // len(jobs)] = job
        return slots

    def run(jobs, v, n=1):
        for _ in range(n):
            if jobs:
                jobs.pop(0)(v)

    def tree(fn, v):
        while len(v) > 1:
            v = [fn(v[i], v[i + 1]) for i in range(0, len(v), 2)]
        return v[0]

    def cp_x(u):
        cols = pl.ds(128 * X_SPLIT[u], 128 * (X_SPLIT[u + 1] - X_SPLIT[u]))
        return pltpu.make_async_copy(x_hbm.at[:, cols], xio.at[:, cols], sems.at[u])

    def cp_out(b, u):
        rows, cols = (pl.ds(256 * b, 256), pl.ds(512 * u, 512)) if b < 2 else (pl.ds(512, 64), pl.ds(0, S))
        return pltpu.make_async_copy(xio.at[rows, cols], out_hbm.at[rows, cols], sems.at[4 * b + u])

    qkv_cols = {"k": pl.ds(512, 640), "v": pl.ds(1152, 576), "q": pl.ds(0, 512)}

    def cp_qkv(name):
        idx = 5 + "kvq".index(name)
        return pltpu.make_async_copy(wqkv_hbm.at[:, qkv_cols[name]], wqkv_raw.at[0:D, qkv_cols[name]], sems.at[idx])

    def cp_wo():
        return pltpu.make_async_copy(wo_hbm, wo_raw.at[0:D], sems.at[8])

    def cp_ffn(c):
        c0 = c * FC if isinstance(c, int) else pl.multiple_of(c * FC, FC)
        cols = pl.ds(c0, FC)
        slot = c % RING
        return (pltpu.make_async_copy(wg_hbm.at[0:512, cols], wg_raw.at[slot], sems.at[11 + 3 * slot]),
                pltpu.make_async_copy(wu_hbm.at[0:512, cols], wu_raw.at[slot], sems.at[12 + 3 * slot]),
                pltpu.make_async_copy(wd_hbm.at[:, cols], wd_raw.at[slot], sems.at[13 + 3 * slot]))

    def cp_tails():
        return (pltpu.make_async_copy(wg_hbm.at[512:D, :], tg, sems.at[9]),
                pltpu.make_async_copy(wu_hbm.at[512:D, :], tu, sems.at[10]))

    def setup_qkv(name):
        part = "qkv".index(name)
        nb0 = (D * part) // 128
        base = D * part - 128 * nb0

        def transpose(nb):
            wn = min(128, D * part + D - 128 * nb)
            for kt in range(5):
                wk = 128 if kt < 4 else 64
                blk = wqkv_raw[128 * kt:128 * kt + wk, 128 * nb:128 * nb + wn].astype(F32)
                wts[kt, 128 * (nb - nb0):128 * (nb - nb0) + wn, 0:wk] = blk.T

        def rows(hg, kt, d):
            return jnp.concatenate([wts[kt, pl.ds(base + MQ * hg + d + e, 8, stride=DH), :] for e in range(2)], axis=0)

        def combine(a, d):
            for j in range(2):
                w = _lhs1(rows(a, j, d), rows(a, 2 + j, d), rows(a + 2, j, d), rows(a + 2, 2 + j, d))
                for b in range(7):
                    wqkv_t[2 * part + a, b, 4 * d:4 * d + 8, 128 * j:128 * j + 128] = _u32(w[b])
                wqkv_t[2 * part + a, 7, 4 * d:4 * d + 8, 128 * j:128 * j + 64] = _u32(rows(a + 2 * j, 4, d)[:, :64])
        return ([(wqkv_raw, lambda nb=nb: transpose(nb)) for nb in range(nb0, nb0 + 5)]
                + [(wts, lambda a=a, d=d: combine(a, d)) for a in range(2) for d in range(0, DH, 2)])

    def setup_wo(nb):
        wn = 128 if nb < 4 else 64
        xf[nb, 0:D, 0:wn] = wo_raw[0:D, 128 * nb:128 * nb + wn].astype(F32)
        rows = []
        for hg in range(4):
            for d in range(0, DH, 2):
                lo = xf[nb, pl.ds(MQ * hg + d, 8, stride=DH), :][:, :wn]
                hi = xf[nb, pl.ds(MQ * hg + d + 1, 8, stride=DH), :][:, :wn]
                rows.append(_pk(lo, hi))
        for kt in range(5):
            blk = _bf(jnp.concatenate(rows[8 * kt:8 * kt + 8], axis=0)).astype(F32).T
            wo_t[64 * nb:64 * nb + wn // 2, pl.ds(128 * kt, blk.shape[1])] = _u32(blk)

    def x_to_rows(t):
        x = xio[:, 128 * t:128 * t + 128]
        st, xs = {}, x.astype(F32)
        for g in range(D // 8):
            add_stats(st, g % 2, xs[8 * g:8 * g + 8])
        m, rs = mean_rstd({0: (st[0][0] + st[1][0], st[0][1] + st[1][1])}, 0)
        stat = jnp.where(lax.broadcasted_iota(jnp.int32, (32, 128), 0) == 0, m, rs)
        words = pltpu.bitcast(x, F32)
        for b in range(3):
            if b < 2:
                w = words[128 * b:128 * b + 128].T
            else:
                w = jnp.concatenate([words[256:288], stat], axis=0).T
                w = jnp.concatenate([w, jnp.zeros((128, 64), F32)], axis=1)
            for jj in range(8):
                perm[pl.ds(49 * (8 * t + jj) + b, 16, stride=3), :] = w[16 * jj:16 * jj + 16]

    def rows_to_tile(s, r, mr, slabs=range(3)):
        for b in slabs:
            w = perm[pl.ds(3 * (2 * r + s) + b, 128, stride=49), :]
            if b < 2:
                xr[8 * s + r, 256 * b:256 * b + 256, :] = _bf(w.T).astype(F32)
            else:
                w = w[:, :64].T
                xr[8 * s + r, 512:D, :] = _bf(w[0:32]).astype(F32)
                mr[r] = (w[32:33], w[33:34])

    def tiles_to_rows(b, s, tiles):
        nw = 128 if b < 2 else 32
        for r in tiles:
            if s == 0:
                w = _pk(xr[r, pl.ds(256 * b, nw, stride=2), :], xr[r, pl.ds(256 * b + 1, nw, stride=2), :])
            else:
                w = ob[z + r, 128 * b:128 * b + nw, :]
            w = jnp.concatenate([pltpu.bitcast(w, F32)] * (128 // nw), axis=0)
            perm[pl.ds(3 * (2 * r + s) + b, 128, stride=49), :] = w.T

    def rows_to_out(b):
        def rows(t):
            return jnp.concatenate([perm[pl.ds(49 * (8 * t + jj) + b, 16, stride=3), :] for jj in range(8)], axis=0)
        group = lax.broadcasted_iota(jnp.int32, (128, 128), 1) // 32
        for u in range(4):
            if b < 2:
                for t in range(4 * u, 4 * u + 4):
                    xio[256 * b:256 * b + 256, 128 * t:128 * t + 128] = _bf(rows(t).T)
                cp_out(b, u).start()
            else:
                w = rows(4 * u)
                for t in range(1, 4):
                    w = jnp.where(group == t, rows(4 * u + t), w)
                w = _bf(w.T)
                for t in range(4):
                    xio[512:D, pl.ds(128 * (4 * u + t), 128)] = w[64 * t:64 * t + 64]
        if b == 2:
            cp_out(b, 0).start()

    def prep_r(c, a):
        slot = c % RING
        for u in range(2):
            for g in range(8):
                def load(quad):
                    ws = [pltpu.bitcast((wg_raw, wu_raw)[u][slot, pl.ds(128 * (2 * quad[0] + i) + 16 * g, 16),
                                                            pl.ds(256 * quad[1], 256)], U32) for i in range(2)]
                    ws = [w[:, 128 * j:128 * j + 128] for w in ws for j in range(2)]
                    return [_lo(w) for w in ws] + [_hi(w) for w in ws]
                v = _select(RHS_SEL[a], load)
                for b, (lo, hi) in enumerate(zip(_rhs1(*v[:4]), _rhs1(*v[4:]))):
                    r_ref[c, 7 * a + b, 8 * g:8 * g + 8, 128 * u:128 * u + 128] = _pk(lo, hi)

    def prep_l(c):
        slot = c % RING
        for g in range(MQ // 16):
            ws = [pltpu.bitcast(wd_raw[slot, pl.ds(MQ * i + 16 * g, 16), :], U32) for i in range(4)]
            ws = [[w[:, 128 * j:128 * j + 128] for j in range(4)] for w in ws]
            lo = _in2(_lhs1, [[_lo(w) for w in row] for row in ws])
            hi = _in2(_lhs1, [[_hi(w) for w in row] for row in ws])
            for k in range(49):
                l_ref[c, pl.ds(72 * k + 8 * g, 8), :] = _pk(lo[k], hi[k])

    def prep_a(a, half, g):
        src, row = (xf, xo)[g // 4], 32 * (g % 4) + half

        def load(quad):
            return [src[z2 + 2 * quad[1] + j, pl.ds(128 * (2 * quad[0] + i) + row + e, 8, stride=4), :]
                    for e in (0, 2) for i in range(2) for j in range(2)]
        v = _select(LHS_SEL[a], load)
        o = [_pk(lo, hi) for lo, hi in zip(_lhs1(*v[:4]), _lhs1(*v[4:]))]
        for b in range(7):
            a_ref[z + 7 * a + b, 64 * half + 8 * g:64 * half + 8 * g + 8, :] = o[b]
        return o[5] ^ o[6]

    def prep_a_tail():
        for i in range(4):
            for half in range(2):
                for u, src in enumerate((xf, xo)):
                    lo = src[z + 4, pl.ds(128 * i + half, 32, stride=4), :][:, :64]
                    hi = src[z + 4, pl.ds(128 * i + half + 2, 32, stride=4), :][:, :64]
                    at_ref[z + i, pl.ds(64 * half + 32 * u, 32), :] = _pk(lo, hi)

    def put(a):
        for g in range(16):
            def load(quad):
                return [hf[z + 4 * (2 * quad[1] + quad[0]) + t, pl.ds(o + 8 * g, 8), :]
                        for o in (0, 128) for t in (0, 2, 1, 3)]
            v = _select(RHS_SEL[a], load)
            for b, (lo, hi) in enumerate(zip(_rhs1(*v[:4]), _rhs1(*v[4:]))):
                h_ref[7 * a + b, 8 * g:8 * g + 8, :] = _pk(lo, hi)

    def strassen_inner(prod, nrow, emit, odd=None):
        ld = lambda s: ti[z + s, 0:nrow, :]
        for s in range(3):
            ti[z + s, 0:nrow, :] = prod(s)
        if not odd:
            emit(3, ((ld(0) - ld(1)) + ld(2)) + prod(5))
        m3 = prod(3)
        emit(2, ld(1) + m3)
        if odd is None:
            ti[z + 3, 0:nrow, :] = ld(0) + m3
        m4 = prod(4)
        emit(1, ld(2) + m4)
        ti[z + 3, 0:nrow, :] = (ld(3) if odd is None else ld(0) + m3) - m4
        if odd:
            emit(3, ((ld(0) - ld(1)) + ld(2)) + prod(5))
        emit(0, ld(3) + prod(6))

    def gate_up(c, before=None):
        c0 = c * FC if isinstance(c, int) else pl.multiple_of(c * FC, FC)

        def inner(a, emit):
            if before is not None:
                before(a)
            strassen_inner(lambda b: _dot(_bf(a_ref[z + 7 * a + b]), _bf(r_ref[c, 7 * a + b])), TQ, emit)

        def fin(quad, q, v):
            i, j = 2 * (quad // 2) + q // 2, 2 * (quad % 2) + q % 2
            cols = pl.ds(c0 + 128 * j, 128)
            wt = jnp.concatenate([tg[:, cols], tu[:, cols]], axis=1)
            v = v + _dot(_bf(at_ref[z + i]), wt)
            hf[z + 4 * quad + q] = v[:, :128] * v[:, 128:]

        def old(s, q):
            return to[z + 4 * s + q]

        def keep(s):
            def emit(q, v):
                to[z + 4 * s + q] = v
            return emit

        def emit3(q, v):
            fin(2, q, old(1, q) + v)
            to[z + 12 + q] = old(0, q) + v

        def emit4(q, v):
            fin(1, q, old(2, q) + v)
            to[z + 12 + q] = old(3, q) - v

        inner(2, keep(2))
        inner(0, keep(0))
        inner(1, keep(1))
        inner(5, lambda q, v: fin(3, q, ((old(0, q) - old(1, q)) + old(2, q)) + v))
        put(4)
        inner(3, emit3)
        put(2)
        inner(4, emit4)
        put(6)
        inner(6, lambda q, v: fin(0, q, old(3, q) + v))

    def down_prod(c, k, prev):
        return prev + lax.dot_general(_bf(l_ref[c, 72 * k:72 * k + 72, :]), _bf(h_ref[k]), NT_DIMS, preferred_element_type=F32)

    def down(c):
        for a, late in ((4, 1), (2, 0), (6, 3), (1, 5), (0, None), (3, None), (5, None)):
            for k in range(7 * a, 7 * a + 7):
                acc[k] = down_prod(c, k, jnp.where(c == 0, 0.0, acc[k]))
            if late is not None:
                put(late)

    def add_stats(st, r, x):
        st[r] = (x, x * x) if st.get(r) is None else (st[r][0] + x, st[r][1] + x * x)

    def mean_rstd(st, r):
        m = jnp.sum(st[r][0], axis=0, keepdims=True) * (1.0 / D)
        v = jnp.sum(st[r][1], axis=0, keepdims=True) * (1.0 / D) - m * m
        return m, lax.rsqrt(jnp.maximum(v, 0.0) + EPS)

    def down_final(base, st, after=None, between=()):
        odd = [False]

        def inner(a, emit, late=None):
            strassen_inner(lambda b: down_prod(NC - 1, 7 * a + b, acc[7 * a + b]), MQ, emit, odd[0])
            if late is not None:
                put(late)
            if a in between:
                between[a]()
            else:
                odd[0] = not odd[0]

        def old(s, q):
            return to[z + 4 * s + q, 0:MQ, :]

        def keep(s, q, v):
            to[z + 4 * s + q, 0:MQ, :] = v

        def fin(quad, q, v):
            i, j = 2 * (quad // 2) + q // 2, 2 * (quad % 2) + q % 2
            rows = pl.ds(MQ * i, MQ)
            for e in range(2):
                ref, slot = xm[2 * j + e]
                x = ref[z + slot, rows, :] + v[:, 128 * e:128 * e + 128]
                if st is None:
                    ob[z + 2 * j + e, 72 * i:72 * i + 72, :] = pltpu.bitcast(x.astype(BF), U32)
                    continue
                xr[base + 2 * j + e, rows, :] = x
                for g in range(MQ // 8):
                    add_stats(st, 2 * j + e, x[8 * g:8 * g + 8])
            if after is not None and q == 0:
                after(quad)

        inner(4, lambda q, v: keep(0, q, v), 0)
        inner(2, lambda q, v: (fin(1, q, old(0, q) + v), keep(1, q, v)), 3)
        inner(6, lambda q, v: keep(0, q, v - old(0, q)), 1)
        inner(0, lambda q, v: (keep(0, q, old(0, q) + v), keep(1, q, old(1, q) + v)), 5)
        inner(3, lambda q, v: (fin(0, q, old(0, q) + v), keep(2, q, v)))
        inner(1, lambda q, v: (fin(2, q, old(2, q) + v), keep(1, q, old(1, q) - v)))
        inner(5, lambda q, v: fin(3, q, old(1, q) + v))

    def chain(ref, last, v, skew=1):
        last.append(pltpu.bitcast(v, F32))
        if len(last) > skew:
            fence(ref, last.pop(0))

    def ln1_fns(base, mr, pairs):
        def norm(r, row, n):
            return (xr[base + r, pl.ds(row, n), :] - mr[r][0]) * mr[r][1]

        def job(u, g):
            if g == 16:
                y = jnp.concatenate([_u32(norm(2 * u + e, 512, 64)) for e in range(2)], axis=0)
                xn[u, 896:960, :] = y
                return tree(jnp.bitwise_xor, [y[8 * k:8 * k + 8] for k in range(8)])
            y = [_u32(v) for v in _rhs1(*[norm(2 * u + e, 256 * k + 16 * g, 16) for k in range(2) for e in range(2)])]
            for b in range(7):
                xn[u, pl.ds(128 * b + 8 * g, 8), :] = y[b]
            return y[5] ^ y[6]
        return [lambda u=u, g=g: job(u, g) for u in pairs for g in range(17)]

    def project(name, a, u, emit, x=None):
        w = 2 * "qkv".index(name) + a
        rows = lambda i, n: xn[u, i:i + n, :] if x is None else x[i:i + n]
        m = lambda b: _dot(_bf(wqkv_t[w, b]), _bf(rows(128 * b, 128)))
        xt = lambda: _bf(jnp.concatenate([rows(896, 32), rows(928, 32)], axis=1))
        tail = lambda i: _dot(_bf(wqkv_t[w, 7, :, 128 * i:128 * i + 64]), xt())
        ta, m4 = tail(0), m(4)
        s11, s12 = ta[:, :128] - m4, ta[:, 128:] + m4
        s22 = m(2)
        emit(a, 2 * u + 1, s12 + s22)
        s11 = s11 + m(6)
        m0 = m(0)
        s11, s22 = s11 + m0, s22 + m0
        s21 = m(3)
        emit(a, 2 * u, s11 + s21)
        tb = tail(1)
        s21, s22 = s21 + tb[:, :128], s22 + tb[:, 128:]
        m1 = m(1)
        emit(a + 2, 2 * u, s21 + m1)
        emit(a + 2, 2 * u + 1, (s22 - m1) + m(5))

    def project_kv(name, a, u, jobs=(), every=1, x=None):
        def emit(hg, r, y):
            dst, rows = (kb, pl.ds(MQ * hg, MQ)) if name == "k" else (vbs[hg], pl.ds(0, MQ))
            dst[z + 7 + r, rows, :] = y
            if r >= 1:
                dst[z + r - 1, rows, :] = pltpu.roll(y, 1, 1)
            for g in range(0, DH, every):
                run(jobs, y[8 * g:8 * g + 8])
        project(name, a, u, emit, x)

    def prow(hg, w):
        return pl.ds(32 * w + 16 * (hg % 2) + 8 * (hg // 2), 8)

    def project_q(a, u, jobs, extra):
        def emit(hg, r, y):
            lg = [None] * W
            for d in range(DH):
                q = y[8 * d:8 * d + 8]
                for w in range(W):
                    v = q * kb[z + 7 + r - w, pl.ds(MQ * hg + 8 * d, 8), :]
                    lg[w] = v if d == 0 else lg[w] + v
                run(extra, q)
            for w in range(W):
                pb[z + r, prow(hg, w), :] = lg[w]
            if hg >= 2:
                jobs.append(softmax_job(r, a))
        project("q", a, u, emit)

    def softmax_job(r, sl):
        def job(v):
            fence(pb, v)
            lane0 = lax.broadcasted_iota(jnp.int32, (16, 128), 1) == 0
            lg = [pb[z2 + r, 32 * w + 16 * sl:32 * w + 16 * sl + 16, :] for w in range(W)]
            lg = [jnp.where(lane0, NEG, lg[w]) if w > r else lg[w] for w in range(W)]
            m = tree(jnp.maximum, lg)
            ex = [jnp.exp2((lg[w] - m) * EXP_C) for w in range(W)]
            inv = 1.0 / tree(jnp.add, ex)
            for w in range(W):
                pb[z2 + r, 32 * w + 16 * sl:32 * w + 16 * sl + 16, :] = ex[w] * inv
        return job

    def mix_jobs(hg, tiles):
        vb = vbs[hg]

        def job(r, d0):
            p = [pb[z2 + r, prow(hg, w), :] for w in range(W)]
            o = [tree(jnp.add, [p[w] * vb[z2 + 7 + r - w, pl.ds(8 * d, 8), :] for w in range(W)])
                 for d in range(d0, d0 + 6)]
            o = [_pk(o[e], o[e + 1]) for e in range(0, 6, 2)]
            ob[z + r, 72 * hg + 4 * d0:72 * hg + 4 * d0 + 24, :] = jnp.concatenate(o, axis=0)
            return o[0] ^ o[1] ^ o[2]
        return paced(vb, [lambda r=r, d0=d0: job(r, d0) for r in tiles for d0 in range(0, DH, 6)], 1)

    def ln2(st, r):
        m, rs = mean_rstd(st, r)
        (ref, slot), last = xm[r], []
        for kt in range(5):
            wk = 128 if kt < 4 else 64
            y = ((ref[z2 + slot, 128 * kt:128 * kt + wk, :] - m) * rs).T
            (xf, xo)[r % 2][z + kt, pl.ds(128 * (r // 2), 128), 0:wk] = y
            if kt < 4:
                chain(ref, last, y[0:8], 2)

    def prep_a_jobs(outer, odd):
        return paced((xf, xo)[odd], [lambda a=a, half=half, g=g: prep_a(a, half, g) for a in outer
                                     for half in range(2) for g in range(4 * odd, 4 * odd + 4)], 2)

    def out_proj(base, st, r, jobs):
        y = _dot(_bf(wo_t[...]), _bf(ob[z + r]))
        for g in range(D // 16):
            rows = pl.ds(16 * g, 16)
            x = xr[base + r, rows, :] + y[16 * g:16 * g + 16]
            xm[r][0][z + xm[r][1], rows, :] = x
            add_stats(st, r, x[0:8])
            add_stats(st, r, x[8:16])
            run(jobs, x[0:8])

    def attention_block(p, first):
        s = 0 if first else p % 2
        cur, nxt = 8 * s, 8 * (1 - s)
        order = (0, 2, 4, 6, 1, 3, 5, 7)
        st1 = {}
        if first:
            st0 = {}
            for r in range(NT_):
                rows_to_tile(0, r, st0)
            for fn in ln1_fns(0, st0, (0, 1)):
                fn()
            project_kv("k", 0, 0)
            jobs = spread([lambda v: fence(xr, v)] + paced(xr, ln1_fns(z2, st0, (2, 3)), 2), 180)
            for a, u in ((1, 0), (0, 1), (1, 1)):
                project_kv("k", a, u, jobs)
            cp_qkv("q").wait()
            cp_qkv("v").wait()
            cp_wo().wait()
            steps = setup_qkv("q")
            for _, fn in steps[:5]:
                fn()
            project_kv("k", 0, 2)
            jobs = spread([gate(*step) for step in steps[5:]], 216)
            jobs[6:6 + 40 * 5:40] = [gate(wo_raw, lambda nb=nb: setup_wo(nb)) for nb in range(5)]
            for a, u in ((1, 2), (0, 3), (1, 3)):
                project_kv("k", a, u, jobs)
            extra = [gate(perm, lambda r=r, b=b: rows_to_tile(1, r, st1, (b,))) for r in range(NT_) for b in range(3)]
            steps = [gate(*step) for step in setup_qkv("v")]
            extra = steps[:5] + extra[:6] + [job for pair in zip(steps[5:], extra[6:]) for job in pair]
            extra = spread(extra, 500)
        else:
            extra = []
            unit = {2: (0, 2), 0: (1, 2), 3: (0, 3), 1: (1, 3)}
            down_final(nxt, st1, None, {g: lambda g=g: project_kv("k", *unit[g]) for g in unit})
            st1 = {r: mean_rstd(st1, r) for r in range(NT_)}
        jobs = []
        for u in range(4):
            for a in range(2):
                project_q(a, u, jobs, extra)
        if first:
            for cp in cp_ffn(0) + cp_tails():
                cp.wait()
        jobs = spread(jobs + [lambda v: fence(pb, v)], 272)
        ln1 = [lambda v: fence(xr, v)] + paced(xr, ln1_fns(z2 + nxt, st1, range(4)), 2)
        for vb in vbs:
            prime(vb, ob)
        prime(xf, a_ref)
        prime(xo, a_ref)

        def mix_pair(a):
            lo, hi = mix_jobs(a, order), mix_jobs(a + 2, order)
            return [job for t in range(NT_) for job in lo[3 * t:3 * t + 3] + hi[3 * t:3 * t + 3]]
        x0 = xn[0]
        jobs[75:75 + 10 * 18:10] = ln1[:18]
        for u in range(4):
            project_kv("v", 0, u, jobs)
        assert not jobs
        jobs = mix_pair(0)
        for u in range(4):
            project_kv("v", 1, u, jobs, 6, x0 if u == 0 else None)
        assert not jobs
        jobs = mix_pair(1)
        for a in range(2):
            project_kv("k", a, 0, jobs, 6)
        jobs = spread(jobs, 72) + spread(ln1[18:52], 72)
        st2 = {}
        for t, r in enumerate(order):
            if t > 0:
                ln2(st2, order[t - 1])
            if t == 0 and first:
                prep_l(0)
            if t == 4:
                assert not jobs
                jobs = spread(prep_a_jobs(G_ORDER, 0), 100) + prep_a_jobs((2,), 1) + spread(ln1[52:], 36)
            out_proj(cur, st2, r, jobs)
        assert not jobs
        ln2(st2, order[-1])
        last = []
        project_kv("k", 0, 1)
        project_kv("k", 1, 1, [last.append])
        for a in G_ORDER[1:]:
            for half in range(2):
                for g in range(4, 8):
                    chain(xo, last, prep_a(a, half, g))
        prep_a_tail()
        gate_up(0, (lambda a: prep_r(0, a)) if first else None)

    def ffn_loop(first):
        def body(c, carry):
            if first:
                for cp in cp_ffn(c + 1):
                    cp.wait()

                @pl.when(c + RING < NC)
                def _():
                    for cp in cp_ffn(c + RING):
                        cp.start()
            down(c)
            if first:
                prep_l(c + 1)

            gate_up(c + 1, (lambda a: prep_r(c + 1, a)) if first else None)
            return carry
        lax.fori_loop(0, NC - 1, body, 0)

    cp_qkv("k").start()
    for u in range(4):
        cp_x(u).start()
    for cp in (cp_qkv("q"), cp_qkv("v"), cp_wo()) + cp_ffn(0) + cp_tails() + cp_ffn(1) + cp_ffn(2):
        cp.start()
    cp_qkv("k").wait()
    for _, fn in setup_qkv("k"):
        fn()
    for u in range(4):
        cp_x(u).wait()
        for t in range(X_SPLIT[u], X_SPLIT[u + 1]):
            x_to_rows(t)

    attention_block(0, True)
    ffn_loop(True)

    def pass_body(p, carry):
        attention_block(p, False)
        ffn_loop(False)
        return carry
    lax.fori_loop(1, 4, pass_body, 0)

    for b in range(3):
        tiles_to_rows(b, 0, range(NT_))

    def after(quad):
        tiles = range(4 * (quad % 2), 4 * (quad % 2) + 4)
        slabs = ((0,), (2, 1))[quad // 2]
        for b in slabs:
            tiles_to_rows(b, 1, tiles)
        if quad in (0, 3):
            for b in slabs:
                rows_to_out(b)
    down_final(None, None, after)
    for b, u in [(b, u) for b in range(2) for u in range(4)] + [(2, 0)]:
        cp_out(b, u).wait()


@jax.jit
def pallas_interleave_layers__sliding_local_dilated__glu_gated_bilinear__prompt_kernel(
    A_x: jax.Array,
    A_wqkv: jax.Array,
    A_wo: jax.Array,
    B_x: jax.Array,
    B_w_gate: jax.Array,
    B_w_up: jax.Array,
    B_w_down: jax.Array,
):
    del B_x
    vm = pltpu.VMEM
    scratch = [
        vm((D, S), BF), vm((D + 32, 3 * D), BF), vm((D + 64, D), BF),
        vm((RING, 512, FC), BF), vm((RING, 512, FC), BF), vm((RING, D, FC), BF),
        vm((D - 512, F), BF), vm((D - 512, F), BF),
        vm((6, 640, 128), F32),
        vm((6, 8, MQ // 2, 256), U32),
        vm((D // 2, D), U32),
        vm((2 * NT_ + 1, D, 128), F32),
        vm((5, D, 128), F32),
        vm((5, D, 128), F32),
        vm((4, 960, 128), U32),
        vm((15, D, 128), F32),
        vm((16, MQ, 128), F32), vm((16, MQ, 128), F32), vm((16, MQ, 128), F32), vm((16, MQ, 128), F32),
        vm((NT_ + 1, W * H, 128), F32),
        vm((NT_, D // 2, 128), U32),
        vm((6, D, 128), F32),
        vm((6, S // 4, 128), F32),
        vm((49 * 128 + 32, 128), F32),
        vm((49, TQ // 2, 128), U32),
        vm((4, TQ // 2, 64), U32),
        vm((49, MQ, TQ), F32),
        vm((49, TQ // 2, 128), U32),
        vm((4, TQ, 256), F32),
        vm((16, TQ, 256), F32),
        vm((16, TQ, 128), F32),
        vm((NC, 49, 64, 256), U32),
        vm((NC, 3552, 128), U32),
        pltpu.SMEM((2,), jnp.int32),
        pltpu.SemaphoreType.DMA((11 + 3 * RING,)),
    ]
    hbm = pl.BlockSpec(memory_space=pl.ANY)
    out = pl.pallas_call(
        _kernel,
        in_specs=[hbm] * 6,
        out_specs=hbm,
        out_shape=jax.ShapeDtypeStruct((D, S), BF),
        scratch_shapes=scratch,
        compiler_params=pltpu.CompilerParams(vmem_limit_bytes=126 * 1024 * 1024),
    )(A_x.reshape(S, D).T, A_wqkv, A_wo, B_w_gate, B_w_up, B_w_down.T)
    return out.T.reshape(1, S, D)
```

```python
import math

import jax
import jax.numpy as jnp
from jax import lax
import jax.experimental.pallas as pl
import jax.experimental.pallas.tpu as pltpu

S, D, F = 2048, 576, 4608
H, DH, W = 32, 18, 8
NT_ = 8
TQ = 256
MQ = D // 4
FC = 512
NC = F // FC
RING = 3
X_SPLIT = (0, 5, 10, 14, 16)
EPS = 1e-5
SCALE = DH ** -0.5
EXP_C = SCALE * math.log2(math.e)
NEG = -1e9 / SCALE

BF, F32, U32 = jnp.bfloat16, jnp.float32, jnp.uint32
NT_DIMS = (((1,), (1,)), ((), ()))

LHS_SEL = {0: ((0, 0), 1, (1, 1)), 1: ((1, 0), 1, (1, 1)), 2: ((0, 0), 0, None), 3: ((1, 1), 0, None),
           4: ((0, 0), 1, (0, 1)), 5: ((1, 0), -1, (0, 0)), 6: ((0, 1), -1, (1, 1))}
RHS_SEL = {0: ((0, 0), 1, (1, 1)), 1: ((0, 0), 0, None), 2: ((0, 1), -1, (1, 1)), 3: ((1, 0), -1, (0, 0)),
           4: ((1, 1), 0, None), 5: ((0, 0), 1, (0, 1)), 6: ((1, 0), 1, (1, 1))}
G_ORDER = (2, 0, 1, 5, 3, 4, 6)


def _lhs1(a11, a12, a21, a22):
    return [a11 + a22, a21 + a22, a11, a22, a11 + a12, a21 - a11, a12 - a22]


def _rhs1(b11, b12, b21, b22):
    return [b11 + b22, b11, b12 - b22, b21 - b11, b22, b11 + b12, b21 + b22]


def _in2(fn, x):
    outer = [[fn(x[i][j], x[i][2 + j], x[2 + i][j], x[2 + i][2 + j]) for j in range(2)] for i in range(2)]
    return [v for a in range(7) for v in fn(outer[0][0][a], outer[0][1][a], outer[1][0][a], outer[1][1][a])]


def _select(sel, load):
    first, sign, second = sel
    v = load(first)
    if sign == 1:
        v = [a + b for a, b in zip(v, load(second))]
    elif sign == -1:
        v = [a - b for a, b in zip(v, load(second))]
    return v


def _pk(lo, hi):
    return pltpu.pack_elementwise([lo, hi], packed_dtype=BF)


def _lo(w):
    return pltpu.unpack_elementwise(w, index=0, packed_dtype=BF, unpacked_dtype=F32)


def _hi(w):
    return pltpu.unpack_elementwise(w, index=1, packed_dtype=BF, unpacked_dtype=F32)


def _bf(w):
    return pltpu.bitcast(w, BF)


def _u32(x):
    return pltpu.bitcast(x.astype(BF), U32)


def _dot(a, b):
    return jnp.dot(a, b, preferred_element_type=F32)


def _kernel(x_hbm, wqkv_hbm, wo_hbm, wg_hbm, wu_hbm, wd_hbm, out_hbm,
            xio, wqkv_raw, wo_raw, wg_raw, wu_raw, wd_raw, tg, tu,
            wts, wt, xr, xm0, xm1, xn, kb, vb0, vb1, pb, ob, xf, xo, perm,
            a_ref, at_ref, acc, h_ref, ti, to, hf, r_ref, l_ref, zero_ref, sems):
    def clear(i, carry):
        zero_ref[i] = 0
        return carry
    lax.fori_loop(0, 2, clear, 0)
    z = zero_ref[0]
    z2 = zero_ref[1]
    vbs = (vb0, vb1)
    xm = [((xm0, xm1)[r // 2 % 2], r // 4 * 2 + r % 2) for r in range(NT_)]

    def fence(ref, v):
        ref[z + (ref.shape[0] - 1), 0:8, 0:128] = v

    def gate(ref, fn):
        def job(v):
            if len(ref.shape) == 3:
                fence(ref, v)
            else:
                rows = pl.ds(pl.multiple_of(16 * z + (ref.shape[0] - 16), 16), 16)
                ref[rows, 0:128] = jnp.concatenate([v, v], axis=0).astype(ref.dtype)
            fn()
        return job

    def prime(ref, other):
        ref[z2 + (ref.shape[0] - 1), 0:8, 0:128] = pltpu.bitcast(other[z, 0:8, 0:128], F32)

    def paced(ref, fns, skew):
        last = []

        def job(v, fn):
            last.append(fn())
            if len(last) > skew:
                v = pltpu.bitcast(last.pop(0) ^ pltpu.bitcast(v, U32), F32)
            fence(ref, v)
        return [lambda v, fn=fn: job(v, fn) for fn in fns]

    def spread(jobs, n):
        slots = [lambda v: None] * n
        for i, job in enumerate(jobs):
            slots[i * n // len(jobs)] = job
        return slots

    def run(jobs, v, n=1):
        for _ in range(n):
            if jobs:
                jobs.pop(0)(v)

    def tree(fn, v):
        while len(v) > 1:
            v = [fn(v[i], v[i + 1]) for i in range(0, len(v), 2)]
        return v[0]

    def cp_x(u):
        cols = pl.ds(128 * X_SPLIT[u], 128 * (X_SPLIT[u + 1] - X_SPLIT[u]))
        return pltpu.make_async_copy(x_hbm.at[:, cols], xio.at[:, cols], sems.at[u])

    def cp_out(b, u):
        rows, cols = (pl.ds(256 * b, 256), pl.ds(512 * u, 512)) if b < 2 else (pl.ds(512, 64), pl.ds(0, S))
        return pltpu.make_async_copy(xio.at[rows, cols], out_hbm.at[rows, cols], sems.at[4 * b + u])

    qkv_cols = {"k": pl.ds(512, 640), "v": pl.ds(1152, 576), "q": pl.ds(0, 512)}

    def cp_qkv(name):
        idx = 5 + "kvq".index(name)
        return pltpu.make_async_copy(wqkv_hbm.at[:, qkv_cols[name]], wqkv_raw.at[0:D, qkv_cols[name]], sems.at[idx])

    def cp_wo():
        return pltpu.make_async_copy(wo_hbm, wo_raw.at[0:D], sems.at[8])

    def cp_ffn(c):
        c0 = c * FC if isinstance(c, int) else pl.multiple_of(c * FC, FC)
        cols = pl.ds(c0, FC)
        slot = c % RING
        return (pltpu.make_async_copy(wg_hbm.at[0:512, cols], wg_raw.at[slot], sems.at[11 + 3 * slot]),
                pltpu.make_async_copy(wu_hbm.at[0:512, cols], wu_raw.at[slot], sems.at[12 + 3 * slot]),
                pltpu.make_async_copy(wd_hbm.at[:, cols], wd_raw.at[slot], sems.at[13 + 3 * slot]))

    def cp_tails():
        return (pltpu.make_async_copy(wg_hbm.at[512:D, :], tg, sems.at[9]),
                pltpu.make_async_copy(wu_hbm.at[512:D, :], tu, sems.at[10]))

    def combine_steps(part, ref, rows):
        def combine(a, g):
            for j in range(2):
                w = _lhs1(rows(a, j, g), rows(a, 2 + j, g), rows(a + 2, j, g), rows(a + 2, 2 + j, g))
                for b in range(7):
                    wt[2 * part + a, b, 8 * g:8 * g + 8, 128 * j:128 * j + 128] = _u32(w[b])
                wt[2 * part + a, 7, 8 * g:8 * g + 8, 128 * j:128 * j + 64] = _u32(rows(a + 2 * j, 4, g)[:, :64])
        return [(ref, lambda a=a, g=g: combine(a, g)) for a in range(2) for g in range(MQ // 16)]

    def setup_qkv(name):
        part = "qkv".index(name)
        nb0 = (D * part) // 128
        base = D * part - 128 * nb0

        def transpose(nb):
            wn = min(128, D * part + D - 128 * nb)
            for kt in range(5):
                wk = 128 if kt < 4 else 64
                blk = wqkv_raw[128 * kt:128 * kt + wk, 128 * nb:128 * nb + wn].astype(F32)
                wts[kt, 128 * (nb - nb0):128 * (nb - nb0) + wn, 0:wk] = blk.T

        def rows(hg, kt, g):
            return jnp.concatenate([wts[kt, pl.ds(base + MQ * hg + 2 * g + e, 8, stride=DH), :]
                                    for e in range(2)], axis=0)
        return [(wqkv_raw, lambda nb=nb: transpose(nb)) for nb in range(nb0, nb0 + 5)] + combine_steps(part, wts, rows)

    def setup_wo():
        def transpose(nb):
            wn = 128 if nb < 4 else 64
            xf[nb, 0:D, 0:wn] = wo_raw[0:D, 128 * nb:128 * nb + wn].astype(F32)
            pair = [[_pk(*[xf[nb, pl.ds(MQ * hg + d + e, 8, stride=DH), :][:, :wn] for e in range(2)])
                     for d in range(0, DH, 2)] for hg in range(4)]
            for kt in range(5):
                w = pair[kt][:8] if kt < 4 else [pair[hg][8] for hg in range(4)]
                blk = _bf(jnp.concatenate(w, axis=0)).astype(F32).T
                hf[3 * kt + nb // 2, pl.ds(128 * (nb % 2), wn), 0:blk.shape[1]] = blk

        def rows(i, kt, g):
            row = MQ * i + 16 * g
            return hf[3 * kt + row // 256, pl.ds(row % 256, 16), :]
        return [(wo_raw, lambda nb=nb: transpose(nb)) for nb in range(5)] + combine_steps(3, hf, rows)

    def x_to_rows(t):
        x = xio[:, 128 * t:128 * t + 128]
        st, xs = {}, x.astype(F32)
        for g in range(D // 8):
            add_stats(st, g % 2, xs[8 * g:8 * g + 8])
        m, rs = mean_rstd({0: (st[0][0] + st[1][0], st[0][1] + st[1][1])}, 0)
        stat = jnp.where(lax.broadcasted_iota(jnp.int32, (32, 128), 0) == 0, m, rs)
        words = pltpu.bitcast(x, F32)
        for b in range(3):
            if b < 2:
                w = words[128 * b:128 * b + 128].T
            else:
                w = jnp.concatenate([words[256:288], stat], axis=0).T
                w = jnp.concatenate([w, jnp.zeros((128, 64), F32)], axis=1)
            for jj in range(8):
                perm[pl.ds(49 * (8 * t + jj) + b, 16, stride=3), :] = w[16 * jj:16 * jj + 16]

    def rows_to_tile(s, r, mr, slabs=range(3)):
        for b in slabs:
            w = perm[pl.ds(3 * (2 * r + s) + b, 128, stride=49), :]
            if b < 2:
                xr[8 * s + r, 256 * b:256 * b + 256, :] = _bf(w.T).astype(F32)
            else:
                w = w[:, :64].T
                xr[8 * s + r, 512:D, :] = _bf(w[0:32]).astype(F32)
                mr[r] = (w[32:33], w[33:34])

    def tiles_to_rows(b, s, tiles):
        nw = 128 if b < 2 else 32
        for r in tiles:
            if s == 0:
                w = _pk(xr[r, pl.ds(256 * b, nw, stride=2), :], xr[r, pl.ds(256 * b + 1, nw, stride=2), :])
            else:
                w = ob[z + r // 2, pl.ds(288 * (r % 2) + 128 * b, nw), :]
            w = jnp.concatenate([pltpu.bitcast(w, F32)] * (128 // nw), axis=0)
            perm[pl.ds(3 * (2 * r + s) + b, 128, stride=49), :] = w.T

    def rows_to_out(b):
        def rows(t):
            return jnp.concatenate([perm[pl.ds(49 * (8 * t + jj) + b, 16, stride=3), :] for jj in range(8)], axis=0)
        group = lax.broadcasted_iota(jnp.int32, (128, 128), 1) // 32
        for u in range(4):
            if b < 2:
                for t in range(4 * u, 4 * u + 4):
                    xio[256 * b:256 * b + 256, 128 * t:128 * t + 128] = _bf(rows(t).T)
                cp_out(b, u).start()
            else:
                w = rows(4 * u)
                for t in range(1, 4):
                    w = jnp.where(group == t, rows(4 * u + t), w)
                w = _bf(w.T)
                for t in range(4):
                    xio[512:D, pl.ds(128 * (4 * u + t), 128)] = w[64 * t:64 * t + 64]
        if b == 2:
            cp_out(b, 0).start()

    def prep_r(c, a):
        slot = c % RING
        for u in range(2):
            for g in range(8):
                def load(quad):
                    ws = [pltpu.bitcast((wg_raw, wu_raw)[u][slot, pl.ds(128 * (2 * quad[0] + i) + 16 * g, 16),
                                                            pl.ds(256 * quad[1], 256)], U32) for i in range(2)]
                    ws = [w[:, 128 * j:128 * j + 128] for w in ws for j in range(2)]
                    return [_lo(w) for w in ws] + [_hi(w) for w in ws]
                v = _select(RHS_SEL[a], load)
                for b, (lo, hi) in enumerate(zip(_rhs1(*v[:4]), _rhs1(*v[4:]))):
                    r_ref[c, 7 * a + b, 8 * g:8 * g + 8, 128 * u:128 * u + 128] = _pk(lo, hi)

    def prep_l(c):
        slot = c % RING
        for g in range(MQ // 16):
            ws = [pltpu.bitcast(wd_raw[slot, pl.ds(MQ * i + 16 * g, 16), :], U32) for i in range(4)]
            ws = [[w[:, 128 * j:128 * j + 128] for j in range(4)] for w in ws]
            lo = _in2(_lhs1, [[_lo(w) for w in row] for row in ws])
            hi = _in2(_lhs1, [[_hi(w) for w in row] for row in ws])
            for k in range(49):
                l_ref[c, pl.ds(72 * k + 8 * g, 8), :] = _pk(lo[k], hi[k])

    def prep_a(a, half, g):
        src, row = (xf, xo)[g // 4], 32 * (g % 4) + half

        def load(quad):
            return [src[z2 + 2 * quad[1] + j, pl.ds(128 * (2 * quad[0] + i) + row + e, 8, stride=4), :]
                    for e in (0, 2) for i in range(2) for j in range(2)]
        v = _select(LHS_SEL[a], load)
        o = [_pk(lo, hi) for lo, hi in zip(_lhs1(*v[:4]), _lhs1(*v[4:]))]
        for b in range(7):
            a_ref[z + 7 * a + b, 64 * half + 8 * g:64 * half + 8 * g + 8, :] = o[b]
        return o[5] ^ o[6]

    def prep_a_tail():
        for i in range(4):
            for half in range(2):
                for u, src in enumerate((xf, xo)):
                    lo = src[z + 4, pl.ds(128 * i + half, 32, stride=4), :][:, :64]
                    hi = src[z + 4, pl.ds(128 * i + half + 2, 32, stride=4), :][:, :64]
                    at_ref[z + i, pl.ds(64 * half + 32 * u, 32), :] = _pk(lo, hi)

    def put(a):
        for g in range(16):
            def load(quad):
                return [hf[z + 4 * (2 * quad[1] + quad[0]) + t, pl.ds(o + 8 * g, 8), :]
                        for o in (0, 128) for t in (0, 2, 1, 3)]
            v = _select(RHS_SEL[a], load)
            for b, (lo, hi) in enumerate(zip(_rhs1(*v[:4]), _rhs1(*v[4:]))):
                h_ref[7 * a + b, 8 * g:8 * g + 8, :] = _pk(lo, hi)

    def strassen_inner(prod, nrow, emit, odd=None):
        ld = lambda s: ti[z + s, 0:nrow, :]
        for s in range(3):
            ti[z + s, 0:nrow, :] = prod(s)
        if not odd:
            emit(3, ((ld(0) - ld(1)) + ld(2)) + prod(5))
        m3 = prod(3)
        emit(2, ld(1) + m3)
        if odd is None:
            ti[z + 3, 0:nrow, :] = ld(0) + m3
        m4 = prod(4)
        emit(1, ld(2) + m4)
        ti[z + 3, 0:nrow, :] = (ld(3) if odd is None else ld(0) + m3) - m4
        if odd:
            emit(3, ((ld(0) - ld(1)) + ld(2)) + prod(5))
        emit(0, ld(3) + prod(6))

    def gate_up(c, before=None):
        c0 = c * FC if isinstance(c, int) else pl.multiple_of(c * FC, FC)

        def inner(a, emit):
            if before is not None:
                before(a)
            strassen_inner(lambda b: _dot(_bf(a_ref[z + 7 * a + b]), _bf(r_ref[c, 7 * a + b])), TQ, emit)

        def fin(quad, q, v):
            i, j = 2 * (quad // 2) + q // 2, 2 * (quad % 2) + q % 2
            cols = pl.ds(c0 + 128 * j, 128)
            wt = jnp.concatenate([tg[:, cols], tu[:, cols]], axis=1)
            v = v + _dot(_bf(at_ref[z + i]), wt)
            hf[z + 4 * quad + q] = v[:, :128] * v[:, 128:]

        def old(s, q):
            return to[z + 4 * s + q]

        def keep(s):
            def emit(q, v):
                to[z + 4 * s + q] = v
            return emit

        def emit3(q, v):
            fin(2, q, old(1, q) + v)
            to[z + 12 + q] = old(0, q) + v

        def emit4(q, v):
            fin(1, q, old(2, q) + v)
            to[z + 12 + q] = old(3, q) - v

        inner(2, keep(2))
        inner(0, keep(0))
        inner(1, keep(1))
        inner(5, lambda q, v: fin(3, q, ((old(0, q) - old(1, q)) + old(2, q)) + v))
        put(4)
        inner(3, emit3)
        put(2)
        inner(4, emit4)
        put(6)
        inner(6, lambda q, v: fin(0, q, old(3, q) + v))

    def down_prod(c, k, prev):
        return prev + lax.dot_general(_bf(l_ref[c, 72 * k:72 * k + 72, :]), _bf(h_ref[k]), NT_DIMS, preferred_element_type=F32)

    def down(c):
        for a, late in ((4, 1), (2, 0), (6, 3), (1, 5), (0, None), (3, None), (5, None)):
            for k in range(7 * a, 7 * a + 7):
                acc[k] = down_prod(c, k, jnp.where(c == 0, 0.0, acc[k]))
            if late is not None:
                put(late)

    def add_stats(st, r, x):
        st[r] = (x, x * x) if st.get(r) is None else (st[r][0] + x, st[r][1] + x * x)

    def mean_rstd(st, r):
        m = jnp.sum(st[r][0], axis=0, keepdims=True) * (1.0 / D)
        v = jnp.sum(st[r][1], axis=0, keepdims=True) * (1.0 / D) - m * m
        return m, lax.rsqrt(jnp.maximum(v, 0.0) + EPS)

    def down_final(base, st, after=None, between=()):
        odd = [False]

        def inner(a, emit, late=None):
            strassen_inner(lambda b: down_prod(NC - 1, 7 * a + b, acc[7 * a + b]), MQ, emit, odd[0])
            if late is not None:
                put(late)
            if a in between:
                between[a]()
            else:
                odd[0] = not odd[0]

        def old(s, q):
            return to[z + 4 * s + q, 0:MQ, :]

        def keep(s, q, v):
            to[z + 4 * s + q, 0:MQ, :] = v

        def fin(quad, q, v):
            i, j = 2 * (quad // 2) + q // 2, 2 * (quad % 2) + q % 2
            rows = pl.ds(MQ * i, MQ)
            for e in range(2):
                r = j + 4 * e
                ref, slot = xm[r]
                x = ref[z + slot, rows, :] + v[:, 128 * e:128 * e + 128]
                if st is None:
                    ob[z + r // 2, pl.ds(288 * (r % 2) + 72 * i, 72), :] = _u32(x)
                    continue
                xr[base + r, rows, :] = x
                for g in range(MQ // 8):
                    add_stats(st, r, x[8 * g:8 * g + 8])
            if after is not None and q == 0:
                after(quad)

        inner(4, lambda q, v: keep(0, q, v), 0)
        inner(2, lambda q, v: (fin(1, q, old(0, q) + v), keep(1, q, v)), 3)
        inner(6, lambda q, v: keep(0, q, v - old(0, q)), 1)
        inner(0, lambda q, v: (keep(0, q, old(0, q) + v), keep(1, q, old(1, q) + v)), 5)
        inner(3, lambda q, v: (fin(0, q, old(0, q) + v), keep(2, q, v)))
        inner(1, lambda q, v: (fin(2, q, old(2, q) + v), keep(1, q, old(1, q) - v)))
        inner(5, lambda q, v: fin(3, q, old(1, q) + v))

    def chain(ref, last, v, skew=1):
        last.append(pltpu.bitcast(v, F32))
        if len(last) > skew:
            fence(ref, last.pop(0))

    def ln1_fns(base, mr, pairs):
        def norm(r, row, n):
            return (xr[base + r, pl.ds(row, n), :] - mr[r][0]) * mr[r][1]

        def job(u, g):
            if g == 16:
                y = jnp.concatenate([_u32(norm(2 * u + e, 512, 64)) for e in range(2)], axis=0)
                xn[u, 896:960, :] = y
                return tree(jnp.bitwise_xor, [y[8 * k:8 * k + 8] for k in range(8)])
            y = [_u32(v) for v in _rhs1(*[norm(2 * u + e, 256 * k + 16 * g, 16) for k in range(2) for e in range(2)])]
            for b in range(7):
                xn[u, pl.ds(128 * b + 8 * g, 8), :] = y[b]
            return y[5] ^ y[6]
        return [lambda u=u, g=g: job(u, g) for u in pairs for g in range(17)]

    ticks, clock = [], [0]

    def project(name, a, u, emit, x=None):
        w = 2 * "qkvo".index(name) + a
        src, slot = (ob, z + u) if name == "o" else (xn, u)
        rows = lambda i, n: src[slot, i:i + n, :] if x is None else x[i:i + n]

        def tick(y):
            clock[0] += 1
            for g in range(DH * (clock[0] % 2)):
                run(ticks, y[8 * g:8 * g + 8, 0:128])
            return y
        m = lambda b: tick(_dot(_bf(wt[w, b]), _bf(rows(128 * b, 128))))
        xt = lambda: _bf(jnp.concatenate([rows(896, 32), rows(928, 32)], axis=1))
        tail = lambda i: tick(_dot(_bf(wt[w, 7, :, 128 * i:128 * i + 64]), xt()))
        ta, m4 = tail(0), m(4)
        s11, s12 = ta[:, :128] - m4, ta[:, 128:] + m4
        s22 = m(2)
        emit(a, 2 * u + 1, s12 + s22)
        s11 = s11 + m(6)
        m0 = m(0)
        s11, s22 = s11 + m0, s22 + m0
        s21 = m(3)
        emit(a, 2 * u, s11 + s21)
        tb = tail(1)
        s21, s22 = s21 + tb[:, :128], s22 + tb[:, 128:]
        m1 = m(1)
        emit(a + 2, 2 * u, s21 + m1)
        emit(a + 2, 2 * u + 1, (s22 - m1) + m(5))

    def project_kv(name, a, u, jobs=(), every=1, x=None):
        def emit(hg, r, y):
            dst, rows = (kb, pl.ds(MQ * hg, MQ)) if name == "k" else (vbs[a], pl.ds(MQ * (hg // 2), MQ))
            dst[z + 7 + r, rows, :] = y
            if r >= 1:
                dst[z + r - 1, rows, :] = pltpu.roll(y, 1, 1)
            for g in range(0, DH, every):
                run(jobs, y[8 * g:8 * g + 8])
        project(name, a, u, emit, x)

    def prow(hg, w):
        return pl.ds(32 * w + 16 * (hg % 2) + 8 * (hg // 2), 8)

    def project_q(a, u, jobs, extra):
        def emit(hg, r, y):
            lg = [None] * W
            for d in range(DH):
                q = y[8 * d:8 * d + 8]
                for w in range(W):
                    v = q * kb[z + 7 + r - w, pl.ds(MQ * hg + 8 * d, 8), :]
                    lg[w] = v if d == 0 else lg[w] + v
                run(extra, q)
            for w in range(W):
                pb[z + r, prow(hg, w), :] = lg[w]
            if hg >= 2:
                jobs.append(softmax_job(r, a))
        project("q", a, u, emit)

    def softmax_job(r, sl):
        def job(v):
            fence(pb, v)
            lane0 = lax.broadcasted_iota(jnp.int32, (16, 128), 1) == 0
            lg = [pb[z2 + r, 32 * w + 16 * sl:32 * w + 16 * sl + 16, :] for w in range(W)]
            lg = [jnp.where(lane0, NEG, lg[w]) if w > r else lg[w] for w in range(W)]
            m = tree(jnp.maximum, lg)
            ex = [jnp.exp2((lg[w] - m) * EXP_C) for w in range(W)]
            inv = 1.0 / tree(jnp.add, ex)
            for w in range(W):
                pb[z2 + r, 32 * w + 16 * sl:32 * w + 16 * sl + 16, :] = ex[w] * inv
        return job

    def mix_jobs(a):
        o = {}

        def job(u, g, i):
            p = [[pb[z2 + 2 * u + e, prow(a + 2 * i, w), :] for w in range(W)] for e in range(2)]
            for d in range(2):
                v = [vbs[a][z2 + 2 * u + t, pl.ds(MQ * i + 16 * g + 8 * d, 8), :] for t in range(W + 1)]
                for e in range(2):
                    o[d, i, e] = tree(jnp.add, [p[e][w] * v[7 + e - w] for w in range(W)])
            if i == 0:
                y = pltpu.bitcast((o[0, 0, 0] + o[0, 0, 1]) + (o[1, 0, 0] + o[1, 0, 1]), U32)
                if (a, u, g) == (0, 0, 0):
                    xn[z, 960:968, :] = y
                return y
            lo, hi = [[o[d, i, e] for i in range(2) for e in range(2)] for d in range(2)]
            if g < 8:
                y = [_pk(*t) for t in zip(_rhs1(*lo), _rhs1(*hi))]
                for b in range(7):
                    ob[z + u, pl.ds(128 * b + 64 * a + 8 * g, 8), :] = y[b]
                return y[5] ^ y[6]
            y = [_pk(*t) for t in zip(lo, hi)]
            for k in range(4):
                ob[z + u, pl.ds(896 + 32 * (k % 2) + 8 * (a + 2 * (k // 2)), 8), :] = y[k]
            return tree(jnp.bitwise_xor, y)
        return paced(vbs[a], [lambda u=u, g=g, i=i: job(u, g, i)
                              for u in range(4) for g in range(9) for i in range(2)], 1)

    def ln2(st, r):
        m, rs = mean_rstd(st, r)
        (ref, slot), last = xm[r], []
        for kt in range(5):
            wk = 128 if kt < 4 else 64
            y = ((ref[z2 + slot, 128 * kt:128 * kt + wk, :] - m) * rs).T
            (xf, xo)[r // 4][z + kt, pl.ds(128 * (r % 4), 128), 0:wk] = y
            if kt < 4:
                chain(ref, last, y[0:8], 2)

    def prep_a_jobs(outer, odd):
        return paced((xf, xo)[odd], [lambda a=a, half=half, g=g: prep_a(a, half, g) for a in outer
                                     for half in range(2) for g in range(4 * odd, 4 * odd + 4)], 2)

    def out_proj(base, st, a, u, jobs):
        def emit(i, r, y):
            for g in range(MQ // 16):
                rows = pl.ds(MQ * i + 16 * g, 16)
                x = xr[base + r, rows, :] + y[16 * g:16 * g + 16]
                xm[r][0][z + xm[r][1], rows, :] = x
                add_stats(st, r, x[0:8])
                add_stats(st, r, x[8:16])
                if (i, r, clock[0] % 2) != (a + 2, 2 * u + 1, 0):
                    run(jobs, x[0:8])
        project("o", a, u, emit)

    def attention_block(p, first):
        s = 0 if first else p % 2
        cur, nxt = 8 * s, 8 * (1 - s)
        st1 = {}
        if first:
            st0 = {}
            for r in range(NT_):
                rows_to_tile(0, r, st0)
            for fn in ln1_fns(0, st0, (0, 1)):
                fn()
            project_kv("k", 0, 0)
            jobs = spread([lambda v: fence(xr, v)] + paced(xr, ln1_fns(z2, st0, (2, 3)), 2), 180)
            for a, u in ((1, 0), (0, 1), (1, 1)):
                project_kv("k", a, u, jobs)
            cp_qkv("q").wait()
            cp_qkv("v").wait()
            cp_wo().wait()
            steps = setup_qkv("q")
            for _, fn in steps[:5]:
                fn()
            project_kv("k", 0, 2)
            jobs = spread([gate(*step) for step in steps[5:]], 216)
            wo_jobs = [gate(*step) for step in setup_wo()]
            jobs[6:6 + 40 * 5:40] = wo_jobs[:5]
            for a, u in ((1, 2), (0, 3), (1, 3)):
                project_kv("k", a, u, jobs)
            extra = [gate(perm, lambda r=r, b=b: rows_to_tile(1, r, st1, (b,))) for r in range(NT_) for b in range(3)]
            steps = [gate(*step) for step in setup_qkv("v")]
            extra = steps[:5] + extra[:6] + [job for pair in zip(steps[5:], extra[6:]) for job in pair]
            extra = spread(extra, 500)
        else:
            extra = []
            unit = {2: (0, 2), 0: (1, 2), 3: (0, 3), 1: (1, 3)}
            down_final(nxt, st1, None, {g: lambda g=g: project_kv("k", *unit[g]) for g in unit})
            st1 = {r: mean_rstd(st1, r) for r in range(NT_)}
        jobs = []
        for u in range(4):
            for a in range(2):
                project_q(a, u, jobs, extra)
        if first:
            for cp in cp_ffn(0) + cp_tails():
                cp.wait()
        clock[0] = 0 if first else 1
        ticks.extend(spread(jobs + [lambda v: fence(pb, v)], 306))
        ln1 = [lambda v: fence(xr, v)] + paced(xr, ln1_fns(z2 + nxt, st1, range(4)), 2)
        for vb in vbs:
            prime(vb, ob)
        prime(xf, a_ref)
        prime(xo, a_ref)
        x0 = xn[0, 0:960, :]
        ticks[93:93 + 12 * 18:12] = ln1[:18]
        if first:
            ticks[1:1 + 4 * 18:4] = wo_jobs[5:]
        for u in range(4):
            project_kv("v", 0, u)
        assert not ticks
        ticks.extend(spread([], 24) + spread(mix_jobs(0), 300))
        for u in range(4):
            project_kv("v", 1, u, x=x0 if u == 0 else None)
        assert not ticks
        ticks.extend(spread([], 24) + spread(mix_jobs(1), 300))
        for a in range(2):
            project_kv("k", a, 0)
        if first:
            prep_l(0)
        st2, jobs = {}, []
        for u in range(4):
            if u == 1:
                jobs = spread(ln1[18:], 126)
            if u == 2:
                assert not ticks
                ticks.extend(spread([], 81) + spread(prep_a_jobs(G_ORDER, 0), 219) + spread(prep_a_jobs((2,), 1), 24))
            for a in range(2):
                out_proj(cur, st2, a, u, jobs)
            ln2(st2, 2 * u)
            ln2(st2, 2 * u + 1)
        assert not jobs and not ticks
        last = []
        project_kv("k", 0, 1)
        project_kv("k", 1, 1, [last.append])
        for a in G_ORDER[1:]:
            for half in range(2):
                for g in range(4, 8):
                    chain(xo, last, prep_a(a, half, g))
        prep_a_tail()
        gate_up(0, (lambda a: prep_r(0, a)) if first else None)

    def ffn_loop(first):
        def body(c, carry):
            if first:
                for cp in cp_ffn(c + 1):
                    cp.wait()

                @pl.when(c + RING < NC)
                def _():
                    for cp in cp_ffn(c + RING):
                        cp.start()
            down(c)
            if first:
                prep_l(c + 1)

            gate_up(c + 1, (lambda a: prep_r(c + 1, a)) if first else None)
            return carry
        lax.fori_loop(0, NC - 1, body, 0)

    cp_qkv("k").start()
    for u in range(4):
        cp_x(u).start()
    for cp in (cp_qkv("q"), cp_qkv("v"), cp_wo()) + cp_ffn(0) + cp_tails() + cp_ffn(1) + cp_ffn(2):
        cp.start()
    cp_qkv("k").wait()
    for _, fn in setup_qkv("k"):
        fn()
    for u in range(4):
        cp_x(u).wait()
        for t in range(X_SPLIT[u], X_SPLIT[u + 1]):
            x_to_rows(t)

    attention_block(0, True)
    ffn_loop(True)

    def pass_body(p, carry):
        attention_block(p, False)
        ffn_loop(False)
        return carry
    lax.fori_loop(1, 4, pass_body, 0)

    for b in range(3):
        tiles_to_rows(b, 0, range(NT_))

    def after(quad):
        tiles = [2 * (quad % 2) + t for t in (0, 1, 4, 5)]
        slabs = ((0,), (2, 1))[quad // 2]
        for b in slabs:
            tiles_to_rows(b, 1, tiles)
        if quad in (0, 3):
            for b in slabs:
                rows_to_out(b)
    down_final(None, None, after)
    for b, u in [(b, u) for b in range(2) for u in range(4)] + [(2, 0)]:
        cp_out(b, u).wait()


@jax.jit
def pallas_interleave_layers__sliding_local_dilated__glu_gated_bilinear__prompt_kernel(
    A_x: jax.Array,
    A_wqkv: jax.Array,
    A_wo: jax.Array,
    B_x: jax.Array,
    B_w_gate: jax.Array,
    B_w_up: jax.Array,
    B_w_down: jax.Array,
):
    del B_x
    vm = pltpu.VMEM
    scratch = [
        vm((D, S), BF), vm((D + 32, 3 * D), BF), vm((D + 64, D), BF),
        vm((RING, 512, FC), BF), vm((RING, 512, FC), BF), vm((RING, D, FC), BF),
        vm((D - 512, F), BF), vm((D - 512, F), BF),
        vm((6, 640, 128), F32),
        vm((8, 8, MQ // 2, 256), U32),
        vm((2 * NT_ + 1, D, 128), F32),
        vm((5, D, 128), F32),
        vm((5, D, 128), F32),
        vm((4, 992, 128), U32),
        vm((15, D, 128), F32),
        vm((16, D // 2, 128), F32),
        vm((16, D // 2, 128), F32),
        vm((NT_ + 1, W * H, 128), F32),
        vm((4, 960, 128), U32),
        vm((6, D, 128), F32),
        vm((6, S // 4, 128), F32),
        vm((49 * 128 + 32, 128), F32),
        vm((49, TQ // 2, 128), U32),
        vm((4, TQ // 2, 64), U32),
        vm((49, MQ, TQ), F32),
        vm((49, TQ // 2, 128), U32),
        vm((4, TQ, 256), F32),
        vm((16, TQ, 256), F32),
        vm((16, TQ, 128), F32),
        vm((NC, 49, 64, 256), U32),
        vm((NC, 3552, 128), U32),
        pltpu.SMEM((2,), jnp.int32),
        pltpu.SemaphoreType.DMA((11 + 3 * RING,)),
    ]
    hbm = pl.BlockSpec(memory_space=pl.ANY)
    out = pl.pallas_call(
        _kernel,
        in_specs=[hbm] * 6,
        out_specs=hbm,
        out_shape=jax.ShapeDtypeStruct((D, S), BF),
        scratch_shapes=scratch,
        compiler_params=pltpu.CompilerParams(vmem_limit_bytes=126 * 1024 * 1024),
    )(A_x.reshape(S, D).T, A_wqkv, A_wo, B_w_gate, B_w_up, B_w_down.T)
    return out.T.reshape(1, S, D)
```

```python
import math

import jax
import jax.numpy as jnp
from jax import lax
import jax.experimental.pallas as pl
import jax.experimental.pallas.tpu as pltpu

S, D, F = 2048, 576, 4608
H, DH, W = 32, 18, 8
NT_ = 8
TQ = 256
MQ = D // 4
FC = 512
NC = F // FC
RING = 3
X_SPLIT = (0, 5, 10, 14, 16)
EPS = 1e-5
SCALE = DH ** -0.5
EXP_C = SCALE * math.log2(math.e)
NEG = -1e9 / SCALE

BF, F32, U32 = jnp.bfloat16, jnp.float32, jnp.uint32
NT_DIMS = (((1,), (1,)), ((), ()))

LHS_SEL = {0: ((0, 0), 1, (1, 1)), 1: ((1, 0), 1, (1, 1)), 2: ((0, 0), 0, None), 3: ((1, 1), 0, None),
           4: ((0, 0), 1, (0, 1)), 5: ((1, 0), -1, (0, 0)), 6: ((0, 1), -1, (1, 1))}
RHS_SEL = {0: ((0, 0), 1, (1, 1)), 1: ((0, 0), 0, None), 2: ((0, 1), -1, (1, 1)), 3: ((1, 0), -1, (0, 0)),
           4: ((1, 1), 0, None), 5: ((0, 0), 1, (0, 1)), 6: ((1, 0), 1, (1, 1))}
G_ORDER = (2, 0, 1, 5, 3, 4, 6)


def _lhs1(a11, a12, a21, a22):
    return [a11 + a22, a21 + a22, a11, a22, a11 + a12, a21 - a11, a12 - a22]


def _rhs1(b11, b12, b21, b22):
    return [b11 + b22, b11, b12 - b22, b21 - b11, b22, b11 + b12, b21 + b22]


def _in2(fn, x):
    outer = [[fn(x[i][j], x[i][2 + j], x[2 + i][j], x[2 + i][2 + j]) for j in range(2)] for i in range(2)]
    return [v for a in range(7) for v in fn(outer[0][0][a], outer[0][1][a], outer[1][0][a], outer[1][1][a])]


def _select(sel, load):
    first, sign, second = sel
    v = load(first)
    if sign == 1:
        v = [a + b for a, b in zip(v, load(second))]
    elif sign == -1:
        v = [a - b for a, b in zip(v, load(second))]
    return v


def _pk(lo, hi):
    return pltpu.pack_elementwise([lo, hi], packed_dtype=BF)


def _lo(w):
    return pltpu.unpack_elementwise(w, index=0, packed_dtype=BF, unpacked_dtype=F32)


def _hi(w):
    return pltpu.unpack_elementwise(w, index=1, packed_dtype=BF, unpacked_dtype=F32)


def _bf(w):
    return pltpu.bitcast(w, BF)


def _u32(x):
    return pltpu.bitcast(x.astype(BF), U32)


def _dot(a, b):
    return jnp.dot(a, b, preferred_element_type=F32)


def _kernel(x_hbm, wqkv_hbm, wo_hbm, wg_hbm, wu_hbm, wd_hbm, out_hbm,
            xio, wqkv_raw, wo_raw, wg_raw, wu_raw, wd_raw, tg, tu,
            wts, wt, xr, xm0, xm1, xn, kb, vb0, vb1, pb, ob, xf, xo, perm,
            a_ref, at_ref, acc, h_ref, ti, to, hf, r_ref, l_ref, t_ref, zero_ref, sems):
    def clear(i, carry):
        zero_ref[i] = 0
        return carry
    lax.fori_loop(0, 2, clear, 0)
    z = zero_ref[0]
    z2 = zero_ref[1]
    vbs = (vb0, vb1)
    ticks, clock = [], [0]
    xm = [((xm0, xm1)[r // 2 % 2], r // 4 * 2 + r % 2) for r in range(NT_)]

    def fence(ref, v):
        ref[z + (ref.shape[0] - 1), 0:8, 0:128] = v

    def gate(ref, fn):
        def job(v):
            if len(ref.shape) == 3:
                fence(ref, v)
            else:
                rows = pl.ds(pl.multiple_of(16 * z + (ref.shape[0] - 16), 16), 16)
                ref[rows, 0:128] = jnp.concatenate([v, v], axis=0).astype(ref.dtype)
            fn()
        return job

    def prime(ref, other):
        ref[z2 + (ref.shape[0] - 1), 0:8, 0:128] = pltpu.bitcast(other[z, 0:8, 0:128], F32)

    def paced(ref, fns, skew):
        last = []

        def job(v, fn):
            last.append(fn())
            if len(last) > skew:
                v = pltpu.bitcast(last.pop(0) ^ pltpu.bitcast(v, U32), F32)
            fence(ref, v)
        return [lambda v, fn=fn: job(v, fn) for fn in fns]

    def spread(jobs, n):
        slots = [lambda v: None] * n
        for i, job in enumerate(jobs):
            slots[i * n // len(jobs)] = job
        return slots

    def overlay(slots, start, step, jobs):
        for i, job in enumerate(jobs):
            k = start + step * i
            slots[k] = lambda v, old=slots[k], job=job: (old(v), job(v))

    def run(jobs, v, n=1):
        for _ in range(n):
            if jobs:
                jobs.pop(0)(v)

    def tree(fn, v):
        while len(v) > 1:
            v = [fn(v[i], v[i + 1]) for i in range(0, len(v), 2)]
        return v[0]

    def cp_x(u):
        cols = pl.ds(128 * X_SPLIT[u], 128 * (X_SPLIT[u + 1] - X_SPLIT[u]))
        return pltpu.make_async_copy(x_hbm.at[:, cols], xio.at[:, cols], sems.at[u])

    def cp_out(b, u):
        rows, cols = (pl.ds(256 * b, 256), pl.ds(512 * u, 512)) if b < 2 else (pl.ds(512, 64), pl.ds(0, S))
        return pltpu.make_async_copy(xio.at[rows, cols], out_hbm.at[rows, cols], sems.at[4 * b + u])

    qkv_cols = {"k": pl.ds(512, 640), "v": pl.ds(1152, 576), "q": pl.ds(0, 512)}

    def cp_qkv(name):
        idx = 5 + "kvq".index(name)
        return pltpu.make_async_copy(wqkv_hbm.at[:, qkv_cols[name]], wqkv_raw.at[0:D, qkv_cols[name]], sems.at[idx])

    def cp_wo():
        return pltpu.make_async_copy(wo_hbm, wo_raw.at[0:D], sems.at[8])

    def cp_ffn(c):
        c0 = c * FC if isinstance(c, int) else pl.multiple_of(c * FC, FC)
        cols = pl.ds(c0, FC)
        slot = c % RING
        return (pltpu.make_async_copy(wg_hbm.at[0:512, cols], wg_raw.at[slot], sems.at[11 + 3 * slot]),
                pltpu.make_async_copy(wu_hbm.at[0:512, cols], wu_raw.at[slot], sems.at[12 + 3 * slot]),
                pltpu.make_async_copy(wd_hbm.at[:, cols], wd_raw.at[slot], sems.at[13 + 3 * slot]))

    def cp_tails():
        return (pltpu.make_async_copy(wg_hbm.at[512:D, :], tg, sems.at[9]),
                pltpu.make_async_copy(wu_hbm.at[512:D, :], tu, sems.at[10]))

    def combine_steps(part, ref, rows):
        def combine(a, g):
            for j in range(2):
                w = _lhs1(rows(a, j, g), rows(a, 2 + j, g), rows(a + 2, j, g), rows(a + 2, 2 + j, g))
                for b in range(7):
                    wt[2 * part + a, b, 8 * g:8 * g + 8, 128 * j:128 * j + 128] = _u32(w[b])
                wt[2 * part + a, 7, 8 * g:8 * g + 8, 128 * j:128 * j + 64] = _u32(rows(a + 2 * j, 4, g)[:, :64])
        return [(ref, lambda a=a, g=g: combine(a, g)) for a in range(2) for g in range(MQ // 16)]

    def setup_qkv(name):
        part = "qkv".index(name)
        nb0 = (D * part) // 128
        base = D * part - 128 * nb0

        def transpose(nb):
            wn = min(128, D * part + D - 128 * nb)
            for kt in range(5):
                wk = 128 if kt < 4 else 64
                blk = wqkv_raw[128 * kt:128 * kt + wk, 128 * nb:128 * nb + wn].astype(F32)
                wts[kt, 128 * (nb - nb0):128 * (nb - nb0) + wn, 0:wk] = blk.T

        def rows(hg, kt, g):
            return jnp.concatenate([wts[kt, pl.ds(base + MQ * hg + 2 * g + e, 8, stride=DH), :]
                                    for e in range(2)], axis=0)
        return [(wqkv_raw, lambda nb=nb: transpose(nb)) for nb in range(nb0, nb0 + 5)] + combine_steps(part, wts, rows)

    def setup_wo():
        def transpose(nb):
            wn = 128 if nb < 4 else 64
            xf[nb, 0:D, 0:wn] = wo_raw[0:D, 128 * nb:128 * nb + wn].astype(F32)
            pair = [[_pk(*[xf[nb, pl.ds(MQ * hg + d + e, 8, stride=DH), :][:, :wn] for e in range(2)])
                     for d in range(0, DH, 2)] for hg in range(4)]
            for kt in range(5):
                w = pair[kt][:8] if kt < 4 else [pair[hg][8] for hg in range(4)]
                blk = _bf(jnp.concatenate(w, axis=0)).astype(F32).T
                hf[3 * kt + nb // 2, pl.ds(128 * (nb % 2), wn), 0:blk.shape[1]] = blk

        def rows(i, kt, g):
            row = MQ * i + 16 * g
            return hf[3 * kt + row // 256, pl.ds(row % 256, 16), :]
        return [(wo_raw, lambda nb=nb: transpose(nb)) for nb in range(5)] + combine_steps(3, hf, rows)

    def x_to_rows(t):
        x = xio[:, 128 * t:128 * t + 128]
        st, xs = {}, x.astype(F32)
        for g in range(D // 8):
            add_stats(st, g % 2, xs[8 * g:8 * g + 8])
        m, rs = mean_rstd({0: (st[0][0] + st[1][0], st[0][1] + st[1][1])}, 0)
        stat = jnp.where(lax.broadcasted_iota(jnp.int32, (32, 128), 0) == 0, m, rs)
        words = pltpu.bitcast(x, F32)
        for b in range(3):
            if b < 2:
                w = words[128 * b:128 * b + 128].T
            else:
                w = jnp.concatenate([words[256:288], stat], axis=0).T
                w = jnp.concatenate([w, jnp.zeros((128, 64), F32)], axis=1)
            for jj in range(8):
                perm[pl.ds(49 * (8 * t + jj) + b, 16, stride=3), :] = w[16 * jj:16 * jj + 16]

    def rows_to_tile(s, r, mr, slabs=range(3)):
        for b in slabs:
            w = perm[pl.ds(3 * (2 * r + s) + b, 128, stride=49), :]
            if b < 2:
                xr[8 * s + r, 256 * b:256 * b + 256, :] = _bf(w.T).astype(F32)
            else:
                w = w[:, :64].T
                xr[8 * s + r, 512:D, :] = _bf(w[0:32]).astype(F32)
                mr[r] = (w[32:33], w[33:34])

    def tiles_to_rows(b, s, tiles):
        nw = 128 if b < 2 else 32
        for r in tiles:
            if s == 0:
                w = _pk(xr[r, pl.ds(256 * b, nw, stride=2), :], xr[r, pl.ds(256 * b + 1, nw, stride=2), :])
            else:
                w = ob[z + r // 2, pl.ds(288 * (r % 2) + 128 * b, nw), :]
            w = jnp.concatenate([pltpu.bitcast(w, F32)] * (128 // nw), axis=0)
            perm[pl.ds(3 * (2 * r + s) + b, 128, stride=49), :] = w.T

    def rows_to_out(b):
        def rows(t):
            return jnp.concatenate([perm[pl.ds(49 * (8 * t + jj) + b, 16, stride=3), :] for jj in range(8)], axis=0)
        group = lax.broadcasted_iota(jnp.int32, (128, 128), 1) // 32
        for u in range(4):
            if b < 2:
                for t in range(4 * u, 4 * u + 4):
                    xio[256 * b:256 * b + 256, 128 * t:128 * t + 128] = _bf(rows(t).T)
                cp_out(b, u).start()
            else:
                w = rows(4 * u)
                for t in range(1, 4):
                    w = jnp.where(group == t, rows(4 * u + t), w)
                w = _bf(w.T)
                for t in range(4):
                    xio[512:D, pl.ds(128 * (4 * u + t), 128)] = w[64 * t:64 * t + 64]
        if b == 2:
            cp_out(b, 0).start()

    def prep_r(c, a):
        slot = c % RING
        for u in range(2):
            for g in range(8):
                def load(quad):
                    ws = [pltpu.bitcast((wg_raw, wu_raw)[u][slot, pl.ds(128 * (2 * quad[0] + i) + 16 * g, 16),
                                                            pl.ds(256 * quad[1], 256)], U32) for i in range(2)]
                    ws = [w[:, 128 * j:128 * j + 128] for w in ws for j in range(2)]
                    return [_lo(w) for w in ws] + [_hi(w) for w in ws]
                v = _select(RHS_SEL[a], load)
                for b, (lo, hi) in enumerate(zip(_rhs1(*v[:4]), _rhs1(*v[4:]))):
                    r_ref[c, 7 * a + b, 8 * g:8 * g + 8, 128 * u:128 * u + 128] = _pk(lo, hi)

    def prep_l(c, g):
        ws = [pltpu.bitcast(wd_raw[c % RING, pl.ds(MQ * i + 16 * g, 16), :], U32) for i in range(4)]
        ws = [[w[:, 128 * j:128 * j + 128] for j in range(4)] for w in ws]
        lo = _in2(_lhs1, [[_lo(w) for w in row] for row in ws])
        hi = _in2(_lhs1, [[_hi(w) for w in row] for row in ws])
        for k in range(49):
            l_ref[c, pl.ds(72 * k + 8 * g, 8), :] = _pk(lo[k], hi[k])

    def prep_a(a, half, g):
        src, row = (xf, xo)[g // 4], 32 * (g % 4) + half

        def load(quad):
            return [src[z2 + 2 * quad[1] + j, pl.ds(128 * (2 * quad[0] + i) + row + e, 8, stride=4), :]
                    for e in (0, 2) for i in range(2) for j in range(2)]
        v = _select(LHS_SEL[a], load)
        o = [_pk(lo, hi) for lo, hi in zip(_lhs1(*v[:4]), _lhs1(*v[4:]))]
        for b in range(7):
            a_ref[z + 7 * a + b, 64 * half + 8 * g:64 * half + 8 * g + 8, :] = o[b]
        return o[5] ^ o[6]

    def prep_a_tail():
        for i in range(4):
            for half in range(2):
                for u, src in enumerate((xf, xo)):
                    lo = src[z + 4, pl.ds(128 * i + half, 32, stride=4), :][:, :64]
                    hi = src[z + 4, pl.ds(128 * i + half + 2, 32, stride=4), :][:, :64]
                    at_ref[z + i, pl.ds(64 * half + 32 * u, 32), :] = _pk(lo, hi)

    def put(a):
        for g in range(16):
            def load(quad):
                return [hf[z + 4 * (2 * quad[1] + quad[0]) + t, pl.ds(o + 8 * g, 8), :]
                        for o in (0, 128) for t in (0, 2, 1, 3)]
            v = _select(RHS_SEL[a], load)
            for b, (lo, hi) in enumerate(zip(_rhs1(*v[:4]), _rhs1(*v[4:]))):
                h_ref[7 * a + b, 8 * g:8 * g + 8, :] = _pk(lo, hi)

    def strassen_inner(prod, nrow, emit, odd=None):
        ld = lambda s: ti[z + s, 0:nrow, :]
        for s in range(3):
            ti[z + s, 0:nrow, :] = prod(s)
        if not odd:
            emit(3, ((ld(0) - ld(1)) + ld(2)) + prod(5))
        m3 = prod(3)
        emit(2, ld(1) + m3)
        if odd is None:
            ti[z + 3, 0:nrow, :] = ld(0) + m3
        m4 = prod(4)
        emit(1, ld(2) + m4)
        ti[z + 3, 0:nrow, :] = (ld(3) if odd is None else ld(0) + m3) - m4
        if odd:
            emit(3, ((ld(0) - ld(1)) + ld(2)) + prod(5))
        emit(0, ld(3) + prod(6))

    def gate_up(c, first):
        if first:
            c0 = c * FC if isinstance(c, int) else pl.multiple_of(c * FC, FC)
            for g in range(MQ // 16):
                prep_l(c, g)
            for j in range(4):
                cols = pl.ds(c0 + 128 * j, 128)
                t_ref[c, j] = pltpu.bitcast(jnp.concatenate([tg[:, cols], tu[:, cols]], axis=1), U32)

        def inner(a, emit):
            if first:
                prep_r(c, a)
            strassen_inner(lambda b: _dot(_bf(a_ref[z + 7 * a + b]), _bf(r_ref[c, 7 * a + b])), TQ, emit)

        def fin(quad, q, v):
            i, j = 2 * (quad // 2) + q // 2, 2 * (quad % 2) + q % 2
            v = v + _dot(_bf(at_ref[z + i]), _bf(t_ref[c, j]))
            hf[z + 4 * quad + q] = v[:, :128] * v[:, 128:]

        def old(s, q):
            return to[z + 4 * s + q]

        def keep(s):
            def emit(q, v):
                to[z + 4 * s + q] = v
            return emit

        def emit3(q, v):
            fin(2, q, old(1, q) + v)
            to[z + 12 + q] = old(0, q) + v

        def emit4(q, v):
            fin(1, q, old(2, q) + v)
            to[z + 12 + q] = old(3, q) - v

        inner(2, keep(2))
        inner(0, keep(0))
        inner(1, keep(1))
        inner(5, lambda q, v: fin(3, q, ((old(0, q) - old(1, q)) + old(2, q)) + v))
        put(4)
        inner(3, emit3)
        put(2)
        inner(4, emit4)
        put(6)
        inner(6, lambda q, v: fin(0, q, old(3, q) + v))

    def down_prod(c, k, prev):
        return prev + lax.dot_general(_bf(l_ref[c, 72 * k:72 * k + 72, :]), _bf(h_ref[k]), NT_DIMS, preferred_element_type=F32)

    def down(c):
        for a, late in ((4, 1), (2, 0), (6, 3), (1, 5), (0, None), (3, None), (5, None)):
            for k in range(7 * a, 7 * a + 7):
                acc[k] = down_prod(c, k, jnp.where(c == 0, 0.0, acc[k]))
            if late is not None:
                put(late)

    def add_stats(st, r, x):
        st[r] = (x, x * x) if st.get(r) is None else (st[r][0] + x, st[r][1] + x * x)

    def mean_rstd(st, r):
        m = jnp.sum(st[r][0], axis=0, keepdims=True) * (1.0 / D)
        v = jnp.sum(st[r][1], axis=0, keepdims=True) * (1.0 / D) - m * m
        return m, lax.rsqrt(jnp.maximum(v, 0.0) + EPS)

    def down_final(base, st, after=None, between=()):
        odd = [False]

        def inner(a, emit, late=None):
            strassen_inner(lambda b: down_prod(NC - 1, 7 * a + b, acc[7 * a + b]), MQ, emit, odd[0] if between else None)
            if late is not None:
                put(late)
            if a in between:
                between[a]()
            else:
                odd[0] = not odd[0]

        def old(s, q):
            return to[z + 4 * s + q, 0:MQ, :]

        def keep(s, q, v):
            to[z + 4 * s + q, 0:MQ, :] = v

        def fin(quad, q, v):
            i, j = 2 * (quad // 2) + q // 2, 2 * (quad % 2) + q % 2
            rows = pl.ds(MQ * i, MQ)
            for e in range(2):
                r = j + 4 * e
                ref, slot = xm[r]
                x = ref[z + slot, rows, :] + v[:, 128 * e:128 * e + 128]
                if st is None:
                    ob[z + r // 2, pl.ds(288 * (r % 2) + 72 * i, 72), :] = _u32(x)
                    continue
                xr[base + r, rows, :] = x
                for g in range(MQ // 8):
                    add_stats(st, r, x[8 * g:8 * g + 8])
            if after is not None and q == 0:
                after(quad)

        inner(4, lambda q, v: keep(0, q, v), 0)
        inner(2, lambda q, v: (fin(1, q, old(0, q) + v), keep(1, q, v)), 3)
        inner(6, lambda q, v: keep(0, q, v - old(0, q)), 1)
        inner(0, lambda q, v: (keep(0, q, old(0, q) + v), keep(1, q, old(1, q) + v)), 5)
        inner(3, lambda q, v: (fin(0, q, old(0, q) + v), keep(2, q, v)))
        inner(1, lambda q, v: (fin(2, q, old(2, q) + v), keep(1, q, old(1, q) - v)))
        inner(5, lambda q, v: fin(3, q, old(1, q) + v))

    def chain(ref, last, v, skew=1):
        last.append(pltpu.bitcast(v, F32))
        if len(last) > skew:
            fence(ref, last.pop(0))

    def ln1_fns(base, mr, pairs):
        def norm(r, row, n):
            return (xr[base + r, pl.ds(row, n), :] - mr[r][0]) * mr[r][1]

        def job(u, g):
            if g == 16:
                y = jnp.concatenate([_u32(norm(2 * u + e, 512, 64)) for e in range(2)], axis=0)
                xn[u, 896:960, :] = y
                return tree(jnp.bitwise_xor, [y[8 * k:8 * k + 8] for k in range(8)])
            y = [_u32(v) for v in _rhs1(*[norm(2 * u + e, 256 * k + 16 * g, 16) for k in range(2) for e in range(2)])]
            for b in range(7):
                xn[u, pl.ds(128 * b + 8 * g, 8), :] = y[b]
            return y[5] ^ y[6]
        return [lambda u=u, g=g: job(u, g) for u in pairs for g in range(17)]

    def project(name, a, u, emit, x=None):
        w = 2 * "qkvo".index(name) + a
        src, slot = (ob, z + u) if name == "o" else (xn, u)
        rows = lambda i, n: src[slot, i:i + n, :] if x is None else x[i:i + n]

        def tick(y):
            clock[0] += 1
            for g in range(DH * (clock[0] % 2)):
                run(ticks, y[8 * g:8 * g + 8, 0:128])
            return y
        m = lambda b: tick(_dot(_bf(wt[w, b]), _bf(rows(128 * b, 128))))
        xt = lambda: _bf(jnp.concatenate([rows(896, 32), rows(928, 32)], axis=1))
        tail = lambda i: tick(_dot(_bf(wt[w, 7, :, 128 * i:128 * i + 64]), xt()))
        ta, m4 = tail(0), m(4)
        s11, s12 = ta[:, :128] - m4, ta[:, 128:] + m4
        s22 = m(2)
        emit(a, 2 * u + 1, s12 + s22)
        s11 = s11 + m(6)
        m0 = m(0)
        s11, s22 = s11 + m0, s22 + m0
        s21 = m(3)
        emit(a, 2 * u, s11 + s21)
        tb = tail(1)
        s21, s22 = s21 + tb[:, :128], s22 + tb[:, 128:]
        m1 = m(1)
        emit(a + 2, 2 * u, s21 + m1)
        emit(a + 2, 2 * u + 1, (s22 - m1) + m(5))

    def project_kv(name, a, u, jobs=(), every=1, x=None):
        def emit(hg, r, y):
            dst, rows = (kb, pl.ds(MQ * hg, MQ)) if name == "k" else (vbs[a], pl.ds(MQ * (hg // 2), MQ))
            dst[z + 7 + r, rows, :] = y
            if r >= 1:
                dst[z + r - 1, rows, :] = pltpu.roll(y, 1, 1)
            for g in range(0, DH, every):
                run(jobs, y[8 * g:8 * g + 8])
        project(name, a, u, emit, x)

    def prow(hg, w):
        return pl.ds(32 * w + 16 * (hg % 2) + 8 * (hg // 2), 8)

    def project_q(a, u, jobs):
        def emit(hg, r, y):
            lg = [None] * W
            for d in range(DH):
                q = y[8 * d:8 * d + 8]
                for w in range(W):
                    v = q * kb[z + 7 + r - w, pl.ds(MQ * hg + 8 * d, 8), :]
                    lg[w] = v if d == 0 else lg[w] + v
            for w in range(W):
                pb[z + r, prow(hg, w), :] = lg[w]
            if hg >= 2:
                jobs.append(softmax_job(r, a))
        project("q", a, u, emit)

    def softmax_job(r, sl):
        def job(v):
            fence(pb, v)
            lane0 = lax.broadcasted_iota(jnp.int32, (16, 128), 1) == 0
            lg = [pb[z2 + r, 32 * w + 16 * sl:32 * w + 16 * sl + 16, :] for w in range(W)]
            lg = [jnp.where(lane0, NEG, lg[w]) if w > r else lg[w] for w in range(W)]
            m = tree(jnp.maximum, lg)
            ex = [jnp.exp2((lg[w] - m) * EXP_C) for w in range(W)]
            inv = 1.0 / tree(jnp.add, ex)
            for w in range(W):
                pb[z2 + r, 32 * w + 16 * sl:32 * w + 16 * sl + 16, :] = ex[w] * inv
        return job

    def mix_jobs(a):
        o = {}

        def job(u, g, i):
            p = [[pb[z2 + 2 * u + e, prow(a + 2 * i, w), :] for w in range(W)] for e in range(2)]
            for d in range(2):
                v = [vbs[a][z2 + 2 * u + t, pl.ds(MQ * i + 16 * g + 8 * d, 8), :] for t in range(W + 1)]
                for e in range(2):
                    o[d, i, e] = tree(jnp.add, [p[e][w] * v[7 + e - w] for w in range(W)])
            if i == 0:
                y = pltpu.bitcast((o[0, 0, 0] + o[0, 0, 1]) + (o[1, 0, 0] + o[1, 0, 1]), U32)
                if (a, u, g) == (0, 0, 0):
                    xn[z, 960:968, :] = y
                return y
            lo, hi = [[o[d, i, e] for i in range(2) for e in range(2)] for d in range(2)]
            if g < 8:
                y = [_pk(*t) for t in zip(_rhs1(*lo), _rhs1(*hi))]
                for b in range(7):
                    ob[z + u, pl.ds(128 * b + 64 * a + 8 * g, 8), :] = y[b]
                return y[5] ^ y[6]
            y = [_pk(*t) for t in zip(lo, hi)]
            for k in range(4):
                ob[z + u, pl.ds(896 + 32 * (k % 2) + 8 * (a + 2 * (k // 2)), 8), :] = y[k]
            return tree(jnp.bitwise_xor, y)
        return paced(vbs[a], [lambda u=u, g=g, i=i: job(u, g, i)
                              for u in range(4) for g in range(9) for i in range(2)], 1)

    def ln2(st, r):
        m, rs = mean_rstd(st, r)
        (ref, slot), last = xm[r], []
        for kt in range(5):
            wk = 128 if kt < 4 else 64
            y = ((ref[z2 + slot, 128 * kt:128 * kt + wk, :] - m) * rs).T
            (xf, xo)[r // 4][z + kt, pl.ds(128 * (r % 4), 128), 0:wk] = y
            if kt < 4:
                chain(ref, last, y[0:8], 2)

    def prep_a_jobs(outer, odd):
        return paced((xf, xo)[odd], [lambda a=a, half=half, g=g: prep_a(a, half, g) for a in outer
                                     for half in range(2) for g in range(4 * odd, 4 * odd + 4)], 2)

    def out_proj(base, st, a, u, jobs):
        def emit(i, r, y):
            for g in range(MQ // 16):
                rows = pl.ds(MQ * i + 16 * g, 16)
                x = xr[base + r, rows, :] + y[16 * g:16 * g + 16]
                xm[r][0][z + xm[r][1], rows, :] = x
                add_stats(st, r, x[0:8])
                add_stats(st, r, x[8:16])
                if (i, r, clock[0] % 2) != (a + 2, 2 * u + 1, 0):
                    run(jobs, x[0:8])
        project("o", a, u, emit)

    def attention_block(p, first):
        s = 0 if first else p % 2
        cur, nxt = 8 * s, 8 * (1 - s)
        st1 = {}
        if first:
            st0 = {}
            for r in range(NT_):
                rows_to_tile(0, r, st0)
            for fn in ln1_fns(0, st0, (0, 1)):
                fn()
            ticks.extend(spread([], 90) + spread([lambda v: fence(xr, v)] + paced(xr, ln1_fns(z2, st0, (2, 3)), 2), 200))
            for u in range(2):
                for a in range(2):
                    project_kv("k", a, u)
            cp_qkv("q").wait()
            cp_qkv("v").wait()
            cp_wo().wait()
            steps = setup_qkv("q")
            for _, fn in steps[:5]:
                fn()
            wo_jobs = [gate(*step) for step in setup_wo()]
            ticks.extend(spread([], 108) + spread([gate(*step) for step in steps[5:]], 216))
            overlay(ticks, 90, 46, wo_jobs[:5])
            for u in range(2, 4):
                for a in range(2):
                    project_kv("k", a, u)
            tiles = [gate(perm, lambda r=r, b=b: rows_to_tile(1, r, st1, (b,))) for r in range(NT_) for b in range(3)]
            steps = [gate(*step) for step in setup_qkv("v")]
            mixed = steps[:5] + tiles[:6] + [job for pair in zip(steps[5:], tiles[6:]) for job in pair]
            ticks.extend(spread([], 36) + spread(mixed, 540))
        else:
            unit = {2: (0, 2), 0: (1, 2), 3: (0, 3), 1: (1, 3)}
            down_final(nxt, st1, None, {g: lambda g=g: project_kv("k", *unit[g]) for g in unit})
            st1 = {r: mean_rstd(st1, r) for r in range(NT_)}
        jobs = []
        for u in range(4):
            for a in range(2):
                project_q(a, u, jobs)
        if first:
            for cp in cp_ffn(0) + cp_tails():
                cp.wait()
        assert not ticks
        clock[0] = 0 if first else 1
        ticks.extend(spread(jobs + [lambda v: fence(pb, v)], 306))
        ln1 = [lambda v: fence(xr, v)] + paced(xr, ln1_fns(z2 + nxt, st1, range(4)), 2)
        for vb in vbs:
            prime(vb, ob)
        prime(xf, a_ref)
        prime(xo, a_ref)
        x0 = xn[0, 0:960, :]
        overlay(ticks, 93, 12, ln1[:18])
        if first:
            overlay(ticks, 50, 14, wo_jobs[5:])
        for u in range(4):
            project_kv("v", 0, u)
        assert not ticks
        ticks.extend(spread([], 24) + spread(mix_jobs(0), 300))
        for u in range(4):
            project_kv("v", 1, u, x=x0 if u == 0 else None)
        assert not ticks
        ticks.extend(spread([], 24) + spread(mix_jobs(1), 300))
        for a in range(2):
            project_kv("k", a, 0)
        st2, jobs = {}, []
        for u in range(4):
            if u == 1:
                jobs = spread(ln1[18:], 126)
            if u == 2:
                assert not ticks
                ticks.extend(spread([], 81) + spread(prep_a_jobs(G_ORDER, 0), 219) + spread(prep_a_jobs((2,), 1), 24))
            for a in range(2):
                out_proj(cur, st2, a, u, jobs)
            ln2(st2, 2 * u)
            ln2(st2, 2 * u + 1)
        assert not jobs and not ticks
        last = []
        project_kv("k", 0, 1)
        project_kv("k", 1, 1, [last.append])
        for a in G_ORDER[1:]:
            for half in range(2):
                for g in range(4, 8):
                    chain(xo, last, prep_a(a, half, g))
        prep_a_tail()
        gate_up(0, first)

    def ffn_loop(first):
        def body(c, carry):
            if first:
                for cp in cp_ffn(c + 1):
                    cp.wait()

                @pl.when(c + RING < NC)
                def _():
                    for cp in cp_ffn(c + RING):
                        cp.start()
            down(c)
            gate_up(c + 1, first)
            return carry
        lax.fori_loop(0, NC - 1, body, 0)

    cp_qkv("k").start()
    for u in range(4):
        cp_x(u).start()
    for cp in (cp_qkv("q"), cp_qkv("v"), cp_wo()) + cp_ffn(0) + cp_tails() + cp_ffn(1) + cp_ffn(2):
        cp.start()
    cp_qkv("k").wait()
    for _, fn in setup_qkv("k"):
        fn()
    for u in range(4):
        cp_x(u).wait()
        for t in range(X_SPLIT[u], X_SPLIT[u + 1]):
            x_to_rows(t)

    attention_block(0, True)
    ffn_loop(True)

    def pass_body(p, carry):
        attention_block(p, False)
        ffn_loop(False)
        return carry
    lax.fori_loop(1, 4, pass_body, 0)

    for b in range(3):
        tiles_to_rows(b, 0, range(NT_))

    def after(quad):
        tiles = [2 * (quad % 2) + t for t in (0, 1, 4, 5)]
        slabs = ((0,), (2, 1))[quad // 2]
        for b in slabs:
            tiles_to_rows(b, 1, tiles)
        if quad in (0, 3):
            for b in slabs:
                rows_to_out(b)
    down_final(None, None, after)
    for b, u in [(b, u) for b in range(2) for u in range(4)] + [(2, 0)]:
        cp_out(b, u).wait()


@jax.jit
def pallas_interleave_layers__sliding_local_dilated__glu_gated_bilinear__prompt_kernel(
    A_x: jax.Array,
    A_wqkv: jax.Array,
    A_wo: jax.Array,
    B_x: jax.Array,
    B_w_gate: jax.Array,
    B_w_up: jax.Array,
    B_w_down: jax.Array,
):
    del B_x
    vm = pltpu.VMEM
    scratch = [
        vm((D, S), BF), vm((D + 32, 3 * D), BF), vm((D + 64, D), BF),
        vm((RING, 512, FC), BF), vm((RING, 512, FC), BF), vm((RING, D, FC), BF),
        vm((D - 512, F), BF), vm((D - 512, F), BF),
        vm((6, 640, 128), F32),
        vm((8, 8, MQ // 2, 256), U32),
        vm((2 * NT_ + 1, D, 128), F32),
        vm((5, D, 128), F32),
        vm((5, D, 128), F32),
        vm((4, 992, 128), U32),
        vm((15, D, 128), F32),
        vm((16, D // 2, 128), F32),
        vm((16, D // 2, 128), F32),
        vm((NT_ + 1, W * H, 128), F32),
        vm((4, 960, 128), U32),
        vm((6, D, 128), F32),
        vm((6, S // 4, 128), F32),
        vm((49 * 128 + 32, 128), F32),
        vm((49, TQ // 2, 128), U32),
        vm((4, TQ // 2, 64), U32),
        vm((49, MQ, TQ), F32),
        vm((49, TQ // 2, 128), U32),
        vm((4, TQ, 256), F32),
        vm((16, TQ, 256), F32),
        vm((16, TQ, 128), F32),
        vm((NC, 49, 64, 256), U32),
        vm((NC, 3552, 128), U32),
        vm((NC, 4, 32, 256), U32),
        pltpu.SMEM((2,), jnp.int32),
        pltpu.SemaphoreType.DMA((11 + 3 * RING,)),
    ]
    hbm = pl.BlockSpec(memory_space=pl.ANY)
    out = pl.pallas_call(
        _kernel,
        in_specs=[hbm] * 6,
        out_specs=hbm,
        out_shape=jax.ShapeDtypeStruct((D, S), BF),
        scratch_shapes=scratch,
        compiler_params=pltpu.CompilerParams(vmem_limit_bytes=126 * 1024 * 1024),
    )(A_x.reshape(S, D).T, A_wqkv, A_wo, B_w_gate, B_w_up, B_w_down.T)
    return out.T.reshape(1, S, D)
```

```python
import math

import jax
import jax.numpy as jnp
from jax import lax
import jax.experimental.pallas as pl
import jax.experimental.pallas.tpu as pltpu

S, D, F = 2048, 576, 4608
H, DH, W = 32, 18, 8
NT_ = 8
TQ = 256
MQ = D // 4
FC = 512
NC = F // FC
X_SPLIT = (0, 5, 10, 14, 16)
EPS = 1e-5
SCALE = DH ** -0.5
EXP_C = SCALE * math.log2(math.e)
NEG = -1e9 / SCALE

BF, F32, U32 = jnp.bfloat16, jnp.float32, jnp.uint32
NT_DIMS = (((1,), (1,)), ((), ()))

LHS_SEL = {0: ((0, 0), 1, (1, 1)), 1: ((1, 0), 1, (1, 1)), 2: ((0, 0), 0, None), 3: ((1, 1), 0, None),
           4: ((0, 0), 1, (0, 1)), 5: ((1, 0), -1, (0, 0)), 6: ((0, 1), -1, (1, 1))}
RHS_SEL = {0: ((0, 0), 1, (1, 1)), 1: ((0, 0), 0, None), 2: ((0, 1), -1, (1, 1)), 3: ((1, 0), -1, (0, 0)),
           4: ((1, 1), 0, None), 5: ((0, 0), 1, (0, 1)), 6: ((1, 0), 1, (1, 1))}
G_ORDER = (2, 0, 1, 5, 3, 4, 6)


def _lhs1(a11, a12, a21, a22):
    return [a11 + a22, a21 + a22, a11, a22, a11 + a12, a21 - a11, a12 - a22]


def _rhs1(b11, b12, b21, b22):
    return [b11 + b22, b11, b12 - b22, b21 - b11, b22, b11 + b12, b21 + b22]


def _in2(fn, x):
    outer = [[fn(x[i][j], x[i][2 + j], x[2 + i][j], x[2 + i][2 + j]) for j in range(2)] for i in range(2)]
    return [v for a in range(7) for v in fn(outer[0][0][a], outer[0][1][a], outer[1][0][a], outer[1][1][a])]


def _select(sel, load):
    first, sign, second = sel
    v = load(first)
    if sign == 1:
        v = [a + b for a, b in zip(v, load(second))]
    elif sign == -1:
        v = [a - b for a, b in zip(v, load(second))]
    return v


def _pk(lo, hi):
    return pltpu.pack_elementwise([lo, hi], packed_dtype=BF)


def _lo(w):
    return pltpu.unpack_elementwise(w, index=0, packed_dtype=BF, unpacked_dtype=F32)


def _hi(w):
    return pltpu.unpack_elementwise(w, index=1, packed_dtype=BF, unpacked_dtype=F32)


def _bf(w):
    return pltpu.bitcast(w, BF)


def _u32(x):
    return pltpu.bitcast(x.astype(BF), U32)


def _dot(a, b):
    return jnp.dot(a, b, preferred_element_type=F32)


def _kernel(x_hbm, wqkv_hbm, wo_hbm, wg_hbm, wu_hbm, wd_hbm, out_hbm,
            xio, wqkv_raw, wo_raw, wg_raw, wu_raw, wd_raw, tg, tu,
            wts, wt, xr, xm0, xm1, xn, kb, vb0, vb1, pb, ob, xf, xo, perm,
            a_ref, at_ref, acc, h_ref, ti, to, hf, r_ref, l_ref, t_ref, zero_ref, sems):
    def clear(i, carry):
        zero_ref[i] = 0
        return carry
    lax.fori_loop(0, 2, clear, 0)
    z = zero_ref[0]
    z2 = zero_ref[1]
    vbs = (vb0, vb1)
    ticks, clock = [], [0]
    xm = [((xm0, xm1)[r // 2 % 2], r // 4 * 2 + r % 2) for r in range(NT_)]

    def fence(ref, v):
        ref[z + (ref.shape[0] - 1), 0:8, 0:128] = v

    def gate(ref, fn):
        def job(v):
            if len(ref.shape) == 3:
                fence(ref, v)
            else:
                rows = pl.ds(pl.multiple_of(16 * z + (ref.shape[0] - 16), 16), 16)
                ref[rows, 0:128] = jnp.concatenate([v, v], axis=0).astype(ref.dtype)
            fn()
        return job

    def prime(ref, other):
        ref[z2 + (ref.shape[0] - 1), 0:8, 0:128] = pltpu.bitcast(other[z, 0:8, 0:128], F32)

    def paced(ref, fns, skew):
        last = []

        def job(v, fn):
            last.append(fn())
            if len(last) > skew:
                v = pltpu.bitcast(last.pop(0) ^ pltpu.bitcast(v, U32), F32)
            fence(ref, v)
        return [lambda v, fn=fn: job(v, fn) for fn in fns]

    def spread(jobs, n):
        slots = [lambda v: None] * n
        for i, job in enumerate(jobs):
            slots[i * n // len(jobs)] = job
        return slots

    def overlay(slots, start, step, jobs):
        for i, job in enumerate(jobs):
            k = start + step * i
            slots[k] = lambda v, old=slots[k], job=job: (old(v), job(v))

    def run(jobs, v, n=1):
        for _ in range(n):
            if jobs:
                jobs.pop(0)(v)

    def tree(fn, v):
        while len(v) > 1:
            v = [fn(v[i], v[i + 1]) for i in range(0, len(v), 2)]
        return v[0]

    def cp_x(u):
        cols = pl.ds(128 * X_SPLIT[u], 128 * (X_SPLIT[u + 1] - X_SPLIT[u]))
        return pltpu.make_async_copy(x_hbm.at[:, cols], xio.at[:, cols], sems.at[u])

    def cp_out(b, u):
        rows, cols = (pl.ds(256 * b, 256), pl.ds(512 * u, 512)) if b < 2 else (pl.ds(512, 64), pl.ds(0, S))
        return pltpu.make_async_copy(xio.at[rows, cols], out_hbm.at[rows, cols], sems.at[4 * b + u])

    qkv_cols = {"k": pl.ds(512, 640), "v": pl.ds(1152, 576), "q": pl.ds(0, 512)}

    def cp_qkv(name):
        idx = 5 + "kvq".index(name)
        return pltpu.make_async_copy(wqkv_hbm.at[:, qkv_cols[name]], wqkv_raw.at[0:D, qkv_cols[name]], sems.at[idx])

    def cp_wo():
        return pltpu.make_async_copy(wo_hbm, wo_raw.at[0:D], sems.at[8])

    def cp_ffn(c):
        c0 = c * FC if isinstance(c, int) else pl.multiple_of(c * FC, FC)
        cols = pl.ds(c0, FC)
        return (pltpu.make_async_copy(wg_hbm.at[0:512, cols], wg_raw.at[c], sems.at[11 + 3 * c]),
                pltpu.make_async_copy(wu_hbm.at[0:512, cols], wu_raw.at[c], sems.at[12 + 3 * c]),
                pltpu.make_async_copy(wd_hbm.at[:, cols], wd_raw.at[c], sems.at[13 + 3 * c]))

    def cp_tails():
        return (pltpu.make_async_copy(wg_hbm.at[512:D, :], tg, sems.at[9]),
                pltpu.make_async_copy(wu_hbm.at[512:D, :], tu, sems.at[10]))

    def combine_steps(part, ref, rows):
        def combine(a, g):
            for j in range(2):
                w = _lhs1(rows(a, j, g), rows(a, 2 + j, g), rows(a + 2, j, g), rows(a + 2, 2 + j, g))
                for b in range(7):
                    wt[2 * part + a, b, 8 * g:8 * g + 8, 128 * j:128 * j + 128] = _u32(w[b])
                wt[2 * part + a, 7, 8 * g:8 * g + 8, 128 * j:128 * j + 64] = _u32(rows(a + 2 * j, 4, g)[:, :64])
        return [(ref, lambda a=a, g=g: combine(a, g)) for a in range(2) for g in range(MQ // 16)]

    def setup_qkv(name):
        part = "qkv".index(name)
        nb0 = (D * part) // 128
        base = D * part - 128 * nb0

        def transpose(nb):
            wn = min(128, D * part + D - 128 * nb)
            for kt in range(5):
                wk = 128 if kt < 4 else 64
                blk = wqkv_raw[128 * kt:128 * kt + wk, 128 * nb:128 * nb + wn].astype(F32)
                wts[kt, 128 * (nb - nb0):128 * (nb - nb0) + wn, 0:wk] = blk.T

        def rows(hg, kt, g):
            return jnp.concatenate([wts[kt, pl.ds(base + MQ * hg + 2 * g + e, 8, stride=DH), :]
                                    for e in range(2)], axis=0)
        return [(wqkv_raw, lambda nb=nb: transpose(nb)) for nb in range(nb0, nb0 + 5)] + combine_steps(part, wts, rows)

    def setup_wo():
        def transpose(nb):
            wn = 128 if nb < 4 else 64
            xf[nb, 0:D, 0:wn] = wo_raw[0:D, 128 * nb:128 * nb + wn].astype(F32)
            pair = [[_pk(*[xf[nb, pl.ds(MQ * hg + d + e, 8, stride=DH), :][:, :wn] for e in range(2)])
                     for d in range(0, DH, 2)] for hg in range(4)]
            for kt in range(5):
                w = pair[kt][:8] if kt < 4 else [pair[hg][8] for hg in range(4)]
                blk = _bf(jnp.concatenate(w, axis=0)).astype(F32).T
                hf[3 * kt + nb // 2, pl.ds(128 * (nb % 2), wn), 0:blk.shape[1]] = blk

        def rows(i, kt, g):
            row = MQ * i + 16 * g
            return hf[3 * kt + row // 256, pl.ds(row % 256, 16), :]
        return [(wo_raw, lambda nb=nb: transpose(nb)) for nb in range(5)] + combine_steps(3, hf, rows)

    def x_to_rows(t):
        x = xio[:, 128 * t:128 * t + 128]
        st, xs = {}, x.astype(F32)
        for g in range(D // 8):
            add_stats(st, g % 2, xs[8 * g:8 * g + 8])
        m, rs = mean_rstd({0: (st[0][0] + st[1][0], st[0][1] + st[1][1])}, 0)
        stat = jnp.where(lax.broadcasted_iota(jnp.int32, (32, 128), 0) == 0, m, rs)
        words = pltpu.bitcast(x, F32)
        for b in range(3):
            if b < 2:
                w = words[128 * b:128 * b + 128].T
            else:
                w = jnp.concatenate([words[256:288], stat], axis=0).T
                w = jnp.concatenate([w, jnp.zeros((128, 64), F32)], axis=1)
            for jj in range(8):
                perm[pl.ds(49 * (8 * t + jj) + b, 16, stride=3), :] = w[16 * jj:16 * jj + 16]

    def rows_to_tile(s, r, mr, slabs=range(3)):
        for b in slabs:
            w = perm[pl.ds(3 * (2 * r + s) + b, 128, stride=49), :]
            if b < 2:
                xr[8 * s + r, 256 * b:256 * b + 256, :] = _bf(w.T).astype(F32)
            else:
                w = w[:, :64].T
                xr[8 * s + r, 512:D, :] = _bf(w[0:32]).astype(F32)
                mr[r] = (w[32:33], w[33:34])

    def tiles_to_rows(b, s, tiles):
        nw = 128 if b < 2 else 32
        for r in tiles:
            if s == 0:
                w = _pk(xr[r, pl.ds(256 * b, nw, stride=2), :], xr[r, pl.ds(256 * b + 1, nw, stride=2), :])
            else:
                w = ob[z + r // 2, pl.ds(288 * (r % 2) + 128 * b, nw), :]
            w = jnp.concatenate([pltpu.bitcast(w, F32)] * (128 // nw), axis=0)
            perm[pl.ds(3 * (2 * r + s) + b, 128, stride=49), :] = w.T

    def rows_to_out(b):
        def rows(t):
            return jnp.concatenate([perm[pl.ds(49 * (8 * t + jj) + b, 16, stride=3), :] for jj in range(8)], axis=0)
        group = lax.broadcasted_iota(jnp.int32, (128, 128), 1) // 32
        for u in range(4):
            if b < 2:
                for t in range(4 * u, 4 * u + 4):
                    xio[256 * b:256 * b + 256, 128 * t:128 * t + 128] = _bf(rows(t).T)
                cp_out(b, u).start()
            else:
                w = rows(4 * u)
                for t in range(1, 4):
                    w = jnp.where(group == t, rows(4 * u + t), w)
                w = _bf(w.T)
                for t in range(4):
                    xio[512:D, pl.ds(128 * (4 * u + t), 128)] = w[64 * t:64 * t + 64]
        if b == 2:
            cp_out(b, 0).start()

    def prep_r(c, a):
        for u in range(2):
            for g in range(8):
                def load(quad):
                    ws = [pltpu.bitcast((wg_raw, wu_raw)[u][c, pl.ds(128 * (2 * quad[0] + i) + 16 * g, 16),
                                                            pl.ds(256 * quad[1], 256)], U32) for i in range(2)]
                    ws = [w[:, 128 * j:128 * j + 128] for w in ws for j in range(2)]
                    return [_lo(w) for w in ws] + [_hi(w) for w in ws]
                v = _select(RHS_SEL[a], load)
                for b, (lo, hi) in enumerate(zip(_rhs1(*v[:4]), _rhs1(*v[4:]))):
                    r_ref[c, 7 * a + b, 8 * g:8 * g + 8, 128 * u:128 * u + 128] = _pk(lo, hi)

    def prep_l(c, g):
        ws = [pltpu.bitcast(wd_raw[c, pl.ds(MQ * i + 16 * g, 16), :], U32) for i in range(4)]
        ws = [[w[:, 128 * j:128 * j + 128] for j in range(4)] for w in ws]
        lo = _in2(_lhs1, [[_lo(w) for w in row] for row in ws])
        hi = _in2(_lhs1, [[_hi(w) for w in row] for row in ws])
        for k in range(49):
            l_ref[c, pl.ds(72 * k + 8 * g, 8), :] = _pk(lo[k], hi[k])

    def prep_a(a, half, g):
        src, row = (xf, xo)[g // 4], 32 * (g % 4) + half

        def load(quad):
            return [src[z2 + 2 * quad[1] + j, pl.ds(128 * (2 * quad[0] + i) + row + e, 8, stride=4), :]
                    for e in (0, 2) for i in range(2) for j in range(2)]
        v = _select(LHS_SEL[a], load)
        o = [_pk(lo, hi) for lo, hi in zip(_lhs1(*v[:4]), _lhs1(*v[4:]))]
        for b in range(7):
            a_ref[z + 7 * a + b, 64 * half + 8 * g:64 * half + 8 * g + 8, :] = o[b]
        return o[5] ^ o[6]

    def prep_a_tail():
        for i in range(4):
            for half in range(2):
                for u, src in enumerate((xf, xo)):
                    lo = src[z + 4, pl.ds(128 * i + half, 32, stride=4), :][:, :64]
                    hi = src[z + 4, pl.ds(128 * i + half + 2, 32, stride=4), :][:, :64]
                    at_ref[z + i, pl.ds(64 * half + 32 * u, 32), :] = _pk(lo, hi)

    def put(a):
        for g in range(16):
            def load(quad):
                return [hf[z + 4 * (2 * quad[1] + quad[0]) + t, pl.ds(o + 8 * g, 8), :]
                        for o in (0, 128) for t in (0, 2, 1, 3)]
            v = _select(RHS_SEL[a], load)
            for b, (lo, hi) in enumerate(zip(_rhs1(*v[:4]), _rhs1(*v[4:]))):
                h_ref[7 * a + b, 8 * g:8 * g + 8, :] = _pk(lo, hi)

    def strassen_inner(prod, nrow, emit, odd=None):
        ld = lambda s: ti[z + s, 0:nrow, :]
        for s in range(3):
            ti[z + s, 0:nrow, :] = prod(s)
        if not odd:
            emit(3, ((ld(0) - ld(1)) + ld(2)) + prod(5))
        m3 = prod(3)
        emit(2, ld(1) + m3)
        if odd is None:
            ti[z + 3, 0:nrow, :] = ld(0) + m3
        m4 = prod(4)
        emit(1, ld(2) + m4)
        ti[z + 3, 0:nrow, :] = (ld(3) if odd is None else ld(0) + m3) - m4
        if odd:
            emit(3, ((ld(0) - ld(1)) + ld(2)) + prod(5))
        emit(0, ld(3) + prod(6))

    def gate_up(c, first):
        if first:
            c0 = c * FC if isinstance(c, int) else pl.multiple_of(c * FC, FC)
            for g in range(MQ // 16):
                prep_l(c, g)
            for j in range(4):
                cols = pl.ds(c0 + 128 * j, 128)
                t_ref[c, j] = pltpu.bitcast(jnp.concatenate([tg[:, cols], tu[:, cols]], axis=1), U32)

        def inner(a, emit):
            if first:
                prep_r(c, a)
            strassen_inner(lambda b: _dot(_bf(a_ref[z + 7 * a + b]), _bf(r_ref[c, 7 * a + b])), TQ, emit)

        def fin(quad, q, v):
            i, j = 2 * (quad // 2) + q // 2, 2 * (quad % 2) + q % 2
            v = v + _dot(_bf(at_ref[z + i]), _bf(t_ref[c, j]))
            hf[z + 4 * quad + q] = v[:, :128] * v[:, 128:]

        def old(s, q):
            return to[z + 4 * s + q]

        def keep(s):
            def emit(q, v):
                to[z + 4 * s + q] = v
            return emit

        def emit3(q, v):
            fin(2, q, old(1, q) + v)
            to[z + 12 + q] = old(0, q) + v

        def emit4(q, v):
            fin(1, q, old(2, q) + v)
            to[z + 12 + q] = old(3, q) - v

        inner(2, keep(2))
        inner(0, keep(0))
        inner(1, keep(1))
        inner(5, lambda q, v: fin(3, q, ((old(0, q) - old(1, q)) + old(2, q)) + v))
        put(4)
        inner(3, emit3)
        put(2)
        inner(4, emit4)
        put(6)
        inner(6, lambda q, v: fin(0, q, old(3, q) + v))

    def down_prod(c, k, prev):
        return prev + lax.dot_general(_bf(l_ref[c, 72 * k:72 * k + 72, :]), _bf(h_ref[k]), NT_DIMS, preferred_element_type=F32)

    def down(c):
        for a, late in ((4, 1), (2, 0), (6, 3), (1, 5), (0, None), (3, None), (5, None)):
            for k in range(7 * a, 7 * a + 7):
                acc[k] = down_prod(c, k, jnp.where(c == 0, 0.0, acc[k]))
            if late is not None:
                put(late)

    def add_stats(st, r, x):
        st[r] = (x, x * x) if st.get(r) is None else (st[r][0] + x, st[r][1] + x * x)

    def mean_rstd(st, r):
        m = jnp.sum(st[r][0], axis=0, keepdims=True) * (1.0 / D)
        v = jnp.sum(st[r][1], axis=0, keepdims=True) * (1.0 / D) - m * m
        return m, lax.rsqrt(jnp.maximum(v, 0.0) + EPS)

    def down_final(base, st, after=None, between=()):
        odd = [False]

        def inner(a, emit, late=None):
            strassen_inner(lambda b: down_prod(NC - 1, 7 * a + b, acc[7 * a + b]), MQ, emit, odd[0] if between else None)
            if late is not None:
                put(late)
            if a in between:
                between[a]()
            else:
                odd[0] = not odd[0]

        def old(s, q):
            return to[z + 4 * s + q, 0:MQ, :]

        def keep(s, q, v):
            to[z + 4 * s + q, 0:MQ, :] = v

        def fin(quad, q, v):
            i, j = 2 * (quad // 2) + q // 2, 2 * (quad % 2) + q % 2
            rows = pl.ds(MQ * i, MQ)
            for e in range(2):
                r = j + 4 * e
                ref, slot = xm[r]
                x = ref[z + slot, rows, :] + v[:, 128 * e:128 * e + 128]
                if st is None:
                    ob[z + r // 2, pl.ds(288 * (r % 2) + 72 * i, 72), :] = _u32(x)
                    continue
                xr[base + r, rows, :] = x
                for g in range(MQ // 8):
                    add_stats(st, r, x[8 * g:8 * g + 8])
            if after is not None and q == 0:
                after(quad)

        inner(4, lambda q, v: keep(0, q, v), 0)
        inner(2, lambda q, v: (fin(1, q, old(0, q) + v), keep(1, q, v)), 3)
        inner(6, lambda q, v: keep(0, q, v - old(0, q)), 1)
        inner(0, lambda q, v: (keep(0, q, old(0, q) + v), keep(1, q, old(1, q) + v)), 5)
        inner(3, lambda q, v: (fin(0, q, old(0, q) + v), keep(2, q, v)))
        inner(1, lambda q, v: (fin(2, q, old(2, q) + v), keep(1, q, old(1, q) - v)))
        inner(5, lambda q, v: fin(3, q, old(1, q) + v))

    def chain(ref, last, v, skew=1):
        last.append(pltpu.bitcast(v, F32))
        if len(last) > skew:
            fence(ref, last.pop(0))

    def ln1_fns(base, mr, pairs):
        def norm(r, row, n):
            return (xr[base + r, pl.ds(row, n), :] - mr[r][0]) * mr[r][1]

        def job(u, g):
            if g == 16:
                y = jnp.concatenate([_u32(norm(2 * u + e, 512, 64)) for e in range(2)], axis=0)
                xn[u, 896:960, :] = y
                return tree(jnp.bitwise_xor, [y[8 * k:8 * k + 8] for k in range(8)])
            y = [_u32(v) for v in _rhs1(*[norm(2 * u + e, 256 * k + 16 * g, 16) for k in range(2) for e in range(2)])]
            for b in range(7):
                xn[u, pl.ds(128 * b + 8 * g, 8), :] = y[b]
            return y[5] ^ y[6]
        return [lambda u=u, g=g: job(u, g) for u in pairs for g in range(17)]

    def project(name, a, u, emit, x=None):
        w = 2 * "qkvo".index(name) + a
        src, slot = (ob, z + u) if name == "o" else (xn, u)
        rows = lambda i, n: src[slot, i:i + n, :] if x is None else x[i:i + n]

        def tick(y):
            clock[0] += 1
            for g in range(DH * (clock[0] % 2)):
                run(ticks, y[8 * g:8 * g + 8, 0:128])
            return y
        m = lambda b: tick(_dot(_bf(wt[w, b]), _bf(rows(128 * b, 128))))
        xt = lambda: _bf(jnp.concatenate([rows(896, 32), rows(928, 32)], axis=1))
        tail = lambda i: tick(_dot(_bf(wt[w, 7, :, 128 * i:128 * i + 64]), xt()))
        ta, m4 = tail(0), m(4)
        s11, s12 = ta[:, :128] - m4, ta[:, 128:] + m4
        s22 = m(2)
        emit(a, 2 * u + 1, s12 + s22)
        s11 = s11 + m(6)
        m0 = m(0)
        s11, s22 = s11 + m0, s22 + m0
        s21 = m(3)
        emit(a, 2 * u, s11 + s21)
        tb = tail(1)
        s21, s22 = s21 + tb[:, :128], s22 + tb[:, 128:]
        m1 = m(1)
        emit(a + 2, 2 * u, s21 + m1)
        emit(a + 2, 2 * u + 1, (s22 - m1) + m(5))

    def project_kv(name, a, u, jobs=(), every=1, x=None):
        def emit(hg, r, y):
            dst, rows = (kb, pl.ds(MQ * hg, MQ)) if name == "k" else (vbs[a], pl.ds(MQ * (hg // 2), MQ))
            dst[z + 7 + r, rows, :] = y
            if r >= 1:
                dst[z + r - 1, rows, :] = pltpu.roll(y, 1, 1)
            for g in range(0, DH, every):
                run(jobs, y[8 * g:8 * g + 8])
        project(name, a, u, emit, x)

    def prow(hg, w):
        return pl.ds(32 * w + 16 * (hg % 2) + 8 * (hg // 2), 8)

    def project_q(a, u, jobs):
        def emit(hg, r, y):
            lg = [None] * W
            for d in range(DH):
                q = y[8 * d:8 * d + 8]
                for w in range(W):
                    v = q * kb[z + 7 + r - w, pl.ds(MQ * hg + 8 * d, 8), :]
                    lg[w] = v if d == 0 else lg[w] + v
            for w in range(W):
                pb[z + r, prow(hg, w), :] = lg[w]
            if hg >= 2:
                jobs.append(softmax_job(r, a))
        project("q", a, u, emit)

    def softmax_job(r, sl):
        def job(v):
            fence(pb, v)
            lane0 = lax.broadcasted_iota(jnp.int32, (16, 128), 1) == 0
            lg = [pb[z2 + r, 32 * w + 16 * sl:32 * w + 16 * sl + 16, :] for w in range(W)]
            lg = [jnp.where(lane0, NEG, lg[w]) if w > r else lg[w] for w in range(W)]
            m = tree(jnp.maximum, lg)
            ex = [jnp.exp2((lg[w] - m) * EXP_C) for w in range(W)]
            inv = 1.0 / tree(jnp.add, ex)
            for w in range(W):
                pb[z2 + r, 32 * w + 16 * sl:32 * w + 16 * sl + 16, :] = ex[w] * inv
        return job

    def mix_jobs(a):
        o = {}

        def job(u, g, i):
            p = [[pb[z2 + 2 * u + e, prow(a + 2 * i, w), :] for w in range(W)] for e in range(2)]
            for d in range(2):
                v = [vbs[a][z2 + 2 * u + t, pl.ds(MQ * i + 16 * g + 8 * d, 8), :] for t in range(W + 1)]
                for e in range(2):
                    o[d, i, e] = tree(jnp.add, [p[e][w] * v[7 + e - w] for w in range(W)])
            if i == 0:
                y = pltpu.bitcast((o[0, 0, 0] + o[0, 0, 1]) + (o[1, 0, 0] + o[1, 0, 1]), U32)
                if (a, u, g) == (0, 0, 0):
                    xn[z, 960:968, :] = y
                return y
            lo, hi = [[o[d, i, e] for i in range(2) for e in range(2)] for d in range(2)]
            if g < 8:
                y = [_pk(*t) for t in zip(_rhs1(*lo), _rhs1(*hi))]
                for b in range(7):
                    ob[z + u, pl.ds(128 * b + 64 * a + 8 * g, 8), :] = y[b]
                return y[5] ^ y[6]
            y = [_pk(*t) for t in zip(lo, hi)]
            for k in range(4):
                ob[z + u, pl.ds(896 + 32 * (k % 2) + 8 * (a + 2 * (k // 2)), 8), :] = y[k]
            return tree(jnp.bitwise_xor, y)
        return paced(vbs[a], [lambda u=u, g=g, i=i: job(u, g, i)
                              for u in range(4) for g in range(9) for i in range(2)], 1)

    def ln2(st, r):
        m, rs = mean_rstd(st, r)
        (ref, slot), last = xm[r], []
        for kt in range(5):
            wk = 128 if kt < 4 else 64
            y = ((ref[z2 + slot, 128 * kt:128 * kt + wk, :] - m) * rs).T
            (xf, xo)[r // 4][z + kt, pl.ds(128 * (r % 4), 128), 0:wk] = y
            if kt < 4:
                chain(ref, last, y[0:8], 2)

    def prep_a_jobs(outer, odd):
        return paced((xf, xo)[odd], [lambda a=a, half=half, g=g: prep_a(a, half, g) for a in outer
                                     for half in range(2) for g in range(4 * odd, 4 * odd + 4)], 2)

    def out_proj(base, st, a, u, jobs):
        def emit(i, r, y):
            for g in range(MQ // 16):
                rows = pl.ds(MQ * i + 16 * g, 16)
                x = xr[base + r, rows, :] + y[16 * g:16 * g + 16]
                xm[r][0][z + xm[r][1], rows, :] = x
                add_stats(st, r, x[0:8])
                add_stats(st, r, x[8:16])
                if (i, r, clock[0] % 2) != (a + 2, 2 * u + 1, 0):
                    run(jobs, x[0:8])
        project("o", a, u, emit)

    def attention_block(p, first):
        s = 0 if first else p % 2
        cur, nxt = 8 * s, 8 * (1 - s)
        st1 = {}
        if first:
            st0 = {}
            for r in range(NT_):
                rows_to_tile(0, r, st0)
            for fn in ln1_fns(0, st0, (0, 1)):
                fn()
            ticks.extend(spread([], 90) + spread([lambda v: fence(xr, v)] + paced(xr, ln1_fns(z2, st0, (2, 3)), 2), 200))
            for u in range(2):
                for a in range(2):
                    project_kv("k", a, u)
            cp_qkv("q").wait()
            cp_qkv("v").wait()
            cp_wo().wait()
            steps = setup_qkv("q")
            for _, fn in steps[:5]:
                fn()
            wo_jobs = [gate(*step) for step in setup_wo()]
            ticks.extend(spread([], 108) + spread([gate(*step) for step in steps[5:]], 216))
            overlay(ticks, 90, 46, wo_jobs[:5])
            for u in range(2, 4):
                for a in range(2):
                    project_kv("k", a, u)
            tiles = [gate(perm, lambda r=r, b=b: rows_to_tile(1, r, st1, (b,))) for r in range(NT_) for b in range(3)]
            steps = [gate(*step) for step in setup_qkv("v")]
            mixed = steps[:5] + tiles[:6] + [job for pair in zip(steps[5:], tiles[6:]) for job in pair]
            ticks.extend(spread([], 36) + spread(mixed, 540))
        else:
            unit = {2: (0, 2), 0: (1, 2), 3: (0, 3), 1: (1, 3)}
            down_final(nxt, st1, None, {g: lambda g=g: project_kv("k", *unit[g]) for g in unit})
            st1 = {r: mean_rstd(st1, r) for r in range(NT_)}
        jobs = []
        for u in range(4):
            for a in range(2):
                project_q(a, u, jobs)
        if first:
            for cp in cp_ffn(0) + cp_tails():
                cp.wait()
        assert not ticks
        clock[0] = 0 if first else 1
        ticks.extend(spread(jobs + [lambda v: fence(pb, v)], 306))
        ln1 = [lambda v: fence(xr, v)] + paced(xr, ln1_fns(z2 + nxt, st1, range(4)), 2)
        for vb in vbs:
            prime(vb, ob)
        prime(xf, a_ref)
        prime(xo, a_ref)
        x0 = xn[0, 0:960, :]
        overlay(ticks, 93, 12, ln1[:18])
        if first:
            overlay(ticks, 50, 14, wo_jobs[5:])
        for u in range(4):
            project_kv("v", 0, u)
        assert not ticks
        ticks.extend(spread([], 24) + spread(mix_jobs(0), 300))
        for u in range(4):
            project_kv("v", 1, u, x=x0 if u == 0 else None)
        assert not ticks
        ticks.extend(spread([], 24) + spread(mix_jobs(1), 300))
        for a in range(2):
            project_kv("k", a, 0)
        st2, jobs = {}, []
        for u in range(4):
            if u == 1:
                jobs = spread(ln1[18:], 126)
            if u == 2:
                assert not ticks
                ticks.extend(spread([], 81) + spread(prep_a_jobs(G_ORDER, 0), 219) + spread(prep_a_jobs((2,), 1), 24))
            for a in range(2):
                out_proj(cur, st2, a, u, jobs)
            ln2(st2, 2 * u)
            ln2(st2, 2 * u + 1)
        assert not jobs and not ticks
        last = []
        project_kv("k", 0, 1)
        project_kv("k", 1, 1, [last.append])
        for a in G_ORDER[1:]:
            for half in range(2):
                for g in range(4, 8):
                    chain(xo, last, prep_a(a, half, g))
        prep_a_tail()
        gate_up(0, first)

    def ffn_loop(first):
        def body(c, carry):
            if first:
                for cp in cp_ffn(c + 1):
                    cp.wait()
            down(c)
            gate_up(c + 1, first)
            return carry
        lax.fori_loop(0, NC - 1, body, 0)

    cp_qkv("k").start()
    for u in range(4):
        cp_x(u).start()
    for cp in (cp_qkv("q"), cp_qkv("v"), cp_wo()) + cp_ffn(0) + cp_tails():
        cp.start()
    for c in range(1, NC):
        for cp in cp_ffn(c):
            cp.start()
    ob[0, 0:8, :] = jnp.zeros((8, 128), U32)
    a_ref[0, 0:8, :] = jnp.zeros((8, 128), U32)
    cp_qkv("k").wait()
    for _, fn in setup_qkv("k"):
        fn()
    for u in range(4):
        cp_x(u).wait()
        for t in range(X_SPLIT[u], X_SPLIT[u + 1]):
            x_to_rows(t)

    attention_block(0, True)
    ffn_loop(True)

    def pass_body(p, carry):
        attention_block(p, False)
        ffn_loop(False)
        return carry
    lax.fori_loop(1, 4, pass_body, 0)

    for b in range(3):
        tiles_to_rows(b, 0, range(NT_))

    def after(quad):
        tiles = [2 * (quad % 2) + t for t in (0, 1, 4, 5)]
        slabs = ((0,), (2, 1))[quad // 2]
        for b in slabs:
            tiles_to_rows(b, 1, tiles)
        if quad in (0, 3):
            for b in slabs:
                rows_to_out(b)
    down_final(None, None, after)
    for b, u in [(b, u) for b in range(2) for u in range(4)] + [(2, 0)]:
        cp_out(b, u).wait()


@jax.jit
def pallas_interleave_layers__sliding_local_dilated__glu_gated_bilinear__prompt_kernel(
    A_x: jax.Array,
    A_wqkv: jax.Array,
    A_wo: jax.Array,
    B_x: jax.Array,
    B_w_gate: jax.Array,
    B_w_up: jax.Array,
    B_w_down: jax.Array,
):
    del B_x
    vm = pltpu.VMEM
    scratch = [
        vm((D, S), BF), vm((D + 32, 3 * D), BF), vm((D + 64, D), BF),
        vm((NC, 512, FC), BF), vm((NC, 512, FC), BF), vm((NC, D, FC), BF),
        vm((D - 512, F), BF), vm((D - 512, F), BF),
        vm((6, 640, 128), F32),
        vm((8, 8, MQ // 2, 256), U32),
        vm((2 * NT_ + 1, D, 128), F32),
        vm((5, D, 128), F32),
        vm((5, D, 128), F32),
        vm((4, 992, 128), U32),
        vm((15, D, 128), F32),
        vm((16, D // 2, 128), F32),
        vm((16, D // 2, 128), F32),
        vm((NT_ + 1, W * H, 128), F32),
        vm((4, 960, 128), U32),
        vm((6, D, 128), F32),
        vm((6, S // 4, 128), F32),
        vm((49 * 128 + 32, 128), F32),
        vm((49, TQ // 2, 128), U32),
        vm((4, TQ // 2, 64), U32),
        vm((49, MQ, TQ), F32),
        vm((49, TQ // 2, 128), U32),
        vm((4, TQ, 256), F32),
        vm((16, TQ, 256), F32),
        vm((16, TQ, 128), F32),
        vm((NC, 49, 64, 256), U32),
        vm((NC, 3552, 128), U32),
        vm((NC, 4, 32, 256), U32),
        pltpu.SMEM((2,), jnp.int32),
        pltpu.SemaphoreType.DMA((11 + 3 * NC,)),
    ]
    hbm = pl.BlockSpec(memory_space=pl.ANY)
    out = pl.pallas_call(
        _kernel,
        in_specs=[hbm] * 6,
        out_specs=hbm,
        out_shape=jax.ShapeDtypeStruct((D, S), BF),
        scratch_shapes=scratch,
        compiler_params=pltpu.CompilerParams(vmem_limit_bytes=126 * 1024 * 1024),
    )(A_x.reshape(S, D).T, A_wqkv, A_wo, B_w_gate, B_w_up, B_w_down.T)
    return out.T.reshape(1, S, D)
```

```python
import math

import jax
import jax.numpy as jnp
from jax import lax
import jax.experimental.pallas as pl
import jax.experimental.pallas.tpu as pltpu

S, D, F = 2048, 576, 4608
H, DH, W = 32, 18, 8
NT_ = 8
TQ = 256
MQ = D // 4
FC = 512
NC = F // FC
X_SPLIT = (0, 5, 10, 14, 16)
O_SPLIT = ((0, 1, 3, 6, 10, 16), (0, 4, 8, 12, 16), (0, 16))
EPS = 1e-5
SCALE = DH ** -0.5
EXP_C = SCALE * math.log2(math.e)
NEG = -1e9 / SCALE

BF, F32, U32 = jnp.bfloat16, jnp.float32, jnp.uint32
NT_DIMS = (((1,), (1,)), ((), ()))

LHS_SEL = {0: ((0, 0), 1, (1, 1)), 1: ((1, 0), 1, (1, 1)), 2: ((0, 0), 0, None), 3: ((1, 1), 0, None),
           4: ((0, 0), 1, (0, 1)), 5: ((1, 0), -1, (0, 0)), 6: ((0, 1), -1, (1, 1))}
RHS_SEL = {0: ((0, 0), 1, (1, 1)), 1: ((0, 0), 0, None), 2: ((0, 1), -1, (1, 1)), 3: ((1, 0), -1, (0, 0)),
           4: ((1, 1), 0, None), 5: ((0, 0), 1, (0, 1)), 6: ((1, 0), 1, (1, 1))}
G_ORDER = (2, 0, 1, 5, 3, 4, 6)


def _lhs1(a11, a12, a21, a22):
    return [a11 + a22, a21 + a22, a11, a22, a11 + a12, a21 - a11, a12 - a22]


def _rhs1(b11, b12, b21, b22):
    return [b11 + b22, b11, b12 - b22, b21 - b11, b22, b11 + b12, b21 + b22]


def _in2(fn, x):
    outer = [[fn(x[i][j], x[i][2 + j], x[2 + i][j], x[2 + i][2 + j]) for j in range(2)] for i in range(2)]
    return [v for a in range(7) for v in fn(outer[0][0][a], outer[0][1][a], outer[1][0][a], outer[1][1][a])]


def _select(sel, load):
    first, sign, second = sel
    v = load(first)
    if sign == 1:
        v = [a + b for a, b in zip(v, load(second))]
    elif sign == -1:
        v = [a - b for a, b in zip(v, load(second))]
    return v


def _pk(lo, hi):
    return pltpu.pack_elementwise([lo, hi], packed_dtype=BF)


def _lo(w):
    return pltpu.unpack_elementwise(w, index=0, packed_dtype=BF, unpacked_dtype=F32)


def _hi(w):
    return pltpu.unpack_elementwise(w, index=1, packed_dtype=BF, unpacked_dtype=F32)


def _bf(w):
    return pltpu.bitcast(w, BF)


def _u32(x):
    return pltpu.bitcast(x.astype(BF), U32)


def _dot(a, b):
    return jnp.dot(a, b, preferred_element_type=F32)


def _kernel(x_hbm, wqkv_hbm, wo_hbm, wg_hbm, wu_hbm, wd_hbm, out_hbm,
            xio, wqkv_raw, wo_raw, wg_raw, wu_raw, wd_raw, tg, tu,
            wts, wt, xr, xm0, xm1, xn, kb, vb0, vb1, pb, ob, xf, xo, perm,
            a_ref, at_ref, acc, h_ref, ti, to, hf, r_ref, l_ref, t_ref, zero_ref, sems):
    def clear(i, carry):
        zero_ref[i] = 0
        return carry
    lax.fori_loop(0, 2, clear, 0)
    z = zero_ref[0]
    z2 = zero_ref[1]
    vbs = (vb0, vb1)
    ticks, clock = [], [0]
    xm = [((xm0, xm1)[r // 2 % 2], r // 4 * 2 + r % 2) for r in range(NT_)]

    def fence(ref, v):
        ref[z + (ref.shape[0] - 1), 0:8, 0:128] = v

    def gate(ref, fn):
        def job(v):
            if len(ref.shape) == 3:
                fence(ref, v)
            else:
                rows = pl.ds(pl.multiple_of(16 * z + (ref.shape[0] - 16), 16), 16)
                ref[rows, 0:128] = jnp.concatenate([v, v], axis=0).astype(ref.dtype)
            fn()
        return job

    def prime(ref, other):
        ref[z2 + (ref.shape[0] - 1), 0:8, 0:128] = pltpu.bitcast(other[z, 0:8, 0:128], F32)

    def paced(ref, fns, skew):
        last = []

        def job(v, fn):
            last.append(fn())
            if len(last) > skew:
                v = pltpu.bitcast(last.pop(0) ^ pltpu.bitcast(v, U32), F32)
            fence(ref, v)
        return [lambda v, fn=fn: job(v, fn) for fn in fns]

    def spread(jobs, n):
        slots = [lambda v: None] * n
        for i, job in enumerate(jobs):
            slots[i * n // len(jobs)] = job
        return slots

    def overlay(slots, start, step, jobs):
        for i, job in enumerate(jobs):
            k = start + step * i
            slots[k] = lambda v, old=slots[k], job=job: (old(v), job(v))

    def run(jobs, v, n=1):
        for _ in range(n):
            if jobs:
                jobs.pop(0)(v)

    def tree(fn, v):
        while len(v) > 1:
            v = [fn(v[i], v[i + 1]) for i in range(0, len(v), 2)]
        return v[0]

    def cp_x(u):
        cols = pl.ds(128 * X_SPLIT[u], 128 * (X_SPLIT[u + 1] - X_SPLIT[u]))
        return pltpu.make_async_copy(x_hbm.at[:, cols], xio.at[:, cols], sems.at[u])

    def cp_out(b, u):
        rows = pl.ds(256 * b, min(256, D - 256 * b))
        cols = pl.ds(128 * O_SPLIT[b][u], 128 * (O_SPLIT[b][u + 1] - O_SPLIT[b][u]))
        return pltpu.make_async_copy(xio.at[rows, cols], out_hbm.at[rows, cols], sems.at[8 * b + u])

    qkv_cols = {"k": pl.ds(512, 640), "v": pl.ds(1152, 576), "q": pl.ds(0, 512)}

    def cp_qkv(name):
        idx = 5 + "kvq".index(name)
        return pltpu.make_async_copy(wqkv_hbm.at[:, qkv_cols[name]], wqkv_raw.at[0:D, qkv_cols[name]], sems.at[idx])

    def cp_wo():
        return pltpu.make_async_copy(wo_hbm, wo_raw.at[0:D], sems.at[8])

    def cp_ffn(c):
        c0 = c * FC if isinstance(c, int) else pl.multiple_of(c * FC, FC)
        cols = pl.ds(c0, FC)
        return (pltpu.make_async_copy(wg_hbm.at[0:512, cols], wg_raw.at[c], sems.at[11 + 3 * c]),
                pltpu.make_async_copy(wu_hbm.at[0:512, cols], wu_raw.at[c], sems.at[12 + 3 * c]),
                pltpu.make_async_copy(wd_hbm.at[:, cols], wd_raw.at[c], sems.at[13 + 3 * c]))

    def cp_tails():
        return (pltpu.make_async_copy(wg_hbm.at[512:D, :], tg, sems.at[9]),
                pltpu.make_async_copy(wu_hbm.at[512:D, :], tu, sems.at[10]))

    def combine_steps(part, ref, rows):
        def combine(a, g):
            for j in range(2):
                w = _lhs1(rows(a, j, g), rows(a, 2 + j, g), rows(a + 2, j, g), rows(a + 2, 2 + j, g))
                for b in range(7):
                    wt[2 * part + a, b, 8 * g:8 * g + 8, 128 * j:128 * j + 128] = _u32(w[b])
                wt[2 * part + a, 7, 8 * g:8 * g + 8, 128 * j:128 * j + 64] = _u32(rows(a + 2 * j, 4, g)[:, :64])
        return [(ref, lambda a=a, g=g: combine(a, g)) for a in range(2) for g in range(MQ // 16)]

    def setup_qkv(name):
        part = "qkv".index(name)
        nb0 = (D * part) // 128
        base = D * part - 128 * nb0

        def transpose(nb):
            wn = min(128, D * part + D - 128 * nb)
            for kt in range(5):
                wk = 128 if kt < 4 else 64
                blk = wqkv_raw[128 * kt:128 * kt + wk, 128 * nb:128 * nb + wn].astype(F32)
                wts[kt, 128 * (nb - nb0):128 * (nb - nb0) + wn, 0:wk] = blk.T

        def rows(hg, kt, g):
            return jnp.concatenate([wts[kt, pl.ds(base + MQ * hg + 2 * g + e, 8, stride=DH), :]
                                    for e in range(2)], axis=0)
        return [(wqkv_raw, lambda nb=nb: transpose(nb)) for nb in range(nb0, nb0 + 5)] + combine_steps(part, wts, rows)

    def setup_wo():
        def transpose(nb):
            wn = 128 if nb < 4 else 64
            xf[nb, 0:D, 0:wn] = wo_raw[0:D, 128 * nb:128 * nb + wn].astype(F32)
            pair = [[_pk(*[xf[nb, pl.ds(MQ * hg + d + e, 8, stride=DH), :][:, :wn] for e in range(2)])
                     for d in range(0, DH, 2)] for hg in range(4)]
            for kt in range(5):
                w = pair[kt][:8] if kt < 4 else [pair[hg][8] for hg in range(4)]
                blk = _bf(jnp.concatenate(w, axis=0)).astype(F32).T
                hf[3 * kt + nb // 2, pl.ds(128 * (nb % 2), wn), 0:blk.shape[1]] = blk

        def rows(i, kt, g):
            row = MQ * i + 16 * g
            return hf[3 * kt + row // 256, pl.ds(row % 256, 16), :]
        return [(wo_raw, lambda nb=nb: transpose(nb)) for nb in range(5)] + combine_steps(3, hf, rows)

    def x_to_rows(t):
        x = xio[:, 128 * t:128 * t + 128]
        st, xs = {}, x.astype(F32)
        for g in range(D // 8):
            add_stats(st, g % 2, xs[8 * g:8 * g + 8])
        m, rs = mean_rstd({0: (st[0][0] + st[1][0], st[0][1] + st[1][1])}, 0)
        stat = jnp.where(lax.broadcasted_iota(jnp.int32, (32, 128), 0) == 0, m, rs)
        words = pltpu.bitcast(x, F32)
        for b in range(3):
            if b < 2:
                w = words[128 * b:128 * b + 128].T
            else:
                w = jnp.concatenate([words[256:288], stat], axis=0).T
                w = jnp.concatenate([w, jnp.zeros((128, 64), F32)], axis=1)
            for jj in range(8):
                perm[pl.ds(49 * (8 * t + jj) + b, 16, stride=3), :] = w[16 * jj:16 * jj + 16]

    def rows_to_tile(s, r, mr, slabs=range(3)):
        for b in slabs:
            w = perm[pl.ds(3 * (2 * r + s) + b, 128, stride=49), :]
            if b < 2:
                xr[8 * s + r, 256 * b:256 * b + 256, :] = _bf(w.T).astype(F32)
            else:
                w = w[:, :64].T
                xr[8 * s + r, 512:D, :] = _bf(w[0:32]).astype(F32)
                mr[r] = (w[32:33], w[33:34])

    def tiles_to_rows(b, s, tiles):
        nw = 128 if b < 2 else 32
        for r in tiles:
            if s == 0:
                w = _pk(xr[r, pl.ds(256 * b, nw, stride=2), :], xr[r, pl.ds(256 * b + 1, nw, stride=2), :])
            else:
                w = ob[z + r // 2, pl.ds(288 * (r % 2) + 128 * b, nw), :]
            w = jnp.concatenate([pltpu.bitcast(w, F32)] * (128 // nw), axis=0)
            perm[pl.ds(3 * (2 * r + s) + b, 128, stride=49), :] = w.T

    def rows_to_out(b):
        def rows(t):
            return jnp.concatenate([perm[pl.ds(49 * (8 * t + jj) + b, 16, stride=3), :] for jj in range(8)], axis=0)
        group = lax.broadcasted_iota(jnp.int32, (128, 128), 1) // 32
        for u in range(4):
            if b < 2:
                for t in range(4 * u, 4 * u + 4):
                    xio[256 * b:256 * b + 256, 128 * t:128 * t + 128] = _bf(rows(t).T)
                    if t + 1 in O_SPLIT[b]:
                        cp_out(b, O_SPLIT[b].index(t + 1) - 1).start()
            else:
                w = rows(4 * u)
                for t in range(1, 4):
                    w = jnp.where(group == t, rows(4 * u + t), w)
                w = _bf(w.T)
                for t in range(4):
                    xio[512:D, pl.ds(128 * (4 * u + t), 128)] = w[64 * t:64 * t + 64]
        if b == 2:
            cp_out(b, 0).start()

    def prep_r(c, a):
        for u in range(2):
            for g in range(8):
                def load(quad):
                    ws = [pltpu.bitcast((wg_raw, wu_raw)[u][c, pl.ds(128 * (2 * quad[0] + i) + 16 * g, 16),
                                                            pl.ds(256 * quad[1], 256)], U32) for i in range(2)]
                    ws = [w[:, 128 * j:128 * j + 128] for w in ws for j in range(2)]
                    return [_lo(w) for w in ws] + [_hi(w) for w in ws]
                v = _select(RHS_SEL[a], load)
                for b, (lo, hi) in enumerate(zip(_rhs1(*v[:4]), _rhs1(*v[4:]))):
                    r_ref[c, 7 * a + b, 8 * g:8 * g + 8, 128 * u:128 * u + 128] = _pk(lo, hi)

    def prep_l(c, g):
        ws = [pltpu.bitcast(wd_raw[c, pl.ds(MQ * i + 16 * g, 16), :], U32) for i in range(4)]
        ws = [[w[:, 128 * j:128 * j + 128] for j in range(4)] for w in ws]
        lo = _in2(_lhs1, [[_lo(w) for w in row] for row in ws])
        hi = _in2(_lhs1, [[_hi(w) for w in row] for row in ws])
        for k in range(49):
            l_ref[c, pl.ds(72 * k + 8 * g, 8), :] = _pk(lo[k], hi[k])

    def prep_a(a, half, g):
        src, row = (xf, xo)[g // 4], 32 * (g % 4) + half

        def load(quad):
            return [src[z2 + 2 * quad[1] + j, pl.ds(128 * (2 * quad[0] + i) + row + e, 8, stride=4), :]
                    for e in (0, 2) for i in range(2) for j in range(2)]
        v = _select(LHS_SEL[a], load)
        o = [_pk(lo, hi) for lo, hi in zip(_lhs1(*v[:4]), _lhs1(*v[4:]))]
        for b in range(7):
            a_ref[z + 7 * a + b, 64 * half + 8 * g:64 * half + 8 * g + 8, :] = o[b]
        return o[5] ^ o[6]

    def prep_a_tail():
        for i in range(4):
            for half in range(2):
                for u, src in enumerate((xf, xo)):
                    lo = src[z + 4, pl.ds(128 * i + half, 32, stride=4), :][:, :64]
                    hi = src[z + 4, pl.ds(128 * i + half + 2, 32, stride=4), :][:, :64]
                    at_ref[z + i, pl.ds(64 * half + 32 * u, 32), :] = _pk(lo, hi)

    def put(a):
        for g in range(16):
            def load(quad):
                return [hf[z + 4 * (2 * quad[1] + quad[0]) + t, pl.ds(o + 8 * g, 8), :]
                        for o in (0, 128) for t in (0, 2, 1, 3)]
            v = _select(RHS_SEL[a], load)
            for b, (lo, hi) in enumerate(zip(_rhs1(*v[:4]), _rhs1(*v[4:]))):
                h_ref[7 * a + b, 8 * g:8 * g + 8, :] = _pk(lo, hi)

    def strassen_inner(prod, nrow, emit, odd=None):
        ld = lambda s: ti[z + s, 0:nrow, :]
        for s in range(3):
            ti[z + s, 0:nrow, :] = prod(s)
        if not odd:
            emit(3, ((ld(0) - ld(1)) + ld(2)) + prod(5))
        m3 = prod(3)
        emit(2, ld(1) + m3)
        if odd is None:
            ti[z + 3, 0:nrow, :] = ld(0) + m3
        m4 = prod(4)
        emit(1, ld(2) + m4)
        ti[z + 3, 0:nrow, :] = (ld(3) if odd is None else ld(0) + m3) - m4
        if odd:
            emit(3, ((ld(0) - ld(1)) + ld(2)) + prod(5))
        emit(0, ld(3) + prod(6))

    def gate_up(c, first):
        if first:
            c0 = c * FC if isinstance(c, int) else pl.multiple_of(c * FC, FC)
            for g in range(MQ // 16):
                prep_l(c, g)
            for j in range(4):
                cols = pl.ds(c0 + 128 * j, 128)
                t_ref[c, j] = pltpu.bitcast(jnp.concatenate([tg[:, cols], tu[:, cols]], axis=1), U32)

        def inner(a, emit):
            if first:
                prep_r(c, a)
            strassen_inner(lambda b: _dot(_bf(a_ref[z + 7 * a + b]), _bf(r_ref[c, 7 * a + b])), TQ, emit)

        def fin(quad, q, v):
            i, j = 2 * (quad // 2) + q // 2, 2 * (quad % 2) + q % 2
            v = v + _dot(_bf(at_ref[z + i]), _bf(t_ref[c, j]))
            hf[z + 4 * quad + q] = v[:, :128] * v[:, 128:]

        def old(s, q):
            return to[z + 4 * s + q]

        def keep(s):
            def emit(q, v):
                to[z + 4 * s + q] = v
            return emit

        def emit3(q, v):
            fin(2, q, old(1, q) + v)
            to[z + 12 + q] = old(0, q) + v

        def emit4(q, v):
            fin(1, q, old(2, q) + v)
            to[z + 12 + q] = old(3, q) - v

        inner(2, keep(2))
        inner(0, keep(0))
        inner(1, keep(1))
        inner(5, lambda q, v: fin(3, q, ((old(0, q) - old(1, q)) + old(2, q)) + v))
        put(4)
        inner(3, emit3)
        put(2)
        inner(4, emit4)
        put(6)
        inner(6, lambda q, v: fin(0, q, old(3, q) + v))

    def down_prod(c, k, prev):
        return prev + lax.dot_general(_bf(l_ref[c, 72 * k:72 * k + 72, :]), _bf(h_ref[k]), NT_DIMS, preferred_element_type=F32)

    def down(c):
        for a, late in ((4, 1), (2, 0), (6, 3), (1, 5), (0, None), (3, None), (5, None)):
            for k in range(7 * a, 7 * a + 7):
                acc[k] = down_prod(c, k, jnp.where(c == 0, 0.0, acc[k]))
            if late is not None:
                put(late)

    def add_stats(st, r, x):
        st[r] = (x, x * x) if st.get(r) is None else (st[r][0] + x, st[r][1] + x * x)

    def mean_rstd(st, r):
        m = jnp.sum(st[r][0], axis=0, keepdims=True) * (1.0 / D)
        v = jnp.sum(st[r][1], axis=0, keepdims=True) * (1.0 / D) - m * m
        return m, lax.rsqrt(jnp.maximum(v, 0.0) + EPS)

    def down_final(base, st, after=None, between=()):
        odd = [False]

        def inner(a, emit, late=None):
            strassen_inner(lambda b: down_prod(NC - 1, 7 * a + b, acc[7 * a + b]), MQ, emit, odd[0] if between else None)
            if late is not None:
                put(late)
            if a in between:
                between[a]()
            else:
                odd[0] = not odd[0]

        def old(s, q):
            return to[z + 4 * s + q, 0:MQ, :]

        def keep(s, q, v):
            to[z + 4 * s + q, 0:MQ, :] = v

        def fin(quad, q, v):
            i, j = 2 * (quad // 2) + q // 2, 2 * (quad % 2) + q % 2
            rows = pl.ds(MQ * i, MQ)
            for e in range(2):
                r = j + 4 * e
                ref, slot = xm[r]
                x = ref[z + slot, rows, :] + v[:, 128 * e:128 * e + 128]
                if st is None:
                    ob[z + r // 2, pl.ds(288 * (r % 2) + 72 * i, 72), :] = _u32(x)
                    continue
                xr[base + r, rows, :] = x
                for g in range(MQ // 8):
                    add_stats(st, r, x[8 * g:8 * g + 8])
            if after is not None and q == 0:
                after(quad)

        inner(4, lambda q, v: keep(0, q, v), 0)
        inner(2, lambda q, v: (fin(1, q, old(0, q) + v), keep(1, q, v)), 3)
        inner(6, lambda q, v: keep(0, q, v - old(0, q)), 1)
        inner(0, lambda q, v: (keep(0, q, old(0, q) + v), keep(1, q, old(1, q) + v)), 5)
        inner(3, lambda q, v: (fin(0, q, old(0, q) + v), keep(2, q, v)))
        inner(1, lambda q, v: (fin(2, q, old(2, q) + v), keep(1, q, old(1, q) - v)))
        inner(5, lambda q, v: fin(3, q, old(1, q) + v))

    def chain(ref, last, v, skew=1):
        last.append(pltpu.bitcast(v, F32))
        if len(last) > skew:
            fence(ref, last.pop(0))

    def ln1_fns(base, mr, pairs):
        def norm(r, row, n):
            return (xr[base + r, pl.ds(row, n), :] - mr[r][0]) * mr[r][1]

        def job(u, g):
            if g == 16:
                y = jnp.concatenate([_u32(norm(2 * u + e, 512, 64)) for e in range(2)], axis=0)
                xn[u, 896:960, :] = y
                return tree(jnp.bitwise_xor, [y[8 * k:8 * k + 8] for k in range(8)])
            y = [_u32(v) for v in _rhs1(*[norm(2 * u + e, 256 * k + 16 * g, 16) for k in range(2) for e in range(2)])]
            for b in range(7):
                xn[u, pl.ds(128 * b + 8 * g, 8), :] = y[b]
            return y[5] ^ y[6]
        return [lambda u=u, g=g: job(u, g) for u in pairs for g in range(17)]

    def project(name, a, u, emit, x=None):
        w = 2 * "qkvo".index(name) + a
        src, slot = (ob, z + u) if name == "o" else (xn, u)
        rows = lambda i, n: src[slot, i:i + n, :] if x is None else x[i:i + n]

        def tick(y):
            clock[0] += 1
            for g in range(DH * (clock[0] % 2)):
                run(ticks, y[8 * g:8 * g + 8, 0:128])
            return y
        m = lambda b: tick(_dot(_bf(wt[w, b]), _bf(rows(128 * b, 128))))
        xt = lambda: _bf(jnp.concatenate([rows(896, 32), rows(928, 32)], axis=1))
        tail = lambda i: tick(_dot(_bf(wt[w, 7, :, 128 * i:128 * i + 64]), xt()))
        ta, m4 = tail(0), m(4)
        s11, s12 = ta[:, :128] - m4, ta[:, 128:] + m4
        s22 = m(2)
        emit(a, 2 * u + 1, s12 + s22)
        s11 = s11 + m(6)
        m0 = m(0)
        s11, s22 = s11 + m0, s22 + m0
        s21 = m(3)
        emit(a, 2 * u, s11 + s21)
        tb = tail(1)
        s21, s22 = s21 + tb[:, :128], s22 + tb[:, 128:]
        m1 = m(1)
        emit(a + 2, 2 * u, s21 + m1)
        emit(a + 2, 2 * u + 1, (s22 - m1) + m(5))

    def project_kv(name, a, u, jobs=(), every=1, x=None):
        def emit(hg, r, y):
            dst, rows = (kb, pl.ds(MQ * hg, MQ)) if name == "k" else (vbs[a], pl.ds(MQ * (hg // 2), MQ))
            dst[z + 7 + r, rows, :] = y
            if r >= 1:
                dst[z + r - 1, rows, :] = pltpu.roll(y, 1, 1)
            for g in range(0, DH, every):
                run(jobs, y[8 * g:8 * g + 8])
        project(name, a, u, emit, x)

    def prow(hg, w):
        return pl.ds(32 * w + 16 * (hg % 2) + 8 * (hg // 2), 8)

    def project_q(a, u, jobs):
        def emit(hg, r, y):
            lg = [None] * W
            for d in range(DH):
                q = y[8 * d:8 * d + 8]
                for w in range(W):
                    v = q * kb[z + 7 + r - w, pl.ds(MQ * hg + 8 * d, 8), :]
                    lg[w] = v if d == 0 else lg[w] + v
            for w in range(W):
                pb[z + r, prow(hg, w), :] = lg[w]
            if hg >= 2:
                jobs.append(softmax_job(r, a))
        project("q", a, u, emit)

    def softmax_job(r, sl):
        def job(v):
            fence(pb, v)
            lane0 = lax.broadcasted_iota(jnp.int32, (16, 128), 1) == 0
            lg = [pb[z2 + r, 32 * w + 16 * sl:32 * w + 16 * sl + 16, :] for w in range(W)]
            lg = [jnp.where(lane0, NEG, lg[w]) if w > r else lg[w] for w in range(W)]
            m = tree(jnp.maximum, lg)
            ex = [jnp.exp2((lg[w] - m) * EXP_C) for w in range(W)]
            inv = 1.0 / tree(jnp.add, ex)
            for w in range(W):
                pb[z2 + r, 32 * w + 16 * sl:32 * w + 16 * sl + 16, :] = ex[w] * inv
        return job

    def mix_jobs(a):
        o = {}

        def job(u, g, i):
            p = [[pb[z2 + 2 * u + e, prow(a + 2 * i, w), :] for w in range(W)] for e in range(2)]
            for d in range(2):
                v = [vbs[a][z2 + 2 * u + t, pl.ds(MQ * i + 16 * g + 8 * d, 8), :] for t in range(W + 1)]
                for e in range(2):
                    o[d, i, e] = tree(jnp.add, [p[e][w] * v[7 + e - w] for w in range(W)])
            if i == 0:
                y = pltpu.bitcast((o[0, 0, 0] + o[0, 0, 1]) + (o[1, 0, 0] + o[1, 0, 1]), U32)
                if (a, u, g) == (0, 0, 0):
                    xn[z, 960:968, :] = y
                return y
            lo, hi = [[o[d, i, e] for i in range(2) for e in range(2)] for d in range(2)]
            if g < 8:
                y = [_pk(*t) for t in zip(_rhs1(*lo), _rhs1(*hi))]
                for b in range(7):
                    ob[z + u, pl.ds(128 * b + 64 * a + 8 * g, 8), :] = y[b]
                return y[5] ^ y[6]
            y = [_pk(*t) for t in zip(lo, hi)]
            for k in range(4):
                ob[z + u, pl.ds(896 + 32 * (k % 2) + 8 * (a + 2 * (k // 2)), 8), :] = y[k]
            return tree(jnp.bitwise_xor, y)
        return paced(vbs[a], [lambda u=u, g=g, i=i: job(u, g, i)
                              for u in range(4) for g in range(9) for i in range(2)], 1)

    def ln2(st, r):
        m, rs = mean_rstd(st, r)
        (ref, slot), last = xm[r], []
        for kt in range(5):
            wk = 128 if kt < 4 else 64
            y = ((ref[z2 + slot, 128 * kt:128 * kt + wk, :] - m) * rs).T
            (xf, xo)[r // 4][z + kt, pl.ds(128 * (r % 4), 128), 0:wk] = y
            if kt < 4:
                chain(ref, last, y[0:8], 2)

    def prep_a_jobs(outer, odd):
        return paced((xf, xo)[odd], [lambda a=a, half=half, g=g: prep_a(a, half, g) for a in outer
                                     for half in range(2) for g in range(4 * odd, 4 * odd + 4)], 2)

    def out_proj(base, st, a, u, jobs):
        def emit(i, r, y):
            for g in range(MQ // 16):
                rows = pl.ds(MQ * i + 16 * g, 16)
                x = xr[base + r, rows, :] + y[16 * g:16 * g + 16]
                xm[r][0][z + xm[r][1], rows, :] = x
                add_stats(st, r, x[0:8])
                add_stats(st, r, x[8:16])
                if (i, r, clock[0] % 2) != (a + 2, 2 * u + 1, 0):
                    run(jobs, x[0:8])
        project("o", a, u, emit)

    def attention_block(p, first):
        s = 0 if first else p % 2
        cur, nxt = 8 * s, 8 * (1 - s)
        st1 = {}
        if first:
            st0 = {}
            for r in range(NT_):
                rows_to_tile(0, r, st0)
            for fn in ln1_fns(0, st0, (0, 1)):
                fn()
            ticks.extend(spread([], 90) + spread([lambda v: fence(xr, v)] + paced(xr, ln1_fns(z2, st0, (2, 3)), 2), 200))
            for u in range(2):
                for a in range(2):
                    project_kv("k", a, u)
            cp_qkv("q").wait()
            cp_qkv("v").wait()
            cp_wo().wait()
            steps = setup_qkv("q")
            for _, fn in steps[:5]:
                fn()
            wo_jobs = [gate(*step) for step in setup_wo()]
            ticks.extend(spread([], 108) + spread([gate(*step) for step in steps[5:]], 216))
            overlay(ticks, 90, 46, wo_jobs[:5])
            for u in range(2, 4):
                for a in range(2):
                    project_kv("k", a, u)
            tiles = [gate(perm, lambda r=r, b=b: rows_to_tile(1, r, st1, (b,))) for r in range(NT_) for b in range(3)]
            steps = [gate(*step) for step in setup_qkv("v")]
            mixed = steps[:5] + tiles[:6] + [job for pair in zip(steps[5:], tiles[6:]) for job in pair]
            ticks.extend(spread([], 36) + spread(mixed, 540))
        else:
            unit = {2: (0, 2), 0: (1, 2), 3: (0, 3), 1: (1, 3)}
            down_final(nxt, st1, None, {g: lambda g=g: project_kv("k", *unit[g]) for g in unit})
            st1 = {r: mean_rstd(st1, r) for r in range(NT_)}
        jobs = []
        for u in range(4):
            for a in range(2):
                project_q(a, u, jobs)
        if first:
            for cp in cp_ffn(0) + cp_tails():
                cp.wait()
        assert not ticks
        clock[0] = 0 if first else 1
        ticks.extend(spread(jobs + [lambda v: fence(pb, v)], 306))
        ln1 = [lambda v: fence(xr, v)] + paced(xr, ln1_fns(z2 + nxt, st1, range(4)), 2)
        for vb in vbs:
            prime(vb, ob)
        prime(xf, a_ref)
        prime(xo, a_ref)
        x0 = xn[0, 0:960, :]
        overlay(ticks, 93, 12, ln1[:18])
        if first:
            overlay(ticks, 50, 14, wo_jobs[5:])
        for u in range(4):
            project_kv("v", 0, u)
        assert not ticks
        ticks.extend(spread([], 24) + spread(mix_jobs(0), 300))
        for u in range(4):
            project_kv("v", 1, u, x=x0 if u == 0 else None)
        assert not ticks
        ticks.extend(spread([], 24) + spread(mix_jobs(1), 300))
        for a in range(2):
            project_kv("k", a, 0)
        st2, jobs = {}, []
        for u in range(4):
            if u == 1:
                jobs = spread(ln1[18:], 126)
            if u == 2:
                assert not ticks
                ticks.extend(spread([], 81) + spread(prep_a_jobs(G_ORDER, 0), 219) + spread(prep_a_jobs((2,), 1), 24))
            for a in range(2):
                out_proj(cur, st2, a, u, jobs)
            ln2(st2, 2 * u)
            ln2(st2, 2 * u + 1)
        assert not jobs and not ticks
        last = []
        project_kv("k", 0, 1)
        project_kv("k", 1, 1, [last.append])
        for a in G_ORDER[1:]:
            for half in range(2):
                for g in range(4, 8):
                    chain(xo, last, prep_a(a, half, g))
        prep_a_tail()
        gate_up(0, first)

    def ffn_loop(first):
        def body(c, carry):
            if first:
                for cp in cp_ffn(c + 1):
                    cp.wait()
            down(c)
            gate_up(c + 1, first)
            return carry
        lax.fori_loop(0, NC - 1, body, 0)

    cp_qkv("k").start()
    for u in range(4):
        cp_x(u).start()
    for cp in (cp_qkv("q"), cp_qkv("v"), cp_wo()) + cp_ffn(0) + cp_tails():
        cp.start()
    for c in range(1, NC):
        for cp in cp_ffn(c):
            cp.start()
    ob[0, 0:8, :] = jnp.zeros((8, 128), U32)
    a_ref[0, 0:8, :] = jnp.zeros((8, 128), U32)
    cp_qkv("k").wait()
    for _, fn in setup_qkv("k"):
        fn()
    for u in range(4):
        cp_x(u).wait()
        for t in range(X_SPLIT[u], X_SPLIT[u + 1]):
            x_to_rows(t)

    attention_block(0, True)
    ffn_loop(True)

    def pass_body(p, carry):
        attention_block(p, False)
        ffn_loop(False)
        return carry
    lax.fori_loop(1, 4, pass_body, 0)

    for b in range(3):
        tiles_to_rows(b, 0, range(NT_))

    def after(quad):
        tiles = [2 * (quad % 2) + t for t in (0, 1, 4, 5)]
        slabs = ((0,), (2, 1))[quad // 2]
        for b in slabs:
            tiles_to_rows(b, 1, tiles)
        if quad in (0, 3):
            for b in slabs:
                rows_to_out(b)
    down_final(None, None, after)
    for b in range(3):
        for u in range(len(O_SPLIT[b]) - 1):
            cp_out(b, u).wait()


@jax.jit
def pallas_interleave_layers__sliding_local_dilated__glu_gated_bilinear__prompt_kernel(
    A_x: jax.Array,
    A_wqkv: jax.Array,
    A_wo: jax.Array,
    B_x: jax.Array,
    B_w_gate: jax.Array,
    B_w_up: jax.Array,
    B_w_down: jax.Array,
):
    del B_x
    vm = pltpu.VMEM
    scratch = [
        vm((D, S), BF), vm((D + 32, 3 * D), BF), vm((D + 64, D), BF),
        vm((NC, 512, FC), BF), vm((NC, 512, FC), BF), vm((NC, D, FC), BF),
        vm((D - 512, F), BF), vm((D - 512, F), BF),
        vm((6, 640, 128), F32),
        vm((8, 8, MQ // 2, 256), U32),
        vm((2 * NT_ + 1, D, 128), F32),
        vm((5, D, 128), F32),
        vm((5, D, 128), F32),
        vm((4, 992, 128), U32),
        vm((15, D, 128), F32),
        vm((16, D // 2, 128), F32),
        vm((16, D // 2, 128), F32),
        vm((NT_ + 1, W * H, 128), F32),
        vm((4, 960, 128), U32),
        vm((6, D, 128), F32),
        vm((6, S // 4, 128), F32),
        vm((49 * 128 + 32, 128), F32),
        vm((49, TQ // 2, 128), U32),
        vm((4, TQ // 2, 64), U32),
        vm((49, MQ, TQ), F32),
        vm((49, TQ // 2, 128), U32),
        vm((4, TQ, 256), F32),
        vm((16, TQ, 256), F32),
        vm((16, TQ, 128), F32),
        vm((NC, 49, 64, 256), U32),
        vm((NC, 3552, 128), U32),
        vm((NC, 4, 32, 256), U32),
        pltpu.SMEM((2,), jnp.int32),
        pltpu.SemaphoreType.DMA((11 + 3 * NC,)),
    ]
    hbm = pl.BlockSpec(memory_space=pl.ANY)
    out = pl.pallas_call(
        _kernel,
        in_specs=[hbm] * 6,
        out_specs=hbm,
        out_shape=jax.ShapeDtypeStruct((D, S), BF),
        scratch_shapes=scratch,
        compiler_params=pltpu.CompilerParams(vmem_limit_bytes=126 * 1024 * 1024),
    )(A_x.reshape(S, D).T, A_wqkv, A_wo, B_w_gate, B_w_up, B_w_down.T)
    return out.T.reshape(1, S, D)
```
